```python
import jax
import jax.numpy as jnp

def _softmax(x, axis=-1):
    return jax.nn.softmax(x, axis=axis)

def _gelu(x):
    return jax.nn.gelu(x, approximate=True)

def _silu(x):
    return jax.nn.silu(x)

def _sigmoid(x):
    return jax.nn.sigmoid(x)

def _layernorm(x, axis=-1, eps=1e-05):
    m = jnp.mean(x, axis=axis, keepdims=True)
    v = jnp.var(x, axis=axis, keepdims=True)
    return (x - m) / jnp.sqrt(v + eps)

def _scatter_add(tgt, idx, src, axis=0):
    return tgt.at[idx].add(src)

def _segment_sum(src, seg, n):
    return jax.ops.segment_sum(src, seg, n)

class _Rng:

    def __init__(self, key):
        self._k = key

    def _next(self):
        self._k, sub = jax.random.split(self._k)
        return sub

    def normal(self, shape):
        return jax.random.normal(self._next(), shape, dtype=jnp.bfloat16)

    def randint(self, lo, hi, shape):
        return jax.random.randint(self._next(), shape, lo, hi, dtype=jnp.int32)

    def uniform(self, shape, lo=0.0, hi=1.0):
        return jax.random.uniform(self._next(), shape, jnp.bfloat16, lo, hi)

    def permutation(self, n):
        return jax.random.permutation(self._next(), n)
kernel_name = 'interleave_layers__memory_aug_recurrent_mem_tr__glu_gated_swiglu__prompt'

def setup_inputs():
    _rng = _Rng(jax.random.key(int.from_bytes(__import__("os").urandom(4), "little")))
    _w = lambda a: (lambda t: t.astype(jnp.bfloat16) if jnp.issubdtype(t.dtype, jnp.floating) else t)(jnp.asarray(a))

    def _A_setup():
        B, S, Dm = (1, 2048, 576)
        H, Dh = (32, 128)
        M, seg = (8, 32)
        seg = min(seg, S)
        S = S // seg * seg
        return {'x': _w((lambda *s: _rng.normal(s) * 0.05)(B, S, Dm)), 'mem0': _w((lambda *s: _rng.normal(s) * 0.05)(B, M, Dm)), 'Wq': _w((lambda *s: _rng.normal(s) * 0.05)(Dm, H, Dh) * Dm ** (-0.5)), 'Wk': _w((lambda *s: _rng.normal(s) * 0.05)(Dm, H, Dh) * Dm ** (-0.5)), 'Wv': _w((lambda *s: _rng.normal(s) * 0.05)(Dm, H, Dh) * Dm ** (-0.5)), 'Wo': _w((lambda *s: _rng.normal(s) * 0.05)(H, Dh, Dm) * (H * Dh) ** (-0.5)), 'seg_len': seg}
    _A_in = _A_setup()

    def _B_setup():
        B, S, D, F = (1, 2048, 576, 4608)
        return {'x': _w((lambda *s: _rng.normal(s) * 0.05)(B, S, D)), 'w1': _w((lambda *s: _rng.normal(s) * 0.05)(D, F) * (2.0 / D) ** 0.5), 'w3': _w((lambda *s: _rng.normal(s) * 0.05)(D, F) * (2.0 / D) ** 0.5), 'w2': _w((lambda *s: _rng.normal(s) * 0.05)(F, D) * (2.0 / F) ** 0.5)}
    _B_in = _B_setup()
    return {'A_x': _A_in['x'], 'A_mem0': _A_in['mem0'], 'A_Wq': _A_in['Wq'], 'A_Wk': _A_in['Wk'], 'A_Wv': _A_in['Wv'], 'A_Wo': _A_in['Wo'], 'A_seg_len': _A_in['seg_len'], 'B_x': _B_in['x'], 'B_w1': _B_in['w1'], 'B_w3': _B_in['w3'], 'B_w2': _B_in['w2']}

def reference(A_x, A_mem0, A_Wq, A_Wk, A_Wv, A_Wo, A_seg_len, B_x, B_w1, B_w3, B_w2):

    def _A_ref(x, mem0, Wq, Wk, Wv, Wo, seg_len):
        B, S, Dm = x.shape
        H, Dh = (Wq.shape[1], Wq.shape[2])
        M = mem0.shape[1]
        scale = Dh ** (-0.5)
        n_seg = S // seg_len
        L = M + seg_len
        idx = jnp.arange(L)
        mask = (idx[:, None] < M) | (idx[:, None] >= idx[None, :])
        mem = mem0
        outs = []
        for s in range(n_seg):
            xs = x[:, s * seg_len:(s + 1) * seg_len, :].copy()
            h = jnp.concatenate([mem, xs], axis=1)
            q = jnp.einsum('btd,dhe->bhte', h, Wq)
            k = jnp.einsum('btd,dhe->bhte', h, Wk)
            v = jnp.einsum('btd,dhe->bhte', h, Wv)
            scores = jnp.einsum('bhqe,bhke->bhqk', q, k) * scale
            scores = jnp.where(mask[None, None], scores, -1000000000.0)
            p = _softmax(scores, axis=-1)
            o = jnp.einsum('bhqk,bhke->bhqe', p, v)
            o = jnp.einsum('bhte,hed->btd', o, Wo)
            mem = o[:, :M, :].copy()
            outs.append(o[:, M:, :])
        return jnp.concatenate(outs, axis=1)

    def _B_ref(x, w1, w3, w2):
        gate = jnp.einsum('bsd,df->bsf', x, w1)
        up = jnp.einsum('bsd,df->bsf', x, w3)
        h = _silu(gate) * up
        out = jnp.einsum('bsf,fd->bsd', h, w2)
        return out
    x = A_x
    x = x + _A_ref(_layernorm(x, axis=-1), A_mem0, A_Wq, A_Wk, A_Wv, A_Wo, A_seg_len)
    x = x + _B_ref(_layernorm(x, axis=-1), B_w1, B_w3, B_w2)
    x = x + _A_ref(_layernorm(x, axis=-1), A_mem0, A_Wq, A_Wk, A_Wv, A_Wo, A_seg_len)
    x = x + _B_ref(_layernorm(x, axis=-1), B_w1, B_w3, B_w2)
    return x
```

```python
import functools
import math

import jax
import jax.numpy as jnp
from jax import lax
import jax.experimental.pallas as pl
import jax.experimental.pallas.tpu as pltpu

F32 = jnp.float32
BF16 = jnp.bfloat16
U32 = jnp.uint32
LANES = 128
HEADS_PER_GROUP = 4
FFN_CHUNK = 512
RELAYOUT_ROWS = 64
DMA_DEPTH = 2
LN_EPS = 1e-5
MASK_VALUE = -1000000000.0
LOG2E = math.log2(math.e)
NT_DIMS = (((1,), (1,)), ((), ()))


def _pack(w):
    return pltpu.bitcast(w, U32)


def _unpack(w):
    return pltpu.bitcast(w, BF16)


def _layernorm(x):
    mean = jnp.mean(x, axis=-1, keepdims=True)
    cen = x - mean
    var = jnp.mean(cen * cen, axis=-1, keepdims=True)
    return cen * lax.rsqrt(var + LN_EPS)


def _attention_mask(n_layers, seg, n_mem):
    rows = n_layers * (seg + n_mem)
    n_tok = n_layers * seg

    def describe(axis):
        i = lax.broadcasted_iota(jnp.int32, (rows, rows), axis)
        is_mem = i >= n_tok
        layer = jnp.zeros_like(i)
        pos = jnp.where(is_mem, i - n_tok, i + n_mem)
        for l in range(1, n_layers):
            in_l = jnp.where(is_mem, i - n_tok - l * n_mem, i - l * seg) >= 0
            layer = jnp.where(in_l, l, layer)
        pos = pos - layer * jnp.where(is_mem, n_mem, seg)
        return layer, pos

    q_layer, q_pos = describe(0)
    k_layer, k_pos = describe(1)
    same = q_layer == k_layer
    visible = same & ((q_pos < n_mem) | (q_pos >= k_pos))
    fill = jnp.where(same, MASK_VALUE * LOG2E, -jnp.inf).astype(F32)
    return visible, fill


def _kernel(xT_hbm, mem0_ref, wq_hbm, wk_hbm, wv_hbm, woT_hbm, w1_hbm, w3_hbm, w2T_hbm,
            outT_hbm,
            stage, woT, w1_raw, w3_raw, w2T, wqkv, wo, w1, w3, w2, xT, xs, ys, outT, mem, a_out, f_in, b_out, sems,
            *, seg, n_seg, n_heads, head_dim):
    d_model = xs.shape[1]
    n_mem = mem0_ref.shape[0]
    n_groups = n_heads // HEADS_PER_GROUP
    group_w = HEADS_PER_GROUP * head_dim
    n_chunks = w1_raw.shape[1] // FFN_CHUNK
    segs_per_blk = LANES // seg
    n_blk = n_seg // segs_per_blk
    score_scale = head_dim ** -0.5 * LOG2E

    copies = [
        pltpu.make_async_copy(src, dst, sems.at[i])
        for i, (src, dst) in enumerate([
            (xT_hbm, xT), (wq_hbm, stage.at[0]), (wk_hbm, stage.at[1]), (wv_hbm, stage.at[2]),
            (woT_hbm, woT), (w2T_hbm, w2T), (w1_hbm, w1_raw), (w3_hbm, w3_raw)])
    ]
    def arrive(i):
        if i + DMA_DEPTH < len(copies):
            copies[i + DMA_DEPTH].start()
        copies[i].wait()

    for c in copies[:DMA_DEPTH]:
        c.start()
    arrive(0)
    for b in range(n_blk):
        blk = xT[:, b * LANES:(b + 1) * LANES].astype(F32)
        xs[b * LANES:(b + 1) * LANES, :] = blk.T.astype(BF16)
    ys[...] = jnp.zeros(ys.shape, ys.dtype)
    a_out[...] = jnp.zeros(a_out.shape, a_out.dtype)
    f_in[...] = jnp.zeros(f_in.shape, f_in.dtype)
    b_out[...] = jnp.zeros(b_out.shape, b_out.dtype)
    mem0 = mem0_ref[...].astype(F32)
    mem[...] = jnp.concatenate([mem0, mem0], axis=0)

    pairs = n_heads // 2
    for m in range(3):
        arrive(1 + m)
        words = stage.at[m].bitcast(jnp.uint32)

        def split_heads(i, carry, m=m, words=words):
            d0 = pl.multiple_of(i * RELAYOUT_ROWS, RELAYOUT_ROWS)
            slab = words.at[pl.ds(pl.multiple_of(d0 * pairs, RELAYOUT_ROWS * pairs),
                                  RELAYOUT_ROWS * pairs)]
            for p in range(pairs):
                w = slab[pl.ds(p, RELAYOUT_ROWS, stride=pairs), :]
                even = lax.bitcast_convert_type(w << 16, F32)
                odd = lax.bitcast_convert_type(w & jnp.uint32(0xFFFF0000), F32)
                g, h = divmod(2 * p, HEADS_PER_GROUP)
                col = m * group_w + h * head_dim
                rows = pl.ds(pl.multiple_of(i * (RELAYOUT_ROWS // 2), RELAYOUT_ROWS // 2),
                             RELAYOUT_ROWS // 2)
                wqkv[g, rows, col:col + head_dim] = _pack(even.astype(BF16))
                wqkv[g, rows, col + head_dim:col + 2 * head_dim] = _pack(odd.astype(BF16))
            return carry

        lax.fori_loop(0, d_model // RELAYOUT_ROWS, split_heads, 0)

    arrive(4)

    def transpose_wo(h, carry):
        rows = pl.ds(pl.multiple_of(h * (head_dim // 2), head_dim // 2), head_dim // 2)
        wo[rows, :] = _pack(woT[h].astype(F32).T.astype(BF16))
        return carry

    lax.fori_loop(0, n_heads, transpose_wo, 0)
    arrive(5)
    for j in range(w2T.shape[1] // LANES):
        blk = w2T[:, j * LANES:(j + 1) * LANES].astype(F32)
        w2[j * (LANES // 2):(j + 1) * (LANES // 2), :] = _pack(blk.T.astype(BF16))
    for i, (raw, packed) in enumerate([(w1_raw, w1), (w3_raw, w3)]):
        arrive(6 + i)

        def repack(r, carry, raw=raw, packed=packed):
            src = pl.ds(pl.multiple_of(r * RELAYOUT_ROWS, RELAYOUT_ROWS), RELAYOUT_ROWS)
            dst = pl.ds(pl.multiple_of(r * (RELAYOUT_ROWS // 2), RELAYOUT_ROWS // 2),
                        RELAYOUT_ROWS // 2)
            packed[dst, :] = _pack(raw[src, :])
            return carry

        lax.fori_loop(0, d_model // RELAYOUT_ROWS, repack, 0)

    def emit_output(s, y):
        ys[pl.ds(pl.multiple_of(s * seg, seg), seg), :] = y
        b = s // segs_per_blk
        rows = ys[pl.ds(pl.multiple_of(b * LANES, LANES), LANES), :]
        outT[b] = rows.T.astype(BF16)

    def step(t, carry):
        visible, fill = _attention_mask(2, seg, n_mem)
        f_lhs = f_in[...]

        def ffn_chunk(c):
            cols = slice(c * FFN_CHUNK, (c + 1) * FFN_CHUNK)
            gate = jnp.dot(f_lhs, _unpack(w1[:, cols]), preferred_element_type=F32)
            up = jnp.dot(f_lhs, _unpack(w3[:, cols]), preferred_element_type=F32)
            hid = (gate * jax.nn.sigmoid(gate) * up).astype(BF16)
            rows = slice(c * FFN_CHUNK // 2, (c + 1) * FFN_CHUNK // 2)
            return jnp.dot(hid, _unpack(w2[rows, :]), preferred_element_type=F32)

        prev = b_out[...]
        x2 = prev[:seg]
        emit_output(jnp.maximum(t - 4, 0), prev[seg:])
        s1 = jnp.minimum(t, n_seg - 1)
        x1 = xs[pl.ds(pl.multiple_of(s1 * seg, seg), seg), :].astype(F32)
        resid = jnp.concatenate([x1, x2], axis=0)
        mem_row = lax.broadcasted_iota(jnp.int32, mem.shape, 0)
        restart = (mem_row >= n_mem) & (t <= 2)
        mem_in = jnp.where(restart, jnp.concatenate([mem0, mem0], axis=0), mem[...])
        a_lhs = jnp.concatenate([_layernorm(resid), mem_in], axis=0).astype(BF16)

        def project(g):
            return jnp.dot(a_lhs, _unpack(wqkv[g]), preferred_element_type=F32).astype(BF16)

        def attend(g, qkv):
            heads = []
            for i in range(HEADS_PER_GROUP):
                q, k, v = (qkv[:, m * group_w + i * head_dim:m * group_w + (i + 1) * head_dim]
                           for m in range(3))
                s = lax.dot_general(q, k, NT_DIMS, preferred_element_type=F32)
                s = jnp.where(visible, s * score_scale, fill)
                p = jnp.exp2(s - jnp.max(s, axis=-1, keepdims=True))
                denom = jnp.sum(p, axis=-1, keepdims=True)
                o = jnp.dot(p.astype(BF16), v, preferred_element_type=F32) / denom
                heads.append(o.astype(BF16))
            rows = slice(g * group_w // 2, (g + 1) * group_w // 2)
            return jnp.dot(jnp.concatenate(heads, axis=1), _unpack(wo[rows, :]),
                           preferred_element_type=F32)

        b_acc = a_out[...] + ffn_chunk(0)
        a_acc = None
        qkv = project(0)
        for g in range(n_groups):
            nxt = project(g + 1) if g + 1 < n_groups else None
            part = attend(g, qkv)
            a_acc = part if a_acc is None else a_acc + part
            qkv = nxt
            if g + 1 < n_chunks - 1:
                b_acc = b_acc + ffn_chunk(g + 1)
        tokens = resid + a_acc[:2 * seg]
        mem[...] = a_acc[2 * seg:]
        a_out[...] = tokens
        f_in[...] = _layernorm(tokens).astype(BF16)
        for c in range(min(n_groups, n_chunks - 1), n_chunks):
            b_acc = b_acc + ffn_chunk(c)
        b_out[...] = b_acc
        return carry

    lax.fori_loop(0, n_seg + 3, step, 0)
    emit_output(n_seg - 1, b_out[seg:, :])

    out_copies = [
        pltpu.make_async_copy(outT.at[b], outT_hbm.at[:, b * LANES:(b + 1) * LANES], sems.at[8])
        for b in range(n_blk)
    ]
    for c in out_copies:
        c.start()
    for c in out_copies:
        c.wait()


@functools.partial(jax.jit, static_argnames=("A_seg_len",))
def pallas_interleave_layers__memory_aug_recurrent_mem_tr__glu_gated_swiglu__prompt_kernel(
    A_x, A_mem0, A_Wq, A_Wk, A_Wv, A_Wo, A_seg_len, B_x, B_w1, B_w3, B_w2,
):
    del B_x
    batch, seq, d_model = A_x.shape
    _, n_heads, head_dim = A_Wq.shape
    n_mem = A_mem0.shape[1]
    d_ff = B_w1.shape[1]
    seg = int(A_seg_len)
    n_seg = seq // seg
    assert batch == 1 and n_seg * seg == seq and LANES % seg == 0 and seq % LANES == 0
    assert head_dim == LANES and n_heads % HEADS_PER_GROUP == 0 and d_ff % FFN_CHUNK == 0

    n_groups = n_heads // HEADS_PER_GROUP
    hbm = pl.BlockSpec(memory_space=pl.ANY)
    outT = pl.pallas_call(
        functools.partial(_kernel, seg=seg, n_seg=n_seg, n_heads=n_heads, head_dim=head_dim),
        out_shape=jax.ShapeDtypeStruct((d_model, seq), A_x.dtype),
        in_specs=[hbm, pl.BlockSpec(memory_space=pltpu.VMEM)] + [hbm] * 7,
        out_specs=hbm,
        scratch_shapes=[
            pltpu.VMEM((3, d_model * n_heads, head_dim), BF16),
            pltpu.VMEM((n_heads, d_model, head_dim), BF16),
            pltpu.VMEM((d_model, d_ff), BF16),
            pltpu.VMEM((d_model, d_ff), BF16),
            pltpu.VMEM((d_model, d_ff), BF16),
            pltpu.VMEM((n_groups, d_model // 2, 3 * HEADS_PER_GROUP * head_dim), U32),
            pltpu.VMEM((n_heads * head_dim // 2, d_model), U32),
            pltpu.VMEM((d_model // 2, d_ff), U32),
            pltpu.VMEM((d_model // 2, d_ff), U32),
            pltpu.VMEM((d_ff // 2, d_model), U32),
            pltpu.VMEM((d_model, seq), BF16),
            pltpu.VMEM((seq, d_model), BF16),
            pltpu.VMEM((seq, d_model), F32),
            pltpu.VMEM((seq // LANES, d_model, LANES), BF16),
            pltpu.VMEM((2 * n_mem, d_model), F32),
            pltpu.VMEM((2 * seg, d_model), F32),
            pltpu.VMEM((2 * seg, d_model), BF16),
            pltpu.VMEM((2 * seg, d_model), F32),
            pltpu.SemaphoreType.DMA((9,)),
        ],
        compiler_params=pltpu.CompilerParams(vmem_limit_bytes=110 * 2**20),
    )(
        A_x.reshape(seq, d_model).T,
        A_mem0.reshape(n_mem, d_model),
        A_Wq.reshape(d_model * n_heads, head_dim),
        A_Wk.reshape(d_model * n_heads, head_dim),
        A_Wv.reshape(d_model * n_heads, head_dim),
        A_Wo.transpose(0, 2, 1),
        B_w1,
        B_w3,
        B_w2.T,
    )
    return outT.T.reshape(batch, seq, d_model)
```

```python
import functools
import math

import jax
import jax.numpy as jnp
from jax import lax
import jax.experimental.pallas as pl
import jax.experimental.pallas.tpu as pltpu

F32 = jnp.float32
BF16 = jnp.bfloat16
U32 = jnp.uint32
LANES = 128
HEADS_PER_GROUP = 4
FFN_CHUNK = 512
RELAYOUT_ROWS = 64
DMA_DEPTH = 2
FILL_START = 2
FILL_FIRST = 2
FILL_SOFTMAX = 2
FILL_PROJECT = (0, 1, 0, 0, 1, 0, 0)
FILL_LAST = 2
LN_EPS = 1e-5
MASK_VALUE = -1000000000.0
LOG2E = math.log2(math.e)
NT_DIMS = (((1,), (1,)), ((), ()))


def _pack(w):
    return pltpu.bitcast(w, U32)


def _unpack(w):
    return pltpu.bitcast(w, BF16)


def _layernorm(x):
    mean = jnp.mean(x, axis=-1, keepdims=True)
    cen = x - mean
    var = jnp.mean(cen * cen, axis=-1, keepdims=True)
    return cen * lax.rsqrt(var + LN_EPS)


def _attention_mask(n_layers, seg, n_mem):
    rows = n_layers * (seg + n_mem)
    n_tok = n_layers * seg

    def describe(axis):
        i = lax.broadcasted_iota(jnp.int32, (rows, rows), axis)
        is_mem = i >= n_tok
        layer = jnp.zeros_like(i)
        pos = jnp.where(is_mem, i - n_tok, i + n_mem)
        for l in range(1, n_layers):
            in_l = jnp.where(is_mem, i - n_tok - l * n_mem, i - l * seg) >= 0
            layer = jnp.where(in_l, l, layer)
        pos = pos - layer * jnp.where(is_mem, n_mem, seg)
        return layer, pos

    q_layer, q_pos = describe(0)
    k_layer, k_pos = describe(1)
    same = q_layer == k_layer
    visible = same & ((q_pos < n_mem) | (q_pos >= k_pos))
    fill = jnp.where(same, MASK_VALUE * LOG2E, -jnp.inf).astype(F32)
    return visible, fill


class _Ffn:
    def __init__(self, lhs, resid, w1, w3, w2, n_chunks):
        self.lhs, self.acc = lhs, resid
        self.w1, self.w3, self.w2 = w1, w3, w2
        self.gate, self.hidden = {}, {}
        self.todo = []
        for c in range(n_chunks):
            self.todo += [(self._gate, c), (self._up, c)]
            if c > 0:
                self.todo.append((self._down, c - 1))
        self.todo.append((self._down, n_chunks - 1))

    def _project(self, w, c):
        cols = slice(c * FFN_CHUNK, (c + 1) * FFN_CHUNK)
        return jnp.dot(self.lhs, _unpack(w[:, cols]), preferred_element_type=F32)

    def _gate(self, c):
        gate = self._project(self.w1, c)
        self.gate[c] = gate * jax.nn.sigmoid(gate)

    def _up(self, c):
        self.hidden[c] = (self.gate.pop(c) * self._project(self.w3, c)).astype(BF16)

    def _down(self, c):
        rows = slice(c * FFN_CHUNK // 2, (c + 1) * FFN_CHUNK // 2)
        self.acc = self.acc + jnp.dot(self.hidden.pop(c), _unpack(self.w2[rows, :]),
                                      preferred_element_type=F32)

    def run(self, count):
        for fn, c in self.todo[:count]:
            fn(c)
        self.todo = self.todo[count:]

    def finish(self):
        self.run(len(self.todo))
        return self.acc


def _attention(resid, mem, wqkv, wo, ffn, *, seg, head_dim):
    n_groups = wqkv.shape[0]
    group_w = HEADS_PER_GROUP * head_dim
    n_tok = resid.shape[0]
    n_layers = n_tok // seg
    visible, fill = _attention_mask(n_layers, seg, mem.shape[0] // n_layers)
    score_scale = head_dim ** -0.5 * LOG2E
    lhs = jnp.concatenate([_layernorm(resid), mem], axis=0).astype(BF16)

    def project(g):
        return jnp.dot(lhs, _unpack(wqkv[g]), preferred_element_type=F32).astype(BF16)

    def head(qkv, m, i):
        return qkv[:, m * group_w + i * head_dim:m * group_w + (i + 1) * head_dim]

    def scores(qkv):
        probs = []
        for i in range(HEADS_PER_GROUP):
            s = lax.dot_general(head(qkv, 0, i), head(qkv, 1, i), NT_DIMS,
                                preferred_element_type=F32)
            s = jnp.where(visible, s * score_scale, fill)
            p = jnp.exp2(s - jnp.max(s, axis=-1, keepdims=True))
            probs.append((p.astype(BF16), 1.0 / jnp.sum(p, axis=-1, keepdims=True)))
        return probs

    def mix(qkv, probs):
        return jnp.concatenate(
            [(jnp.dot(p, head(qkv, 2, i), preferred_element_type=F32) * inv).astype(BF16)
             for i, (p, inv) in enumerate(probs)], axis=1)

    def output(g, o, acc):
        rows = slice(g * group_w // 2, (g + 1) * group_w // 2)
        part = jnp.dot(o, _unpack(wo[rows, :]), preferred_element_type=F32)
        return part if acc is None else acc + part

    acc = None
    if ffn is not None:
        ffn.run(FILL_START)
        qkv = project(0)
        ffn.run(FILL_FIRST)
        for g in range(n_groups):
            probs = scores(qkv)
            ffn.run(FILL_SOFTMAX)
            o = mix(qkv, probs)
            if g + 1 < n_groups:
                qkv = project(g + 1)
                ffn.run(FILL_PROJECT[g % len(FILL_PROJECT)])
            else:
                ffn.run(FILL_LAST)
            acc = output(g, o, acc)
    else:
        qkv, o = project(0), None
        nxt = project(1)
        for g in range(n_groups):
            probs = scores(qkv)
            if o is not None:
                acc = output(g - 1, o, acc)
            after = project(g + 2) if g + 2 < n_groups else None
            o = mix(qkv, probs)
            qkv, nxt = nxt, after
        acc = output(n_groups - 1, o, acc)
    return resid + acc[:n_tok], acc[n_tok:]


def _kernel(xT_hbm, mem0_ref, wq_hbm, wk_hbm, wv_hbm, woT_hbm, w1_hbm, w3_hbm, w2T_hbm,
            outT_hbm,
            stage, woT, w1_raw, w3_raw, w2T, wqkv, wo, w1, w3, w2, xT, xs, ys, outT,
            mem, a_out, f_in, b_out, in_sems, out_sems,
            *, seg, n_seg, n_heads, head_dim):
    d_model = xs.shape[1]
    n_mem = mem0_ref.shape[0]
    group_w = HEADS_PER_GROUP * head_dim
    n_chunks = w1_raw.shape[1] // FFN_CHUNK
    segs_per_blk = LANES // seg
    n_blk = n_seg // segs_per_blk
    attention = functools.partial(_attention, wqkv=wqkv, wo=wo, seg=seg, head_dim=head_dim)

    copies = [
        pltpu.make_async_copy(src, dst, in_sems.at[i])
        for i, (src, dst) in enumerate([
            (xT_hbm, xT), (wq_hbm, stage.at[0]), (wk_hbm, stage.at[1]), (wv_hbm, stage.at[2]),
            (woT_hbm, woT), (w2T_hbm, w2T), (w1_hbm, w1_raw), (w3_hbm, w3_raw)])
    ]

    def out_copy(b):
        cols = pl.ds(pl.multiple_of(b * LANES, LANES), LANES)
        return pltpu.make_async_copy(outT.at[b], outT_hbm.at[:, cols], out_sems.at[b])

    def seg_rows(s):
        return pl.ds(pl.multiple_of(s * seg, seg), seg)

    def half_rows(i, n):
        return pl.ds(pl.multiple_of(i * (n // 2), n // 2), n // 2)

    def emit_output(s, y):
        ys[seg_rows(s), :] = y
        b = s // segs_per_blk
        rows = ys[pl.ds(pl.multiple_of(b * LANES, LANES), LANES), :]
        outT[b] = rows.T.astype(BF16)

    def new_ffn():
        return _Ffn(f_in[...], a_out[...], w1, w3, w2, n_chunks)

    def store_attention(rows, tokens):
        a_out[rows, :] = tokens
        f_in[rows, :] = _layernorm(tokens).astype(BF16)

    for c in copies[:DMA_DEPTH]:
        c.start()

    def arrive(i):
        if i + DMA_DEPTH < len(copies):
            copies[i + DMA_DEPTH].start()
        copies[i].wait()

    arrive(0)
    for b in range(n_blk):
        blk = xT[:, b * LANES:(b + 1) * LANES].astype(F32)
        xs[b * LANES:(b + 1) * LANES, :] = blk.T.astype(BF16)
    ys[...] = jnp.zeros(ys.shape, ys.dtype)

    pairs = n_heads // 2
    for m in range(3):
        arrive(1 + m)
        words = stage.at[m].bitcast(U32)

        def split_heads(i, carry, m=m, words=words):
            n = RELAYOUT_ROWS * pairs
            slab = words.at[pl.ds(pl.multiple_of(i * n, n), n)]
            for p in range(pairs):
                w = slab[pl.ds(p, RELAYOUT_ROWS, stride=pairs), :]
                even = lax.bitcast_convert_type(w << 16, F32)
                odd = lax.bitcast_convert_type(w & jnp.uint32(0xFFFF0000), F32)
                g, h = divmod(2 * p, HEADS_PER_GROUP)
                col = m * group_w + h * head_dim
                rows = half_rows(i, RELAYOUT_ROWS)
                wqkv[g, rows, col:col + head_dim] = _pack(even.astype(BF16))
                wqkv[g, rows, col + head_dim:col + 2 * head_dim] = _pack(odd.astype(BF16))
            return carry

        lax.fori_loop(0, d_model // RELAYOUT_ROWS, split_heads, 0)

    arrive(4)
    for c in copies[5 + DMA_DEPTH:]:
        c.start()

    def transpose_wo(h, carry):
        wo[half_rows(h, head_dim), :] = _pack(woT[h].astype(F32).T.astype(BF16))
        return carry

    lax.fori_loop(0, n_heads, transpose_wo, 0)

    mem0 = mem0_ref[...].astype(F32)
    mem[...] = jnp.concatenate([mem0, mem0], axis=0)

    def fill_step(s, carry):
        tokens, new_mem = attention(xs[seg_rows(s), :].astype(F32), mem[:n_mem, :], ffn=None)
        mem[:n_mem, :] = new_mem
        store_attention(seg_rows(s), tokens)
        return carry

    lax.fori_loop(0, 2, fill_step, 0)

    copies[5].wait()
    for j in range(w2T.shape[1] // LANES):
        blk = w2T[:, j * LANES:(j + 1) * LANES].astype(F32)
        w2[j * (LANES // 2):(j + 1) * (LANES // 2), :] = _pack(blk.T.astype(BF16))
    for i, (raw, packed) in enumerate([(w1_raw, w1), (w3_raw, w3)]):
        copies[6 + i].wait()

        def repack(r, carry, raw=raw, packed=packed):
            src = pl.ds(pl.multiple_of(r * RELAYOUT_ROWS, RELAYOUT_ROWS), RELAYOUT_ROWS)
            packed[half_rows(r, RELAYOUT_ROWS), :] = _pack(raw[src, :])
            return carry

        lax.fori_loop(0, d_model // RELAYOUT_ROWS, repack, 0)

    b_out[...] = new_ffn().finish()
    a_out[:seg, :] = a_out[seg:, :]
    f_in[:seg, :] = f_in[seg:, :]

    def step(t, carry):
        ffn = new_ffn()
        prev = b_out[...]
        emit_output(jnp.maximum(t - 4, 0), prev[seg:])
        resid = jnp.concatenate([xs[seg_rows(t), :].astype(F32), prev[:seg]], axis=0)
        tokens, new_mem = attention(resid, mem[...], ffn=ffn)
        mem[...] = new_mem
        store_attention(slice(None), tokens)
        b_out[...] = ffn.finish()

        @pl.when((t >= 4) & ((t - 4) % segs_per_blk == segs_per_blk - 1))
        def _():
            out_copy((t - 4) // segs_per_blk).start()

        return carry

    lax.fori_loop(2, n_seg, step, 0)

    ffn = new_ffn()
    prev = b_out[...]
    emit_output(n_seg - 4, prev[seg:])
    tokens, new_mem = attention(prev[:seg], mem[n_mem:, :], ffn=ffn)
    last = ffn.finish()
    store_attention(slice(0, seg), tokens)
    emit_output(n_seg - 3, last[seg:])
    tokens, _ = attention(last[:seg], new_mem, ffn=None)
    store_attention(slice(seg, 2 * seg), tokens)
    last = new_ffn().finish()
    ys[(n_seg - 2) * seg:(n_seg - 1) * seg, :] = last[:seg]
    emit_output(n_seg - 1, last[seg:])
    out_copy(n_blk - 1).start()
    for b in range(n_blk):
        out_copy(b).wait()


@functools.partial(jax.jit, static_argnames=("A_seg_len",))
def pallas_interleave_layers__memory_aug_recurrent_mem_tr__glu_gated_swiglu__prompt_kernel(
    A_x, A_mem0, A_Wq, A_Wk, A_Wv, A_Wo, A_seg_len, B_x, B_w1, B_w3, B_w2,
):
    del B_x
    batch, seq, d_model = A_x.shape
    _, n_heads, head_dim = A_Wq.shape
    n_mem = A_mem0.shape[1]
    d_ff = B_w1.shape[1]
    seg = int(A_seg_len)
    n_seg = seq // seg
    assert batch == 1 and n_seg * seg == seq and LANES == 4 * seg and seq % LANES == 0
    assert head_dim == LANES and n_heads % HEADS_PER_GROUP == 0 and d_ff % FFN_CHUNK == 0

    n_groups = n_heads // HEADS_PER_GROUP
    hbm = pl.BlockSpec(memory_space=pl.ANY)
    outT = pl.pallas_call(
        functools.partial(_kernel, seg=seg, n_seg=n_seg, n_heads=n_heads, head_dim=head_dim),
        out_shape=jax.ShapeDtypeStruct((d_model, seq), A_x.dtype),
        in_specs=[hbm, pl.BlockSpec(memory_space=pltpu.VMEM)] + [hbm] * 7,
        out_specs=hbm,
        scratch_shapes=[
            pltpu.VMEM((3, d_model * n_heads, head_dim), BF16),
            pltpu.VMEM((n_heads, d_model, head_dim), BF16),
            pltpu.VMEM((d_model, d_ff), BF16),
            pltpu.VMEM((d_model, d_ff), BF16),
            pltpu.VMEM((d_model, d_ff), BF16),
            pltpu.VMEM((n_groups, d_model // 2, 3 * HEADS_PER_GROUP * head_dim), U32),
            pltpu.VMEM((n_heads * head_dim // 2, d_model), U32),
            pltpu.VMEM((d_model // 2, d_ff), U32),
            pltpu.VMEM((d_model // 2, d_ff), U32),
            pltpu.VMEM((d_ff // 2, d_model), U32),
            pltpu.VMEM((d_model, seq), BF16),
            pltpu.VMEM((seq, d_model), BF16),
            pltpu.VMEM((seq, d_model), F32),
            pltpu.VMEM((seq // LANES, d_model, LANES), BF16),
            pltpu.VMEM((2 * n_mem, d_model), F32),
            pltpu.VMEM((2 * seg, d_model), F32),
            pltpu.VMEM((2 * seg, d_model), BF16),
            pltpu.VMEM((2 * seg, d_model), F32),
            pltpu.SemaphoreType.DMA((8,)),
            pltpu.SemaphoreType.DMA((seq // LANES,)),
        ],
        compiler_params=pltpu.CompilerParams(vmem_limit_bytes=110 * 2**20),
    )(
        A_x.reshape(seq, d_model).T,
        A_mem0.reshape(n_mem, d_model),
        A_Wq.reshape(d_model * n_heads, head_dim),
        A_Wk.reshape(d_model * n_heads, head_dim),
        A_Wv.reshape(d_model * n_heads, head_dim),
        A_Wo.transpose(0, 2, 1),
        B_w1,
        B_w3,
        B_w2.T,
    )
    return outT.T.reshape(batch, seq, d_model)
```

```python
import functools
import math

import jax
import jax.numpy as jnp
from jax import lax
import jax.experimental.pallas as pl
import jax.experimental.pallas.tpu as pltpu

F32 = jnp.float32
BF16 = jnp.bfloat16
U32 = jnp.uint32
LANES = 128
HEADS_PER_GROUP = 4
FFN_CHUNK = 512
RELAYOUT_ROWS = 64
DMA_DEPTH = 2
LOAD_SPLIT = 3
EARLY_CHUNKS = 3
FILL_START = 2
FILL_FIRST = 2
FILL_SOFTMAX = 2
FILL_PROJECT = (0, 1, 0, 0, 1, 0, 0)
FILL_LAST = 2
LN_EPS = 1e-5
MASK_VALUE = -1000000000.0
LOG2E = math.log2(math.e)
NT_DIMS = (((1,), (1,)), ((), ()))


def _pack(w):
    return pltpu.bitcast(w, U32)


def _unpack(w):
    return pltpu.bitcast(w, BF16)


def _layernorm(x):
    mean = jnp.mean(x, axis=-1, keepdims=True)
    cen = x - mean
    var = jnp.mean(cen * cen, axis=-1, keepdims=True)
    return cen * lax.rsqrt(var + LN_EPS)


def _attention_mask(n_layers, seg, n_mem):
    rows = n_layers * (seg + n_mem)
    n_tok = n_layers * seg

    def describe(axis):
        i = lax.broadcasted_iota(jnp.int32, (rows, rows), axis)
        is_mem = i >= n_tok
        layer = jnp.zeros_like(i)
        pos = jnp.where(is_mem, i - n_tok, i + n_mem)
        for l in range(1, n_layers):
            in_l = jnp.where(is_mem, i - n_tok - l * n_mem, i - l * seg) >= 0
            layer = jnp.where(in_l, l, layer)
        pos = pos - layer * jnp.where(is_mem, n_mem, seg)
        return layer, pos

    q_layer, q_pos = describe(0)
    k_layer, k_pos = describe(1)
    same = q_layer == k_layer
    visible = same & ((q_pos < n_mem) | (q_pos >= k_pos))
    fill = jnp.where(same, MASK_VALUE * LOG2E, -jnp.inf).astype(F32)
    return visible, fill


class _Ffn:
    def __init__(self, lhs, resid, w1, w3, w2, n_chunks, before_chunk=None):
        self.lhs, self.acc = lhs, resid
        self.w1, self.w3, self.w2 = w1, w3, w2
        self.before_chunk = before_chunk
        self.gate, self.hidden = {}, {}
        self.todo = []
        for c in range(n_chunks):
            self.todo += [(self._gate, c), (self._up, c)]
            if c > 0:
                self.todo.append((self._down, c - 1))
        self.todo.append((self._down, n_chunks - 1))

    def _project(self, w, c):
        cols = slice(c * FFN_CHUNK, (c + 1) * FFN_CHUNK)
        return jnp.dot(self.lhs, _unpack(w[:, cols]), preferred_element_type=F32)

    def _gate(self, c):
        if self.before_chunk is not None:
            self.before_chunk(c)
        gate = self._project(self.w1, c)
        self.gate[c] = gate * jax.nn.sigmoid(gate)

    def _up(self, c):
        self.hidden[c] = (self.gate.pop(c) * self._project(self.w3, c)).astype(BF16)

    def _down(self, c):
        rows = slice(c * FFN_CHUNK // 2, (c + 1) * FFN_CHUNK // 2)
        self.acc = self.acc + jnp.dot(self.hidden.pop(c), _unpack(self.w2[rows, :]),
                                      preferred_element_type=F32)

    def run(self, count):
        for fn, c in self.todo[:count]:
            fn(c)
        self.todo = self.todo[count:]

    def finish(self):
        self.run(len(self.todo))
        return self.acc


def _attention(resid, mem, wqkv, wo, ffn, *, seg, head_dim):
    n_groups = wqkv.shape[0]
    group_w = HEADS_PER_GROUP * head_dim
    n_tok = resid.shape[0]
    n_layers = n_tok // seg
    visible, fill = _attention_mask(n_layers, seg, mem.shape[0] // n_layers)
    score_scale = head_dim ** -0.5 * LOG2E
    lhs = jnp.concatenate([_layernorm(resid), mem], axis=0).astype(BF16)

    def project(g):
        return jnp.dot(lhs, _unpack(wqkv[g]), preferred_element_type=F32).astype(BF16)

    def head(qkv, m, i):
        return qkv[:, m * group_w + i * head_dim:m * group_w + (i + 1) * head_dim]

    def scores(qkv):
        probs = []
        for i in range(HEADS_PER_GROUP):
            s = lax.dot_general(head(qkv, 0, i), head(qkv, 1, i), NT_DIMS,
                                preferred_element_type=F32)
            s = jnp.where(visible, s * score_scale, fill)
            p = jnp.exp2(s - jnp.max(s, axis=-1, keepdims=True))
            probs.append((p.astype(BF16), 1.0 / jnp.sum(p, axis=-1, keepdims=True)))
        return probs

    def mix(qkv, probs):
        return jnp.concatenate(
            [(jnp.dot(p, head(qkv, 2, i), preferred_element_type=F32) * inv).astype(BF16)
             for i, (p, inv) in enumerate(probs)], axis=1)

    def output(g, o, acc):
        rows = slice(g * group_w // 2, (g + 1) * group_w // 2)
        part = jnp.dot(o, _unpack(wo[rows, :]), preferred_element_type=F32)
        return part if acc is None else acc + part

    acc = None
    if ffn is not None:
        ffn.run(FILL_START)
        qkv = project(0)
        ffn.run(FILL_FIRST)
        for g in range(n_groups):
            probs = scores(qkv)
            ffn.run(FILL_SOFTMAX)
            o = mix(qkv, probs)
            if g + 1 < n_groups:
                qkv = project(g + 1)
                ffn.run(FILL_PROJECT[g % len(FILL_PROJECT)])
            else:
                ffn.run(FILL_LAST)
            acc = output(g, o, acc)
    else:
        qkv, o = project(0), None
        nxt = project(1)
        for g in range(n_groups):
            probs = scores(qkv)
            if o is not None:
                acc = output(g - 1, o, acc)
            after = project(g + 2) if g + 2 < n_groups else None
            o = mix(qkv, probs)
            qkv, nxt = nxt, after
        acc = output(n_groups - 1, o, acc)
    return resid + acc[:n_tok], acc[n_tok:]


def _kernel(xT_hbm, mem0_ref, wq_hbm, wk_hbm, wv_hbm, woT_hbm, w1_hbm, w3_hbm, w2T_hbm,
            outT_hbm,
            stage, woT, w1_raw, w3_raw, w2T, wqkv, wo, w1, w3, w2, xT, xs, ys, outT,
            mem, a_out, f_in, b_out, in_sems, out_sems,
            *, seg, n_seg, n_heads, head_dim):
    d_model = xs.shape[1]
    n_mem = mem0_ref.shape[0]
    group_w = HEADS_PER_GROUP * head_dim
    n_chunks = w1_raw.shape[1] // FFN_CHUNK
    segs_per_blk = LANES // seg
    n_blk = n_seg // segs_per_blk
    attention = functools.partial(_attention, wqkv=wqkv, wo=wo, seg=seg, head_dim=head_dim)

    def out_copy(b):
        cols = pl.ds(pl.multiple_of(b * LANES, LANES), LANES)
        return pltpu.make_async_copy(outT.at[b], outT_hbm.at[:, cols], out_sems.at[b])

    def seg_rows(s):
        return pl.ds(pl.multiple_of(s * seg, seg), seg)

    def half_rows(i, n):
        return pl.ds(pl.multiple_of(i * (n // 2), n // 2), n // 2)

    def emit_output(s, y):
        ys[seg_rows(s), :] = y
        b = s // segs_per_blk
        rows = ys[pl.ds(pl.multiple_of(b * LANES, LANES), LANES), :]
        outT[b] = rows.T.astype(BF16)

    def new_ffn(before_chunk=None):
        return _Ffn(f_in[...], a_out[...], w1, w3, w2, n_chunks, before_chunk)

    def store_attention(rows, tokens):
        a_out[rows, :] = tokens
        f_in[rows, :] = _layernorm(tokens).astype(BF16)

    def load_x_block(b):
        start = b * LANES if isinstance(b, int) else pl.multiple_of(b * LANES, LANES)
        xs[pl.ds(start, LANES), :] = xT[b].astype(F32).T.astype(BF16)

    pairs = n_heads // 2
    d_rows = d_model // LOAD_SPLIT

    def x_load(b):
        return xT_hbm.at[:, b * LANES:(b + 1) * LANES], xT.at[b], lambda: None

    def qkv_load(m, src, part):
        rows = pl.ds(part * d_rows * n_heads, d_rows * n_heads)

        def split_heads(i, carry):
            n = RELAYOUT_ROWS * pairs
            slab = stage.at[m].bitcast(U32).at[pl.ds(pl.multiple_of(i * n, n), n)]
            for p in range(pairs):
                w = slab[pl.ds(p, RELAYOUT_ROWS, stride=pairs), :]
                even = lax.bitcast_convert_type(w << 16, F32)
                odd = lax.bitcast_convert_type(w & jnp.uint32(0xFFFF0000), F32)
                g, h = divmod(2 * p, HEADS_PER_GROUP)
                col = m * group_w + h * head_dim
                dst = half_rows(i, RELAYOUT_ROWS)
                wqkv[g, dst, col:col + head_dim] = _pack(even.astype(BF16))
                wqkv[g, dst, col + head_dim:col + 2 * head_dim] = _pack(odd.astype(BF16))
            return carry

        steps = d_rows // RELAYOUT_ROWS
        return (src.at[rows], stage.at[m, rows],
                lambda: lax.fori_loop(part * steps, (part + 1) * steps, split_heads, 0))

    def wo_load(g):
        def transpose():
            for h in range(g * HEADS_PER_GROUP, (g + 1) * HEADS_PER_GROUP):
                rows = slice(h * head_dim // 2, (h + 1) * head_dim // 2)
                wo[rows, :] = _pack(woT[h].astype(F32).T.astype(BF16))

        heads = pl.ds(g * HEADS_PER_GROUP, HEADS_PER_GROUP)
        return woT_hbm.at[heads], woT.at[heads], transpose

    def w2_load(c):
        def transpose():
            for j in range(c * FFN_CHUNK // LANES, (c + 1) * FFN_CHUNK // LANES):
                blk = w2T[:, j * LANES:(j + 1) * LANES].astype(F32)
                w2[j * (LANES // 2):(j + 1) * (LANES // 2), :] = _pack(blk.T.astype(BF16))

        cols = slice(c * FFN_CHUNK, (c + 1) * FFN_CHUNK)
        return w2T_hbm.at[:, cols], w2T.at[:, cols], transpose

    def w13_load(src, raw, packed, c):
        cols = slice(c * FFN_CHUNK, (c + 1) * FFN_CHUNK)

        def repack():
            packed[:, cols] = _pack(raw[:, cols])

        return src.at[:, cols], raw.at[:, cols], repack

    loads = [x_load(0)]
    loads += [qkv_load(m, src, part) for m, src in enumerate([wq_hbm, wk_hbm, wv_hbm])
              for part in range(LOAD_SPLIT)]
    loads += [wo_load(g) for g in range(n_heads // HEADS_PER_GROUP)]
    n_attention_loads = len(loads)
    for c in range(n_chunks):
        loads += [w13_load(w1_hbm, w1_raw, w1, c), w13_load(w3_hbm, w3_raw, w3, c), w2_load(c)]
    n_early_loads = n_attention_loads + 3 * EARLY_CHUNKS
    n_weight_loads = len(loads)
    loads += [x_load(b) for b in range(1, n_blk)]
    copies = [pltpu.make_async_copy(src, dst, in_sems.at[i])
              for i, (src, dst, _) in enumerate(loads)]

    def finish_loads(lo, hi):
        for i in range(lo, hi):
            copies[i].wait()
            loads[i][2]()

    for c in copies[:DMA_DEPTH]:
        c.start()
    ys[...] = jnp.zeros(ys.shape, ys.dtype)
    for i in range(n_attention_loads):
        copies[i].wait()
        if i + DMA_DEPTH < n_attention_loads:
            copies[i + DMA_DEPTH].start()
        elif i + DMA_DEPTH == n_attention_loads:
            for c in copies[n_attention_loads:n_early_loads]:
                c.start()
        loads[i][2]()
    load_x_block(0)

    mem0 = mem0_ref[...].astype(F32)
    mem[...] = jnp.concatenate([mem0, mem0], axis=0)

    def fill_step(s, carry):
        tokens, new_mem = attention(xs[seg_rows(s), :].astype(F32), mem[:n_mem, :], ffn=None)
        mem[:n_mem, :] = new_mem
        store_attention(seg_rows(s), tokens)

        @pl.when(s == 0)
        def _():
            for c in copies[n_early_loads:]:
                c.start()

        return carry

    lax.fori_loop(0, 2, fill_step, 0)

    def finish_chunk_loads(c):
        finish_loads(n_attention_loads + 3 * c, n_attention_loads + 3 * (c + 1))

    b_out[...] = new_ffn(finish_chunk_loads).finish()
    a_out[:seg, :] = a_out[seg:, :]
    f_in[:seg, :] = f_in[seg:, :]
    finish_loads(n_weight_loads, len(loads))

    def step(t):
        ffn = new_ffn()
        prev = b_out[...]
        emit_output(jnp.maximum(t - 4, 0), prev[seg:])
        resid = jnp.concatenate([xs[seg_rows(t), :].astype(F32), prev[:seg]], axis=0)
        tokens, new_mem = attention(resid, mem[...], ffn=ffn)
        mem[...] = new_mem
        store_attention(slice(None), tokens)
        load_x_block(jnp.minimum(t // segs_per_blk + 1, n_blk - 1))
        b_out[...] = ffn.finish()

    def loop_body(t, carry):
        step(t)
        done = t - 4

        @pl.when((done >= 0) & (done % segs_per_blk == segs_per_blk - 1))
        def _():
            out_copy(done // segs_per_blk).start()

        return carry

    lax.fori_loop(2, n_seg, loop_body, 0)

    ffn = new_ffn()
    prev = b_out[...]
    emit_output(n_seg - 4, prev[seg:])
    tokens, new_mem = attention(prev[:seg], mem[n_mem:, :], ffn=ffn)
    last = ffn.finish()
    store_attention(slice(0, seg), tokens)
    emit_output(n_seg - 3, last[seg:])
    tokens, _ = attention(last[:seg], new_mem, ffn=None)
    store_attention(slice(seg, 2 * seg), tokens)
    last = new_ffn().finish()
    ys[(n_seg - 2) * seg:(n_seg - 1) * seg, :] = last[:seg]
    emit_output(n_seg - 1, last[seg:])
    out_copy(n_blk - 1).start()
    for b in range(n_blk):
        out_copy(b).wait()


@functools.partial(jax.jit, static_argnames=("A_seg_len",))
def pallas_interleave_layers__memory_aug_recurrent_mem_tr__glu_gated_swiglu__prompt_kernel(
    A_x, A_mem0, A_Wq, A_Wk, A_Wv, A_Wo, A_seg_len, B_x, B_w1, B_w3, B_w2,
):
    del B_x
    batch, seq, d_model = A_x.shape
    _, n_heads, head_dim = A_Wq.shape
    n_mem = A_mem0.shape[1]
    d_ff = B_w1.shape[1]
    seg = int(A_seg_len)
    n_seg = seq // seg
    assert batch == 1 and n_seg * seg == seq and LANES == 4 * seg and seq % LANES == 0
    assert head_dim == LANES and n_heads % HEADS_PER_GROUP == 0 and d_ff % FFN_CHUNK == 0

    n_groups = n_heads // HEADS_PER_GROUP
    hbm = pl.BlockSpec(memory_space=pl.ANY)
    outT = pl.pallas_call(
        functools.partial(_kernel, seg=seg, n_seg=n_seg, n_heads=n_heads, head_dim=head_dim),
        out_shape=jax.ShapeDtypeStruct((d_model, seq), A_x.dtype),
        in_specs=[hbm, pl.BlockSpec(memory_space=pltpu.VMEM)] + [hbm] * 7,
        out_specs=hbm,
        scratch_shapes=[
            pltpu.VMEM((3, d_model * n_heads, head_dim), BF16),
            pltpu.VMEM((n_heads, d_model, head_dim), BF16),
            pltpu.VMEM((d_model, d_ff), BF16),
            pltpu.VMEM((d_model, d_ff), BF16),
            pltpu.VMEM((d_model, d_ff), BF16),
            pltpu.VMEM((n_groups, d_model // 2, 3 * HEADS_PER_GROUP * head_dim), U32),
            pltpu.VMEM((n_heads * head_dim // 2, d_model), U32),
            pltpu.VMEM((d_model // 2, d_ff), U32),
            pltpu.VMEM((d_model // 2, d_ff), U32),
            pltpu.VMEM((d_ff // 2, d_model), U32),
            pltpu.VMEM((seq // LANES, d_model, LANES), BF16),
            pltpu.VMEM((seq, d_model), BF16),
            pltpu.VMEM((seq, d_model), F32),
            pltpu.VMEM((seq // LANES, d_model, LANES), BF16),
            pltpu.VMEM((2 * n_mem, d_model), F32),
            pltpu.VMEM((2 * seg, d_model), F32),
            pltpu.VMEM((2 * seg, d_model), BF16),
            pltpu.VMEM((2 * seg, d_model), F32),
            pltpu.SemaphoreType.DMA((3 * LOAD_SPLIT + n_groups + 3 * (d_ff // FFN_CHUNK) + seq // LANES,)),
            pltpu.SemaphoreType.DMA((seq // LANES,)),
        ],
        compiler_params=pltpu.CompilerParams(vmem_limit_bytes=110 * 2**20),
    )(
        A_x.reshape(seq, d_model).T,
        A_mem0.reshape(n_mem, d_model),
        A_Wq.reshape(d_model * n_heads, head_dim),
        A_Wk.reshape(d_model * n_heads, head_dim),
        A_Wv.reshape(d_model * n_heads, head_dim),
        A_Wo.transpose(0, 2, 1),
        B_w1,
        B_w3,
        B_w2.T,
    )
    return outT.T.reshape(batch, seq, d_model)
```

```python
import functools
import math

import jax
import jax.numpy as jnp
from jax import lax
import jax.experimental.pallas as pl
import jax.experimental.pallas.tpu as pltpu

F32 = jnp.float32
BF16 = jnp.bfloat16
U32 = jnp.uint32
LANES = 128
HEADS_PER_GROUP = 4
HALF = 2 * LANES
FFN_CHUNK = 2 * HALF
RELAYOUT_ROWS = 64
DMA_DEPTH = 2
EARLY_CHUNKS = 3
FILL_START = 2
FILL_FIRST = 2
FILL_SOFTMAX = 2
FILL_PROJECT = (0, 1, 0, 0, 1, 0, 0)
FILL_LAST = 2
LN_EPS = 1e-5
MASK_VALUE = -1000000000.0
LOG2E = math.log2(math.e)
NT_DIMS = (((1,), (1,)), ((), ()))


def _pack(w):
    return pltpu.bitcast(w, U32)


def _unpack(w):
    return pltpu.bitcast(w, BF16)


def _layernorm(x):
    mean = jnp.mean(x, axis=-1, keepdims=True)
    cen = x - mean
    var = jnp.mean(cen * cen, axis=-1, keepdims=True)
    return cen * lax.rsqrt(var + LN_EPS)


def _dot(lhs, packed_rhs):
    return jnp.dot(lhs, _unpack(packed_rhs), preferred_element_type=F32)


def _strassen_rhs(b11, b12, b21, b22):
    return [b11 + b22, b11, b12 - b22, b21 - b11, b22, b11 + b12, b21 + b22]


def _pad_rows(x, rows):
    if x.shape[0] == rows:
        return x
    return jnp.concatenate([x, jnp.zeros((rows - x.shape[0], x.shape[1]), x.dtype)], axis=0)


def _strassen_lhs(left, right, top):
    a11, a12 = left[:top], right[:top]
    if left.shape[0] == top:
        ops = [a11, None, a11, None, a11 + a12, None, a12]
    else:
        a21, a22 = left[top:], right[top:]
        a22_tall = _pad_rows(a22, top)
        ops = [a11 + a22_tall, a21 + a22, a11, a22, a11 + a12,
               a21 - a11[:a21.shape[0]], a12 - a22_tall]
    return [None if op is None else op.astype(BF16) for op in ops]


def _strassen_combine(m):
    m1, m2, m3, m4, m5, m6, m7 = m
    if m2 is None:
        return m1 - m5 + m7, m3 + m5
    bottom = m2.shape[0]
    left = [m1 + _pad_rows(m4, m1.shape[0]) - m5 + m7, m2 + m4]
    right = [m3 + m5, m1[:bottom] - m2 + m3[:bottom] + m6]
    return jnp.concatenate(left, axis=0), jnp.concatenate(right, axis=0)


class _InProjection:
    def __init__(self, x, top, w_main, w_rest):
        self.ops = _strassen_lhs(x[:, :HALF], x[:, HALF:2 * HALF], top)
        self.rest = x[:, 2 * HALF:].astype(BF16)
        self.w_main, self.w_rest = w_main, w_rest

    def products(self, block, which):
        return [None if self.ops[j] is None else _dot(self.ops[j], self.w_main[block, j])
                for j in which]

    def combine(self, block, products):
        rest = _dot(self.rest, self.w_rest[block])
        left, right = _strassen_combine(products)
        width = left.shape[1]
        return left + rest[:, :width], right + rest[:, width:]


class _OutProjection:
    def __init__(self, top, w_main, w_rest):
        self.top, self.w_main, self.w_rest = top, w_main, w_rest
        self.acc = None

    def add(self, block, left, right):
        parts = [None if op is None else _dot(op, self.w_main[block, j])
                 for j, op in enumerate(_strassen_lhs(left, right, self.top))]
        both = jnp.concatenate([left, right], axis=1).astype(BF16)
        parts.append(_dot(both, self.w_rest[block]))
        if self.acc is None:
            self.acc = parts
        else:
            self.acc = [None if a is None else a + b for a, b in zip(self.acc, parts)]

    def result(self):
        return jnp.concatenate([*_strassen_combine(self.acc[:7]), self.acc[7]], axis=1)


class _Ffn:
    def __init__(self, normed, weights, before_chunk=None):
        in_main, in_rest, out_main, out_rest = weights
        top = normed.shape[0] // 2
        self.project = _InProjection(normed, top, in_main, in_rest)
        self.output = _OutProjection(top, out_main, out_rest)
        self.before_chunk = before_chunk
        self.partial, self.hidden = {}, {}
        n_chunks = in_main.shape[0]
        self.todo = []
        for c in range(n_chunks):
            self.todo += [(self._begin, c), (self._activate, c)]
            if c > 0:
                self.todo.append((self._down, c - 1))
        self.todo.append((self._down, n_chunks - 1))

    def _begin(self, c):
        if self.before_chunk is not None:
            self.before_chunk(c)
        self.partial[c] = self.project.products(c, range(4))

    def _activate(self, c):
        products = self.partial.pop(c) + self.project.products(c, range(4, 7))
        self.hidden[c] = [
            half[:, :HALF] * jax.nn.sigmoid(half[:, :HALF]) * half[:, HALF:]
            for half in self.project.combine(c, products)]

    def _down(self, c):
        self.output.add(c, *self.hidden.pop(c))

    def run(self, count):
        for fn, c in self.todo[:count]:
            fn(c)
        self.todo = self.todo[count:]

    def finish(self):
        self.run(len(self.todo))
        return self.output.result()


def _attention_mask(rows, seg, n_mem):
    def describe(axis):
        i = lax.broadcasted_iota(jnp.int32, (rows, rows), axis)
        second = i >= seg + n_mem
        pos = jnp.where(second, i - seg - n_mem, jnp.where(i < seg, i + n_mem, i - seg))
        return second.astype(jnp.int32), pos

    q_layer, q_pos = describe(0)
    k_layer, k_pos = describe(1)
    same = q_layer == k_layer
    visible = same & ((q_pos < n_mem) | (q_pos >= k_pos))
    fill = jnp.where(same, MASK_VALUE * LOG2E, -jnp.inf).astype(F32)
    return visible, fill


def _attention(resid, mem, ffn, *, weights, seg, head_dim):
    in_main, in_rest, out_main, out_rest = weights
    n_groups = in_main.shape[0]
    mem_rows = mem.shape[0]
    top = seg + mem_rows
    normed = _layernorm(resid)
    stacked = [normed[:seg], mem] + ([normed[seg:]] if resid.shape[0] > seg else [])
    stacked = jnp.concatenate(stacked, axis=0)
    visible, fill = _attention_mask(stacked.shape[0], seg, mem_rows * seg // resid.shape[0])
    score_scale = head_dim ** -0.5 * LOG2E
    projection = _InProjection(stacked, top, in_main, in_rest)
    output = _OutProjection(top, out_main, out_rest)

    def project(g):
        halves = projection.combine(g, projection.products(g, range(7)))
        return [half.astype(BF16) for half in halves]

    def head(qkv, m, i):
        col = m * HALF + (i % 2) * head_dim
        return qkv[i // 2][:, col:col + head_dim]

    def scores(qkv):
        probs = []
        for i in range(HEADS_PER_GROUP):
            s = lax.dot_general(head(qkv, 0, i), head(qkv, 1, i), NT_DIMS,
                                preferred_element_type=F32)
            s = jnp.where(visible, s * score_scale, fill)
            p = jnp.exp2(s - jnp.max(s, axis=-1, keepdims=True))
            probs.append((p.astype(BF16), 1.0 / jnp.sum(p, axis=-1, keepdims=True)))
        return probs

    def mix(qkv, probs):
        o = [jnp.dot(p, head(qkv, 2, i), preferred_element_type=F32) * inv
             for i, (p, inv) in enumerate(probs)]
        return jnp.concatenate(o[:2], axis=1), jnp.concatenate(o[2:], axis=1)

    if ffn is not None:
        ffn.run(FILL_START)
        qkv = project(0)
        ffn.run(FILL_FIRST)
        for g in range(n_groups):
            probs = scores(qkv)
            ffn.run(FILL_SOFTMAX)
            o = mix(qkv, probs)
            if g + 1 < n_groups:
                qkv = project(g + 1)
                ffn.run(FILL_PROJECT[g % len(FILL_PROJECT)])
            else:
                ffn.run(FILL_LAST)
            output.add(g, *o)
    else:
        qkv, o = project(0), None
        nxt = project(1)
        for g in range(n_groups):
            probs = scores(qkv)
            if o is not None:
                output.add(g - 1, *o)
            after = project(g + 2) if g + 2 < n_groups else None
            o = mix(qkv, probs)
            qkv, nxt = nxt, after
        output.add(n_groups - 1, *o)
    out = output.result()
    tokens = [out[:seg]] + ([out[top:]] if resid.shape[0] > seg else [])
    return resid + jnp.concatenate(tokens, axis=0), out[seg:top]


def _kernel(xT_hbm, mem0_ref, wq_hbm, wk_hbm, wv_hbm, woT_hbm, w1_hbm, w3_hbm, w2T_hbm,
            outT_hbm,
            stage, woT, w1_raw, w3_raw, w2T,
            qkv_main, qkv_rest, wo_main, wo_rest, w13_main, w13_rest, w2_main, w2_rest,
            xT, xs, ys, outT,
            mem, a_out, f_in, b_out, in_sems, out_sems,
            *, seg, n_seg, n_heads, head_dim):
    d_model = xs.shape[1]
    n_mem = mem0_ref.shape[0]
    n_chunks = w1_raw.shape[1] // FFN_CHUNK
    segs_per_blk = LANES // seg
    n_blk = n_seg // segs_per_blk
    attention = functools.partial(_attention, weights=(qkv_main, qkv_rest, wo_main, wo_rest),
                                  seg=seg, head_dim=head_dim)

    def out_copy(b):
        cols = pl.ds(pl.multiple_of(b * LANES, LANES), LANES)
        return pltpu.make_async_copy(outT.at[b], outT_hbm.at[:, cols], out_sems.at[b])

    def seg_rows(s):
        return pl.ds(pl.multiple_of(s * seg, seg), seg)

    def half_rows(i, n):
        return pl.ds(pl.multiple_of(i * (n // 2), n // 2), n // 2)

    def emit_output(s, y):
        ys[seg_rows(s), :] = y
        b = s // segs_per_blk
        rows = ys[pl.ds(pl.multiple_of(b * LANES, LANES), LANES), :]
        outT[b] = rows.T.astype(BF16)

    def new_ffn(before_chunk=None):
        return _Ffn(f_in[...], (w13_main, w13_rest, w2_main, w2_rest), before_chunk)

    def store_attention(rows, tokens):
        a_out[rows, :] = tokens
        f_in[rows, :] = _layernorm(tokens)

    def load_x_block(b):
        start = b * LANES if isinstance(b, int) else pl.multiple_of(b * LANES, LANES)
        xs[pl.ds(start, LANES), :] = xT[b].astype(F32).T.astype(BF16)

    pairs = n_heads // 2
    half_blocks = HALF // RELAYOUT_ROWS

    def x_load(b):
        return xT_hbm.at[:, b * LANES:(b + 1) * LANES], xT.at[b], lambda: None

    def qkv_load(m, src):
        def head_pair(block, p):
            n = RELAYOUT_ROWS * pairs
            start = block * n if isinstance(block, int) else pl.multiple_of(block * n, n)
            slab = stage.at[m].bitcast(U32).at[pl.ds(start, n)]
            w = slab[pl.ds(p, RELAYOUT_ROWS, stride=pairs), :]
            return (lax.bitcast_convert_type(w << 16, F32),
                    lax.bitcast_convert_type(w & jnp.uint32(0xFFFF0000), F32))

        def split(i, carry):
            for g in range(pairs // 2):
                quads = [head_pair(i + k * half_blocks, 2 * g + n)
                         for k in range(2) for n in range(2)]
                for h in range(2):
                    col = m * HALF + h * head_dim
                    for j, op in enumerate(_strassen_rhs(*(q[h] for q in quads))):
                        qkv_main[g, j, half_rows(i, RELAYOUT_ROWS), col:col + head_dim] = (
                            _pack(op.astype(BF16)))
            return carry

        def relayout():
            lax.fori_loop(0, half_blocks, split, 0)
            for p in range(pairs):
                for h, w in enumerate(head_pair(2 * half_blocks, p)):
                    col = ((p % 2) * 3 + m) * HALF + h * head_dim
                    qkv_rest[p // 2, :, col:col + head_dim] = _pack(w.astype(BF16))

        return src, stage.at[m], relayout

    def store_out_weights(main, rest, block, transposed):
        for i in range(2):
            upper, lower = transposed(i).astype(F32).T, transposed(2 + i).astype(F32).T
            ops = _strassen_rhs(upper[:, :HALF], upper[:, HALF:2 * HALF],
                                lower[:, :HALF], lower[:, HALF:2 * HALF])
            for j, op in enumerate(ops):
                main[block, j, i * LANES // 2:(i + 1) * LANES // 2, :] = _pack(op.astype(BF16))
            for k, w in ((i, upper), (2 + i, lower)):
                rest[block, k * LANES // 2:(k + 1) * LANES // 2, :] = (
                    _pack(w[:, 2 * HALF:].astype(BF16)))

    def wo_load(g):
        heads = pl.ds(g * HEADS_PER_GROUP, HEADS_PER_GROUP)
        return (woT_hbm.at[heads], woT.at[heads], lambda: store_out_weights(
            wo_main, wo_rest, g, lambda i: woT[g * HEADS_PER_GROUP + i]))

    def w2_load(c):
        def piece(i):
            return w2T[:, c * FFN_CHUNK + i * LANES:c * FFN_CHUNK + (i + 1) * LANES]

        cols = slice(c * FFN_CHUNK, (c + 1) * FFN_CHUNK)
        return (w2T_hbm.at[:, cols], w2T.at[:, cols],
                lambda: store_out_weights(w2_main, w2_rest, c, piece))

    def w13_load(i, src, raw, c):
        def relayout():
            for r in range(half_blocks):
                quads = [
                    raw[k * HALF + r * RELAYOUT_ROWS:k * HALF + (r + 1) * RELAYOUT_ROWS,
                        c * FFN_CHUNK + n * HALF:c * FFN_CHUNK + (n + 1) * HALF].astype(F32)
                    for k in range(2) for n in range(2)]
                rows = slice(r * RELAYOUT_ROWS // 2, (r + 1) * RELAYOUT_ROWS // 2)
                for j, op in enumerate(_strassen_rhs(*quads)):
                    w13_main[c, j, rows, i * HALF:(i + 1) * HALF] = _pack(op.astype(BF16))
            for n in range(2):
                w13_rest[c, :, (2 * n + i) * HALF:(2 * n + i + 1) * HALF] = _pack(
                    raw[2 * HALF:, c * FFN_CHUNK + n * HALF:c * FFN_CHUNK + (n + 1) * HALF])

        cols = slice(c * FFN_CHUNK, (c + 1) * FFN_CHUNK)
        return src.at[:, cols], raw.at[:, cols], relayout

    loads = [x_load(0)]
    loads += [qkv_load(m, src) for m, src in enumerate([wq_hbm, wk_hbm, wv_hbm])]
    loads += [wo_load(g) for g in range(n_heads // HEADS_PER_GROUP)]
    n_attention_loads = len(loads)
    for c in range(n_chunks):
        loads += [w13_load(0, w1_hbm, w1_raw, c), w13_load(1, w3_hbm, w3_raw, c), w2_load(c)]
    n_early_loads = n_attention_loads + 3 * EARLY_CHUNKS
    n_weight_loads = len(loads)
    loads += [x_load(b) for b in range(1, n_blk)]
    copies = [pltpu.make_async_copy(src, dst, in_sems.at[i])
              for i, (src, dst, _) in enumerate(loads)]

    def finish_loads(lo, hi):
        for i in range(lo, hi):
            copies[i].wait()
            loads[i][2]()

    for c in copies[:DMA_DEPTH]:
        c.start()
    ys[...] = jnp.zeros(ys.shape, ys.dtype)
    for i in range(n_attention_loads):
        copies[i].wait()
        if i + DMA_DEPTH < n_attention_loads:
            copies[i + DMA_DEPTH].start()
        elif i + DMA_DEPTH == n_attention_loads:
            for c in copies[n_attention_loads:n_early_loads]:
                c.start()
        loads[i][2]()
    load_x_block(0)

    mem0 = mem0_ref[...].astype(F32)
    mem[...] = jnp.concatenate([mem0, mem0], axis=0)

    def fill_step(s, carry):
        tokens, new_mem = attention(xs[seg_rows(s), :].astype(F32), mem[:n_mem, :], ffn=None)
        mem[:n_mem, :] = new_mem
        store_attention(seg_rows(s), tokens)

        @pl.when(s == 0)
        def _():
            for c in copies[n_early_loads:]:
                c.start()

        return carry

    lax.fori_loop(0, 2, fill_step, 0)

    def finish_chunk_loads(c):
        finish_loads(n_attention_loads + 3 * c, n_attention_loads + 3 * (c + 1))

    b_out[...] = a_out[...] + new_ffn(finish_chunk_loads).finish()
    a_out[:seg, :] = a_out[seg:, :]
    f_in[:seg, :] = f_in[seg:, :]
    finish_loads(n_weight_loads, len(loads))

    def step(t):
        ffn, ffn_resid = new_ffn(), a_out[...]
        prev = b_out[...]
        emit_output(jnp.maximum(t - 4, 0), prev[seg:])
        resid = jnp.concatenate([xs[seg_rows(t), :].astype(F32), prev[:seg]], axis=0)
        tokens, new_mem = attention(resid, mem[...], ffn=ffn)
        mem[...] = new_mem
        store_attention(slice(None), tokens)
        load_x_block(jnp.minimum(t // segs_per_blk + 1, n_blk - 1))
        b_out[...] = ffn_resid + ffn.finish()

    def loop_body(t, carry):
        step(t)
        done = t - 4

        @pl.when((done >= 0) & (done % segs_per_blk == segs_per_blk - 1))
        def _():
            out_copy(done // segs_per_blk).start()

        return carry

    lax.fori_loop(2, n_seg, loop_body, 0)

    ffn, ffn_resid = new_ffn(), a_out[...]
    prev = b_out[...]
    emit_output(n_seg - 4, prev[seg:])
    tokens, new_mem = attention(prev[:seg], mem[n_mem:, :], ffn=ffn)
    last = ffn_resid + ffn.finish()
    store_attention(slice(0, seg), tokens)
    emit_output(n_seg - 3, last[seg:])
    tokens, _ = attention(last[:seg], new_mem, ffn=None)
    store_attention(slice(seg, 2 * seg), tokens)
    last = a_out[...] + new_ffn().finish()
    ys[(n_seg - 2) * seg:(n_seg - 1) * seg, :] = last[:seg]
    emit_output(n_seg - 1, last[seg:])
    out_copy(n_blk - 1).start()
    for b in range(n_blk):
        out_copy(b).wait()


@functools.partial(jax.jit, static_argnames=("A_seg_len",))
def pallas_interleave_layers__memory_aug_recurrent_mem_tr__glu_gated_swiglu__prompt_kernel(
    A_x, A_mem0, A_Wq, A_Wk, A_Wv, A_Wo, A_seg_len, B_x, B_w1, B_w3, B_w2,
):
    del B_x
    batch, seq, d_model = A_x.shape
    _, n_heads, head_dim = A_Wq.shape
    n_mem = A_mem0.shape[1]
    d_ff = B_w1.shape[1]
    seg = int(A_seg_len)
    n_seg = seq // seg
    assert batch == 1 and n_seg * seg == seq and LANES == 4 * seg and seq % LANES == 0
    assert head_dim == LANES and n_heads % HEADS_PER_GROUP == 0 and d_ff % FFN_CHUNK == 0

    n_groups = n_heads // HEADS_PER_GROUP
    n_chunks = d_ff // FFN_CHUNK
    rest = d_model - 2 * HALF
    assert rest == RELAYOUT_ROWS
    hbm = pl.BlockSpec(memory_space=pl.ANY)
    outT = pl.pallas_call(
        functools.partial(_kernel, seg=seg, n_seg=n_seg, n_heads=n_heads, head_dim=head_dim),
        out_shape=jax.ShapeDtypeStruct((d_model, seq), A_x.dtype),
        in_specs=[hbm, pl.BlockSpec(memory_space=pltpu.VMEM)] + [hbm] * 7,
        out_specs=hbm,
        scratch_shapes=[
            pltpu.VMEM((3, d_model * n_heads, head_dim), BF16),
            pltpu.VMEM((n_heads, d_model, head_dim), BF16),
            pltpu.VMEM((d_model, d_ff), BF16),
            pltpu.VMEM((d_model, d_ff), BF16),
            pltpu.VMEM((d_model, d_ff), BF16),
            pltpu.VMEM((n_groups, 7, HALF // 2, 3 * HALF), U32),
            pltpu.VMEM((n_groups, rest // 2, 6 * HALF), U32),
            pltpu.VMEM((n_groups, 7, HALF // 2, HALF), U32),
            pltpu.VMEM((n_groups, HALF, rest), U32),
            pltpu.VMEM((n_chunks, 7, HALF // 2, 2 * HALF), U32),
            pltpu.VMEM((n_chunks, rest // 2, 4 * HALF), U32),
            pltpu.VMEM((n_chunks, 7, HALF // 2, HALF), U32),
            pltpu.VMEM((n_chunks, HALF, rest), U32),
            pltpu.VMEM((seq // LANES, d_model, LANES), BF16),
            pltpu.VMEM((seq, d_model), BF16),
            pltpu.VMEM((seq, d_model), F32),
            pltpu.VMEM((seq // LANES, d_model, LANES), BF16),
            pltpu.VMEM((2 * n_mem, d_model), F32),
            pltpu.VMEM((2 * seg, d_model), F32),
            pltpu.VMEM((2 * seg, d_model), F32),
            pltpu.VMEM((2 * seg, d_model), F32),
            pltpu.SemaphoreType.DMA((3 + n_groups + 3 * n_chunks + seq // LANES,)),
            pltpu.SemaphoreType.DMA((seq // LANES,)),
        ],
        compiler_params=pltpu.CompilerParams(vmem_limit_bytes=120 * 2**20),
    )(
        A_x.reshape(seq, d_model).T,
        A_mem0.reshape(n_mem, d_model),
        A_Wq.reshape(d_model * n_heads, head_dim),
        A_Wk.reshape(d_model * n_heads, head_dim),
        A_Wv.reshape(d_model * n_heads, head_dim),
        A_Wo.transpose(0, 2, 1),
        B_w1,
        B_w3,
        B_w2.T,
    )
    return outT.T.reshape(batch, seq, d_model)
```

```python
import functools
import math

import jax
import jax.numpy as jnp
from jax import lax
import jax.experimental.pallas as pl
import jax.experimental.pallas.tpu as pltpu

F32 = jnp.float32
BF16 = jnp.bfloat16
U32 = jnp.uint32
LANES = 128
HEADS_PER_GROUP = 4
HALF = 2 * LANES
FFN_CHUNK = 2 * HALF
RELAYOUT_ROWS = 64
DMA_DEPTH = 2
EARLY_CHUNKS = 3
FILL_START = 2
FILL_FIRST = 2
FILL_SOFTMAX = 2
FILL_PROJECT = (0, 1, 0, 0, 1, 0, 0)
FILL_LAST = 2
LN_EPS = 1e-5
MASK_VALUE = -1000000000.0
LOG2E = math.log2(math.e)
NT_DIMS = (((1,), (1,)), ((), ()))


def _pack(w):
    return pltpu.bitcast(w, U32)


def _unpack(w):
    return pltpu.bitcast(w, BF16)


def _layernorm(x):
    mean = jnp.mean(x, axis=-1, keepdims=True)
    cen = x - mean
    var = jnp.mean(cen * cen, axis=-1, keepdims=True)
    return cen * lax.rsqrt(var + LN_EPS)


def _dot(lhs, packed_rhs):
    return jnp.dot(lhs, _unpack(packed_rhs), preferred_element_type=F32)


def _strassen_rhs(b11, b12, b21, b22):
    return [b11 + b22, b11, b12 - b22, b21 - b11, b22, b11 + b12, b21 + b22]


def _pad_rows(x, rows):
    if x.shape[0] == rows:
        return x
    return jnp.concatenate([x, jnp.zeros((rows - x.shape[0], x.shape[1]), x.dtype)], axis=0)


def _strassen_lhs(left, right, top):
    a11, a12 = left[:top], right[:top]
    if left.shape[0] == top:
        ops = [a11, None, a11, None, a11 + a12, None, a12]
    else:
        a21, a22 = left[top:], right[top:]
        a22_tall = _pad_rows(a22, top)
        ops = [a11 + a22_tall, a21 + a22, a11, a22, a11 + a12,
               a21 - a11[:a21.shape[0]], a12 - a22_tall]
    return [None if op is None else op.astype(BF16) for op in ops]


def _strassen_combine(m):
    m1, m2, m3, m4, m5, m6, m7 = m
    if m2 is None:
        return m1 - m5 + m7, m3 + m5
    bottom = m2.shape[0]
    left = [m1 + _pad_rows(m4, m1.shape[0]) - m5 + m7, m2 + m4]
    right = [m3 + m5, m1[:bottom] - m2 + m3[:bottom] + m6]
    return jnp.concatenate(left, axis=0), jnp.concatenate(right, axis=0)


class _InProjection:
    def __init__(self, x, top, w_main, w_rest):
        self.ops = _strassen_lhs(x[:, :HALF], x[:, HALF:2 * HALF], top)
        self.rest = x[:, 2 * HALF:].astype(BF16)
        self.w_main, self.w_rest = w_main, w_rest

    def tile(self, block, n):
        cols = slice(n * LANES, (n + 1) * LANES)
        width = self.w_main.shape[-1]
        rest = [_dot(self.rest, self.w_rest[block, :, base + n * LANES:base + (n + 1) * LANES])
                for base in (0, width)]
        left, right = _strassen_combine(
            [None if op is None else _dot(op, self.w_main[block, j, :, cols])
             for j, op in enumerate(self.ops)])
        return left + rest[0], right + rest[1]


class _OutProjection:
    def __init__(self, top, w_main, w_rest):
        self.top, self.w_main, self.w_rest = top, w_main, w_rest
        self.acc = None

    def add(self, block, left, right):
        parts = [None if op is None else _dot(op, self.w_main[block, j])
                 for j, op in enumerate(_strassen_lhs(left, right, self.top))]
        both = jnp.concatenate([left, right], axis=1).astype(BF16)
        parts.append(_dot(both, self.w_rest[block]))
        if self.acc is None:
            self.acc = parts
        else:
            self.acc = [None if a is None else a + b for a, b in zip(self.acc, parts)]

    def result(self):
        return jnp.concatenate([*_strassen_combine(self.acc[:7]), self.acc[7]], axis=1)


class _Ffn:
    def __init__(self, normed, weights, before_chunk=None):
        in_main, in_rest, out_main, out_rest = weights
        top = normed.shape[0] // 2
        self.project = _InProjection(normed, top, in_main, in_rest)
        self.output = _OutProjection(top, out_main, out_rest)
        self.before_chunk = before_chunk
        self.partial, self.hidden = {}, {}
        n_chunks = in_main.shape[0]
        self.todo = []
        for c in range(n_chunks):
            self.todo += [(self._begin, c), (self._activate, c)]
            if c > 0:
                self.todo.append((self._down, c - 1))
        self.todo.append((self._down, n_chunks - 1))

    def _hidden_tile(self, c, n):
        gate = self.project.tile(c, n)
        up = self.project.tile(c, HALF // LANES + n)
        return [g * jax.nn.sigmoid(g) * u for g, u in zip(gate, up)]

    def _begin(self, c):
        if self.before_chunk is not None:
            self.before_chunk(c)
        self.partial[c] = self._hidden_tile(c, 0)

    def _activate(self, c):
        self.hidden[c] = [jnp.concatenate(pair, axis=1)
                          for pair in zip(self.partial.pop(c), self._hidden_tile(c, 1))]

    def _down(self, c):
        self.output.add(c, *self.hidden.pop(c))

    def run(self, count):
        for fn, c in self.todo[:count]:
            fn(c)
        self.todo = self.todo[count:]

    def finish(self):
        self.run(len(self.todo))
        return self.output.result()


def _attention_mask(rows, seg, n_mem):
    def describe(axis):
        i = lax.broadcasted_iota(jnp.int32, (rows, rows), axis)
        second = i >= seg + n_mem
        pos = jnp.where(second, i - seg - n_mem, jnp.where(i < seg, i + n_mem, i - seg))
        return second.astype(jnp.int32), pos

    q_layer, q_pos = describe(0)
    k_layer, k_pos = describe(1)
    same = q_layer == k_layer
    visible = same & ((q_pos < n_mem) | (q_pos >= k_pos))
    fill = jnp.where(same, MASK_VALUE * LOG2E, -jnp.inf).astype(F32)
    return visible, fill


def _attention(resid, mem, ffn, *, weights, seg, head_dim):
    in_main, in_rest, out_main, out_rest = weights
    n_groups = in_main.shape[0]
    mem_rows = mem.shape[0]
    top = seg + mem_rows
    normed = _layernorm(resid)
    stacked = [normed[:seg], mem] + ([normed[seg:]] if resid.shape[0] > seg else [])
    stacked = jnp.concatenate(stacked, axis=0)
    visible, fill = _attention_mask(stacked.shape[0], seg, mem_rows * seg // resid.shape[0])
    score_scale = head_dim ** -0.5 * LOG2E
    projection = _InProjection(stacked, top, in_main, in_rest)
    output = _OutProjection(top, out_main, out_rest)

    def project(g):
        return [[half.astype(BF16) for half in projection.tile(g, n)]
                for n in range(3 * HALF // LANES)]

    def head(qkv, m, i):
        return qkv[2 * m + i % 2][i // 2]

    def scores(qkv):
        probs = []
        for i in range(HEADS_PER_GROUP):
            s = lax.dot_general(head(qkv, 0, i), head(qkv, 1, i), NT_DIMS,
                                preferred_element_type=F32)
            s = jnp.where(visible, s * score_scale, fill)
            p = jnp.exp2(s - jnp.max(s, axis=-1, keepdims=True))
            probs.append((p.astype(BF16), 1.0 / jnp.sum(p, axis=-1, keepdims=True)))
        return probs

    def mix(qkv, probs):
        o = [jnp.dot(p, head(qkv, 2, i), preferred_element_type=F32) * inv
             for i, (p, inv) in enumerate(probs)]
        return jnp.concatenate(o[:2], axis=1), jnp.concatenate(o[2:], axis=1)

    if ffn is not None:
        ffn.run(FILL_START)
        qkv = project(0)
        ffn.run(FILL_FIRST)
        for g in range(n_groups):
            probs = scores(qkv)
            ffn.run(FILL_SOFTMAX)
            o = mix(qkv, probs)
            if g + 1 < n_groups:
                qkv = project(g + 1)
                ffn.run(FILL_PROJECT[g % len(FILL_PROJECT)])
            else:
                ffn.run(FILL_LAST)
            output.add(g, *o)
    else:
        qkv, o = project(0), None
        nxt = project(1)
        for g in range(n_groups):
            probs = scores(qkv)
            if o is not None:
                output.add(g - 1, *o)
            after = project(g + 2) if g + 2 < n_groups else None
            o = mix(qkv, probs)
            qkv, nxt = nxt, after
        output.add(n_groups - 1, *o)
    out = output.result()
    tokens = [out[:seg]] + ([out[top:]] if resid.shape[0] > seg else [])
    return resid + jnp.concatenate(tokens, axis=0), out[seg:top]


def _kernel(xT_hbm, mem0_ref, wq_hbm, wk_hbm, wv_hbm, woT_hbm, w1_hbm, w3_hbm, w2T_hbm,
            outT_hbm,
            stage, woT, w1_raw, w3_raw, w2T,
            qkv_main, qkv_rest, wo_main, wo_rest, w13_main, w13_rest, w2_main, w2_rest,
            xT, xs, ys, outT,
            mem, a_out, f_in, b_out, in_sems, out_sems,
            *, seg, n_seg, n_heads, head_dim):
    d_model = xs.shape[1]
    n_mem = mem0_ref.shape[0]
    n_chunks = w1_raw.shape[1] // FFN_CHUNK
    segs_per_blk = LANES // seg
    n_blk = n_seg // segs_per_blk
    attention = functools.partial(_attention, weights=(qkv_main, qkv_rest, wo_main, wo_rest),
                                  seg=seg, head_dim=head_dim)

    def out_copy(b):
        cols = pl.ds(pl.multiple_of(b * LANES, LANES), LANES)
        return pltpu.make_async_copy(outT.at[b], outT_hbm.at[:, cols], out_sems.at[b])

    def seg_rows(s):
        return pl.ds(pl.multiple_of(s * seg, seg), seg)

    def half_rows(i, n):
        return pl.ds(pl.multiple_of(i * (n // 2), n // 2), n // 2)

    def emit_output(s, y):
        ys[seg_rows(s), :] = y
        b = s // segs_per_blk
        rows = ys[pl.ds(pl.multiple_of(b * LANES, LANES), LANES), :]
        outT[b] = rows.T.astype(BF16)

    def new_ffn(before_chunk=None):
        return _Ffn(f_in[...], (w13_main, w13_rest, w2_main, w2_rest), before_chunk)

    def store_attention(rows, tokens):
        a_out[rows, :] = tokens
        f_in[rows, :] = _layernorm(tokens)

    def load_x_block(b):
        start = b * LANES if isinstance(b, int) else pl.multiple_of(b * LANES, LANES)
        xs[pl.ds(start, LANES), :] = xT[b].astype(F32).T.astype(BF16)

    pairs = n_heads // 2
    half_blocks = HALF // RELAYOUT_ROWS

    def x_load(b):
        return xT_hbm.at[:, b * LANES:(b + 1) * LANES], xT.at[b], lambda: None

    def qkv_load(m, src):
        def head_pair(block, p):
            n = RELAYOUT_ROWS * pairs
            start = block * n if isinstance(block, int) else pl.multiple_of(block * n, n)
            slab = stage.at[m].bitcast(U32).at[pl.ds(start, n)]
            w = slab[pl.ds(p, RELAYOUT_ROWS, stride=pairs), :]
            return (lax.bitcast_convert_type(w << 16, F32),
                    lax.bitcast_convert_type(w & jnp.uint32(0xFFFF0000), F32))

        def split(i, carry):
            for g in range(pairs // 2):
                quads = [head_pair(i + k * half_blocks, 2 * g + n)
                         for k in range(2) for n in range(2)]
                for h in range(2):
                    col = m * HALF + h * head_dim
                    for j, op in enumerate(_strassen_rhs(*(q[h] for q in quads))):
                        qkv_main[g, j, half_rows(i, RELAYOUT_ROWS), col:col + head_dim] = (
                            _pack(op.astype(BF16)))
            return carry

        def relayout():
            lax.fori_loop(0, half_blocks, split, 0)
            for p in range(pairs):
                for h, w in enumerate(head_pair(2 * half_blocks, p)):
                    col = ((p % 2) * 3 + m) * HALF + h * head_dim
                    qkv_rest[p // 2, :, col:col + head_dim] = _pack(w.astype(BF16))

        return src, stage.at[m], relayout

    def store_out_weights(main, rest, block, transposed):
        for i in range(2):
            upper, lower = transposed(i).astype(F32).T, transposed(2 + i).astype(F32).T
            ops = _strassen_rhs(upper[:, :HALF], upper[:, HALF:2 * HALF],
                                lower[:, :HALF], lower[:, HALF:2 * HALF])
            for j, op in enumerate(ops):
                main[block, j, i * LANES // 2:(i + 1) * LANES // 2, :] = _pack(op.astype(BF16))
            for k, w in ((i, upper), (2 + i, lower)):
                rest[block, k * LANES // 2:(k + 1) * LANES // 2, :] = (
                    _pack(w[:, 2 * HALF:].astype(BF16)))

    def wo_load(g):
        heads = pl.ds(g * HEADS_PER_GROUP, HEADS_PER_GROUP)
        return (woT_hbm.at[heads], woT.at[heads], lambda: store_out_weights(
            wo_main, wo_rest, g, lambda i: woT[g * HEADS_PER_GROUP + i]))

    def w2_load(c):
        def piece(i):
            return w2T[:, c * FFN_CHUNK + i * LANES:c * FFN_CHUNK + (i + 1) * LANES]

        cols = slice(c * FFN_CHUNK, (c + 1) * FFN_CHUNK)
        return (w2T_hbm.at[:, cols], w2T.at[:, cols],
                lambda: store_out_weights(w2_main, w2_rest, c, piece))

    def w13_load(i, src, raw, c):
        def relayout():
            for r in range(half_blocks):
                quads = [
                    raw[k * HALF + r * RELAYOUT_ROWS:k * HALF + (r + 1) * RELAYOUT_ROWS,
                        c * FFN_CHUNK + n * HALF:c * FFN_CHUNK + (n + 1) * HALF].astype(F32)
                    for k in range(2) for n in range(2)]
                rows = slice(r * RELAYOUT_ROWS // 2, (r + 1) * RELAYOUT_ROWS // 2)
                for j, op in enumerate(_strassen_rhs(*quads)):
                    w13_main[c, j, rows, i * HALF:(i + 1) * HALF] = _pack(op.astype(BF16))
            for n in range(2):
                w13_rest[c, :, (2 * n + i) * HALF:(2 * n + i + 1) * HALF] = _pack(
                    raw[2 * HALF:, c * FFN_CHUNK + n * HALF:c * FFN_CHUNK + (n + 1) * HALF])

        cols = slice(c * FFN_CHUNK, (c + 1) * FFN_CHUNK)
        return src.at[:, cols], raw.at[:, cols], relayout

    loads = [x_load(0)]
    loads += [qkv_load(m, src) for m, src in enumerate([wq_hbm, wk_hbm, wv_hbm])]
    loads += [wo_load(g) for g in range(n_heads // HEADS_PER_GROUP)]
    n_attention_loads = len(loads)
    for c in range(n_chunks):
        loads += [w13_load(0, w1_hbm, w1_raw, c), w13_load(1, w3_hbm, w3_raw, c), w2_load(c)]
    n_early_loads = n_attention_loads + 3 * EARLY_CHUNKS
    n_weight_loads = len(loads)
    loads += [x_load(b) for b in range(1, n_blk)]
    copies = [pltpu.make_async_copy(src, dst, in_sems.at[i])
              for i, (src, dst, _) in enumerate(loads)]

    def finish_loads(lo, hi):
        for i in range(lo, hi):
            copies[i].wait()
            loads[i][2]()

    for c in copies[:DMA_DEPTH]:
        c.start()
    ys[...] = jnp.zeros(ys.shape, ys.dtype)
    for i in range(n_attention_loads):
        copies[i].wait()
        if i + DMA_DEPTH < n_attention_loads:
            copies[i + DMA_DEPTH].start()
        elif i + DMA_DEPTH == n_attention_loads:
            for c in copies[n_attention_loads:n_early_loads]:
                c.start()
        loads[i][2]()
    load_x_block(0)

    mem0 = mem0_ref[...].astype(F32)
    mem[...] = jnp.concatenate([mem0, mem0], axis=0)

    def fill_step(s, carry):
        tokens, new_mem = attention(xs[seg_rows(s), :].astype(F32), mem[:n_mem, :], ffn=None)
        mem[:n_mem, :] = new_mem
        store_attention(seg_rows(s), tokens)

        @pl.when(s == 0)
        def _():
            for c in copies[n_early_loads:]:
                c.start()

        return carry

    lax.fori_loop(0, 2, fill_step, 0)

    def finish_chunk_loads(c):
        finish_loads(n_attention_loads + 3 * c, n_attention_loads + 3 * (c + 1))

    b_out[...] = a_out[...] + new_ffn(finish_chunk_loads).finish()
    a_out[:seg, :] = a_out[seg:, :]
    f_in[:seg, :] = f_in[seg:, :]
    finish_loads(n_weight_loads, len(loads))

    def step(t):
        ffn, ffn_resid = new_ffn(), a_out[...]
        prev = b_out[...]
        emit_output(jnp.maximum(t - 4, 0), prev[seg:])
        resid = jnp.concatenate([xs[seg_rows(t), :].astype(F32), prev[:seg]], axis=0)
        tokens, new_mem = attention(resid, mem[...], ffn=ffn)
        mem[...] = new_mem
        store_attention(slice(None), tokens)
        load_x_block(jnp.minimum(t // segs_per_blk + 1, n_blk - 1))
        b_out[...] = ffn_resid + ffn.finish()

    def loop_body(t, carry):
        step(t)
        done = t - 4

        @pl.when((done >= 0) & (done % segs_per_blk == segs_per_blk - 1))
        def _():
            out_copy(done // segs_per_blk).start()

        return carry

    lax.fori_loop(2, n_seg, loop_body, 0)

    ffn, ffn_resid = new_ffn(), a_out[...]
    prev = b_out[...]
    emit_output(n_seg - 4, prev[seg:])
    tokens, new_mem = attention(prev[:seg], mem[n_mem:, :], ffn=ffn)
    last = ffn_resid + ffn.finish()
    store_attention(slice(0, seg), tokens)
    emit_output(n_seg - 3, last[seg:])
    tokens, _ = attention(last[:seg], new_mem, ffn=None)
    store_attention(slice(seg, 2 * seg), tokens)
    last = a_out[...] + new_ffn().finish()
    ys[(n_seg - 2) * seg:(n_seg - 1) * seg, :] = last[:seg]
    emit_output(n_seg - 1, last[seg:])
    out_copy(n_blk - 1).start()
    for b in range(n_blk):
        out_copy(b).wait()


@functools.partial(jax.jit, static_argnames=("A_seg_len",))
def pallas_interleave_layers__memory_aug_recurrent_mem_tr__glu_gated_swiglu__prompt_kernel(
    A_x, A_mem0, A_Wq, A_Wk, A_Wv, A_Wo, A_seg_len, B_x, B_w1, B_w3, B_w2,
):
    del B_x
    batch, seq, d_model = A_x.shape
    _, n_heads, head_dim = A_Wq.shape
    n_mem = A_mem0.shape[1]
    d_ff = B_w1.shape[1]
    seg = int(A_seg_len)
    n_seg = seq // seg
    assert batch == 1 and n_seg * seg == seq and LANES == 4 * seg and seq % LANES == 0
    assert head_dim == LANES and n_heads % HEADS_PER_GROUP == 0 and d_ff % FFN_CHUNK == 0

    n_groups = n_heads // HEADS_PER_GROUP
    n_chunks = d_ff // FFN_CHUNK
    rest = d_model - 2 * HALF
    assert rest == RELAYOUT_ROWS
    hbm = pl.BlockSpec(memory_space=pl.ANY)
    outT = pl.pallas_call(
        functools.partial(_kernel, seg=seg, n_seg=n_seg, n_heads=n_heads, head_dim=head_dim),
        out_shape=jax.ShapeDtypeStruct((d_model, seq), A_x.dtype),
        in_specs=[hbm, pl.BlockSpec(memory_space=pltpu.VMEM)] + [hbm] * 7,
        out_specs=hbm,
        scratch_shapes=[
            pltpu.VMEM((3, d_model * n_heads, head_dim), BF16),
            pltpu.VMEM((n_heads, d_model, head_dim), BF16),
            pltpu.VMEM((d_model, d_ff), BF16),
            pltpu.VMEM((d_model, d_ff), BF16),
            pltpu.VMEM((d_model, d_ff), BF16),
            pltpu.VMEM((n_groups, 7, HALF // 2, 3 * HALF), U32),
            pltpu.VMEM((n_groups, rest // 2, 6 * HALF), U32),
            pltpu.VMEM((n_groups, 7, HALF // 2, HALF), U32),
            pltpu.VMEM((n_groups, HALF, rest), U32),
            pltpu.VMEM((n_chunks, 7, HALF // 2, 2 * HALF), U32),
            pltpu.VMEM((n_chunks, rest // 2, 4 * HALF), U32),
            pltpu.VMEM((n_chunks, 7, HALF // 2, HALF), U32),
            pltpu.VMEM((n_chunks, HALF, rest), U32),
            pltpu.VMEM((seq // LANES, d_model, LANES), BF16),
            pltpu.VMEM((seq, d_model), BF16),
            pltpu.VMEM((seq, d_model), F32),
            pltpu.VMEM((seq // LANES, d_model, LANES), BF16),
            pltpu.VMEM((2 * n_mem, d_model), F32),
            pltpu.VMEM((2 * seg, d_model), F32),
            pltpu.VMEM((2 * seg, d_model), F32),
            pltpu.VMEM((2 * seg, d_model), F32),
            pltpu.SemaphoreType.DMA((3 + n_groups + 3 * n_chunks + seq // LANES,)),
            pltpu.SemaphoreType.DMA((seq // LANES,)),
        ],
        compiler_params=pltpu.CompilerParams(vmem_limit_bytes=120 * 2**20),
    )(
        A_x.reshape(seq, d_model).T,
        A_mem0.reshape(n_mem, d_model),
        A_Wq.reshape(d_model * n_heads, head_dim),
        A_Wk.reshape(d_model * n_heads, head_dim),
        A_Wv.reshape(d_model * n_heads, head_dim),
        A_Wo.transpose(0, 2, 1),
        B_w1,
        B_w3,
        B_w2.T,
    )
    return outT.T.reshape(batch, seq, d_model)
```

```python
import functools
import math

import jax
import jax.numpy as jnp
from jax import lax
import jax.experimental.pallas as pl
import jax.experimental.pallas.tpu as pltpu

F32 = jnp.float32
BF16 = jnp.bfloat16
U32 = jnp.uint32
LANES = 128
HEADS_PER_GROUP = 4
HALF = 2 * LANES
FFN_CHUNK = 2 * HALF
RELAYOUT_ROWS = 64
LOADS_AHEAD = 4
FILL_CHUNKS = ((0, 0, 0, 1, 1, 1, 2, 2), (2, 3, 3, 3, 4, 4, 5, 5))
CHUNKS_AHEAD = 3
FILL_START = 2
FILL_FIRST = 2
FILL_SOFTMAX = 2
FILL_PROJECT = (0, 1, 0, 0, 1, 0, 0)
FILL_LAST = 2
LN_EPS = 1e-5
MASK_VALUE = -1000000000.0
LOG2E = math.log2(math.e)
NT_DIMS = (((1,), (1,)), ((), ()))


def _pack(even_rows, odd_rows):
    return pltpu.pack_elementwise([even_rows, odd_rows], packed_dtype=BF16).astype(U32)


def _split_words(words):
    return (lax.bitcast_convert_type(words << 16, F32),
            lax.bitcast_convert_type(words & jnp.uint32(0xFFFF0000), F32))


def _layernorm(x):
    mean = jnp.mean(x, axis=-1, keepdims=True)
    cen = x - mean
    var = jnp.mean(cen * cen, axis=-1, keepdims=True)
    return cen * lax.rsqrt(var + LN_EPS)


def _dot(lhs, packed_rhs):
    return jnp.dot(lhs, pltpu.bitcast(packed_rhs, BF16), preferred_element_type=F32)


def _strassen_rhs(quads):
    def operands(b11, b12, b21, b22):
        return [b11 + b22, b11, b12 - b22, b21 - b11, b22, b11 + b12, b21 + b22]

    return [_pack(even, odd) for even, odd in
            zip(operands(*(q[0] for q in quads)), operands(*(q[1] for q in quads)))]


def _pad_rows(x, rows):
    if x.shape[0] == rows:
        return x
    return jnp.concatenate([x, jnp.zeros((rows - x.shape[0], x.shape[1]), x.dtype)], axis=0)


def _strassen_lhs(left, right, top):
    a11, a12 = left[:top], right[:top]
    if left.shape[0] == top:
        ops = [a11, None, a11, None, a11 + a12, None, a12]
    else:
        a21, a22 = left[top:], right[top:]
        a22_tall = _pad_rows(a22, top)
        ops = [a11 + a22_tall, a21 + a22, a11, a22, a11 + a12,
               a21 - a11[:a21.shape[0]], a12 - a22_tall]
    return [None if op is None else op.astype(BF16) for op in ops]


def _strassen_combine(m):
    m1, m2, m3, m4, m5, m6, m7 = m
    if m2 is None:
        return m1 - m5 + m7, m3 + m5
    bottom = m2.shape[0]
    left = [m1 + _pad_rows(m4, m1.shape[0]) - m5 + m7, m2 + m4]
    right = [m3 + m5, m1[:bottom] - m2 + m3[:bottom] + m6]
    return jnp.concatenate(left, axis=0), jnp.concatenate(right, axis=0)


class _InProjection:
    def __init__(self, x, top, w_main, w_rest):
        self.ops = _strassen_lhs(x[:, :HALF], x[:, HALF:2 * HALF], top)
        self.rest = x[:, 2 * HALF:].astype(BF16)
        self.w_main, self.w_rest = w_main, w_rest

    def tile(self, block, n):
        cols = slice(n * LANES, (n + 1) * LANES)
        width = self.w_main.shape[-1]
        rest = [_dot(self.rest, self.w_rest[block, :, base + n * LANES:base + (n + 1) * LANES])
                for base in (0, width)]
        left, right = _strassen_combine(
            [None if op is None else _dot(op, self.w_main[block, j, :, cols])
             for j, op in enumerate(self.ops)])
        return left + rest[0], right + rest[1]


class _OutProjection:
    def __init__(self, top, w_main, w_rest):
        self.top, self.w_main, self.w_rest = top, w_main, w_rest
        self.acc = None

    def add(self, block, left, right):
        parts = [None if op is None else _dot(op, self.w_main[block, j])
                 for j, op in enumerate(_strassen_lhs(left, right, self.top))]
        both = jnp.concatenate([left, right], axis=1).astype(BF16)
        parts.append(_dot(both, self.w_rest[block]))
        if self.acc is None:
            self.acc = parts
        else:
            self.acc = [None if a is None else a + b for a, b in zip(self.acc, parts)]

    def result(self):
        return jnp.concatenate([*_strassen_combine(self.acc[:7]), self.acc[7]], axis=1)


class _Ffn:
    def __init__(self, normed, weights, before_chunk=None):
        in_main, in_rest, out_main, out_rest = weights
        top = normed.shape[0] // 2
        self.project = _InProjection(normed, top, in_main, in_rest)
        self.output = _OutProjection(top, out_main, out_rest)
        self.before_chunk = before_chunk
        self.partial, self.hidden = {}, {}
        n_chunks = in_main.shape[0]
        self.todo = []
        for c in range(n_chunks):
            self.todo += [(self._begin, c), (self._activate, c)]
            if c > 0:
                self.todo.append((self._down, c - 1))
        self.todo.append((self._down, n_chunks - 1))

    def _hidden_tile(self, c, n):
        gate = self.project.tile(c, n)
        up = self.project.tile(c, HALF // LANES + n)
        return [g * jax.nn.sigmoid(g) * u for g, u in zip(gate, up)]

    def _begin(self, c):
        if self.before_chunk is not None:
            self.before_chunk(c)
        self.partial[c] = self._hidden_tile(c, 0)

    def _activate(self, c):
        self.hidden[c] = [jnp.concatenate(pair, axis=1)
                          for pair in zip(self.partial.pop(c), self._hidden_tile(c, 1))]

    def _down(self, c):
        self.output.add(c, *self.hidden.pop(c))

    def run(self, count):
        for fn, c in self.todo[:count]:
            fn(c)
        self.todo = self.todo[count:]

    def finish(self):
        self.run(len(self.todo))
        return self.output.result()


def _attention_mask(rows, seg, n_mem):
    def describe(axis):
        i = lax.broadcasted_iota(jnp.int32, (rows, rows), axis)
        second = i >= seg + n_mem
        pos = jnp.where(second, i - seg - n_mem, jnp.where(i < seg, i + n_mem, i - seg))
        return second.astype(jnp.int32), pos

    q_layer, q_pos = describe(0)
    k_layer, k_pos = describe(1)
    same = q_layer == k_layer
    visible = same & ((q_pos < n_mem) | (q_pos >= k_pos))
    fill = jnp.where(same, MASK_VALUE * LOG2E, -jnp.inf).astype(F32)
    return visible, fill


def _attention(resid, mem, ffn, before_group=None, *, weights, seg, head_dim):
    in_main, in_rest, out_main, out_rest = weights
    n_groups = in_main.shape[0]
    mem_rows = mem.shape[0]
    top = seg + mem_rows
    normed = _layernorm(resid)
    stacked = [normed[:seg], mem] + ([normed[seg:]] if resid.shape[0] > seg else [])
    stacked = jnp.concatenate(stacked, axis=0)
    visible, fill = _attention_mask(stacked.shape[0], seg, mem_rows * seg // resid.shape[0])
    score_scale = head_dim ** -0.5 * LOG2E
    projection = _InProjection(stacked, top, in_main, in_rest)
    output = _OutProjection(top, out_main, out_rest)

    def project(g):
        return [[half.astype(BF16) for half in projection.tile(g, n)]
                for n in range(3 * HALF // LANES)]

    def head(qkv, m, i):
        return qkv[2 * m + i % 2][i // 2]

    def scores(qkv):
        probs = []
        for i in range(HEADS_PER_GROUP):
            s = lax.dot_general(head(qkv, 0, i), head(qkv, 1, i), NT_DIMS,
                                preferred_element_type=F32)
            s = jnp.where(visible, s * score_scale, fill)
            p = jnp.exp2(s - jnp.max(s, axis=-1, keepdims=True))
            probs.append((p.astype(BF16), 1.0 / jnp.sum(p, axis=-1, keepdims=True)))
        return probs

    def mix(qkv, probs):
        o = [jnp.dot(p, head(qkv, 2, i), preferred_element_type=F32) * inv
             for i, (p, inv) in enumerate(probs)]
        return jnp.concatenate(o[:2], axis=1), jnp.concatenate(o[2:], axis=1)

    if ffn is not None:
        ffn.run(FILL_START)
        qkv = project(0)
        ffn.run(FILL_FIRST)
        for g in range(n_groups):
            probs = scores(qkv)
            ffn.run(FILL_SOFTMAX)
            o = mix(qkv, probs)
            if g + 1 < n_groups:
                qkv = project(g + 1)
                ffn.run(FILL_PROJECT[g % len(FILL_PROJECT)])
            else:
                ffn.run(FILL_LAST)
            output.add(g, *o)
    else:
        qkv, o = project(0), None
        nxt = project(1)
        for g in range(n_groups):
            if before_group is not None:
                before_group(g)
            probs = scores(qkv)
            if o is not None:
                output.add(g - 1, *o)
            after = project(g + 2) if g + 2 < n_groups else None
            o = mix(qkv, probs)
            qkv, nxt = nxt, after
        output.add(n_groups - 1, *o)
    out = output.result()
    tokens = [out[:seg]] + ([out[top:]] if resid.shape[0] > seg else [])
    return resid + jnp.concatenate(tokens, axis=0), out[seg:top]


def _kernel(xT_hbm, mem0_ref, wq_hbm, wk_hbm, wv_hbm, woT_hbm, w1_hbm, w3_hbm, w2T_hbm,
            outT_hbm,
            stage, woT, w1_raw, w3_raw, w2T, flipped,
            qkv_main, qkv_rest, wo_main, wo_rest, w13_main, w13_rest, w2_main, w2_rest,
            xT, xs, ys, outT,
            mem, a_out, f_in, b_out, in_sems, out_sems,
            *, seg, n_seg, n_heads, head_dim):
    d_model = xs.shape[1]
    n_mem = mem0_ref.shape[0]
    n_chunks = w1_raw.shape[1] // FFN_CHUNK
    segs_per_blk = LANES // seg
    n_blk = n_seg // segs_per_blk
    attention = functools.partial(_attention, weights=(qkv_main, qkv_rest, wo_main, wo_rest),
                                  seg=seg, head_dim=head_dim)

    def out_copy(b):
        cols = pl.ds(pl.multiple_of(b * LANES, LANES), LANES)
        return pltpu.make_async_copy(outT.at[b], outT_hbm.at[:, cols], out_sems.at[b])

    def seg_rows(s):
        return pl.ds(pl.multiple_of(s * seg, seg), seg)

    def emit_output(s, y):
        ys[seg_rows(s), :] = y
        b = s // segs_per_blk
        rows = ys[pl.ds(pl.multiple_of(b * LANES, LANES), LANES), :]
        outT[b] = rows.T.astype(BF16)

    def new_ffn(before_chunk=None):
        return _Ffn(f_in[...], (w13_main, w13_rest, w2_main, w2_rest), before_chunk)

    def store_attention(rows, tokens):
        a_out[rows, :] = tokens
        f_in[rows, :] = _layernorm(tokens)

    def load_x_block(b):
        start = b * LANES if isinstance(b, int) else pl.multiple_of(b * LANES, LANES)
        xs[pl.ds(start, LANES), :] = xT[b].astype(F32).T.astype(BF16)

    pairs = n_heads // 2
    half_blocks = HALF // RELAYOUT_ROWS

    def x_load(b):
        return xT_hbm.at[:, b * LANES:(b + 1) * LANES], xT.at[b], lambda: None

    def qkv_loads(m, src):
        def head_pair(block, p):
            n = RELAYOUT_ROWS * pairs
            slab = stage.at[m, pl.ds(block * n, n)]
            even, odd = (
                _split_words(slab[pl.ds(r * pairs + p, RELAYOUT_ROWS // 2, stride=2 * pairs), :])
                for r in range(2))
            return list(zip(even, odd))

        def split_main(i):
            rows = slice(i * RELAYOUT_ROWS // 2, (i + 1) * RELAYOUT_ROWS // 2)
            for g in range(pairs // 2):
                quads = [head_pair(i + k * half_blocks, 2 * g + n)
                         for k in range(2) for n in range(2)]
                for h in range(2):
                    col = m * HALF + h * head_dim
                    for j, op in enumerate(_strassen_rhs([q[h] for q in quads])):
                        qkv_main[g, j, rows, col:col + head_dim] = op

        def split_rest():
            for p in range(pairs):
                for h, w in enumerate(head_pair(2 * half_blocks, p)):
                    col = ((p % 2) * 3 + m) * HALF + h * head_dim
                    qkv_rest[p // 2, :, col:col + head_dim] = _pack(*w)

        def load(block, relayout):
            rows = pl.ds(block * RELAYOUT_ROWS * pairs, RELAYOUT_ROWS * pairs)
            return src.bitcast(U32).at[rows], stage.at[m, rows], relayout

        out = [load(2 * half_blocks, split_rest)]
        for i in range(half_blocks):
            out += [load(i, lambda: None),
                    load(i + half_blocks, functools.partial(split_main, i))]
        return out

    def store_out_weights(main, rest, block, transposed):
        def columns(k, lo, hi):
            return tuple(
                jnp.concatenate([flipped[k, t, pl.ds(r, LANES // 2, stride=2), :]
                                 for t in range(lo // LANES, hi // LANES)], axis=1)
                for r in range(2))

        for k in range(4):
            piece = _pad_rows(transposed(k).astype(F32), flipped.shape[1] * LANES)
            for t in range(flipped.shape[1]):
                flipped[k, t] = piece[t * LANES:(t + 1) * LANES].T
        for i in range(2):
            quads = [columns(i + 2 * k, n * HALF, (n + 1) * HALF)
                     for k in range(2) for n in range(2)]
            for j, op in enumerate(_strassen_rhs(quads)):
                main[block, j, i * LANES // 2:(i + 1) * LANES // 2, :] = op
        for k in range(4):
            words = _pack(*columns(k, 2 * HALF, 2 * HALF + LANES))
            rest[block, k * LANES // 2:(k + 1) * LANES // 2, :] = words[:, :rest.shape[-1]]

    def wo_load(g):
        heads = pl.ds(g * HEADS_PER_GROUP, HEADS_PER_GROUP)
        return (woT_hbm.at[heads], woT.at[heads], lambda: store_out_weights(
            wo_main, wo_rest, g, lambda i: woT[g * HEADS_PER_GROUP + i]))

    def w2_load(c):
        def piece(i):
            return w2T[:, c * FFN_CHUNK + i * LANES:c * FFN_CHUNK + (i + 1) * LANES]

        cols = slice(c * FFN_CHUNK, (c + 1) * FFN_CHUNK)
        return (w2T_hbm.at[:, cols], w2T.at[:, cols],
                lambda: store_out_weights(w2_main, w2_rest, c, piece))

    def w13_load(i, src, raw, c):
        def relayout():
            def piece(row, n_rows, n):
                col = c * FFN_CHUNK + n * HALF
                return pltpu.bitcast(raw[row:row + n_rows, col:col + HALF], U32)

            for r in range(half_blocks):
                quads = [_split_words(piece(k * HALF + r * RELAYOUT_ROWS, RELAYOUT_ROWS, n))
                         for k in range(2) for n in range(2)]
                rows = slice(r * RELAYOUT_ROWS // 2, (r + 1) * RELAYOUT_ROWS // 2)
                for j, op in enumerate(_strassen_rhs(quads)):
                    w13_main[c, j, rows, i * HALF:(i + 1) * HALF] = op
            for n in range(2):
                w13_rest[c, :, (2 * n + i) * HALF:(2 * n + i + 1) * HALF] = (
                    piece(2 * HALF, d_model - 2 * HALF, n))

        cols = slice(c * FFN_CHUNK, (c + 1) * FFN_CHUNK)
        return src.at[:, cols], raw.at[:, cols], relayout

    loads = [x_load(0)]
    loads += qkv_loads(0, wq_hbm) + qkv_loads(1, wk_hbm)
    loads += [wo_load(g) for g in range(n_heads // HEADS_PER_GROUP)]
    loads += qkv_loads(2, wv_hbm)
    n_attention_loads = len(loads)
    for c in range(n_chunks):
        loads += [w13_load(0, w1_hbm, w1_raw, c), w13_load(1, w3_hbm, w3_raw, c), w2_load(c)]
    n_weight_loads = len(loads)
    loads += [x_load(b) for b in range(1, n_blk)]
    copies = [pltpu.make_async_copy(src, dst, in_sems.at[i])
              for i, (src, dst, _) in enumerate(loads)]

    started = 0

    def start_loads(upto):
        nonlocal started
        for c in copies[started:upto]:
            c.start()
        started = max(started, min(upto, len(copies)))

    def finish_loads(lo, hi, ahead):
        for i in range(lo, hi):
            copies[i].wait()
        start_loads(hi + ahead)
        for i in range(lo, hi):
            loads[i][2]()

    start_loads(1 + LOADS_AHEAD)
    ys[...] = jnp.zeros(ys.shape, ys.dtype)
    for i in range(n_attention_loads):
        finish_loads(i, i + 1, LOADS_AHEAD)
    start_loads(n_attention_loads + 3 * CHUNKS_AHEAD)
    load_x_block(0)

    chunks_ready = 0

    def prepare_chunks(upto):
        nonlocal chunks_ready
        for c in range(chunks_ready, min(upto, n_chunks)):
            first = n_attention_loads + 3 * c
            finish_loads(first, first + 3, 3 * CHUNKS_AHEAD)
        chunks_ready = max(chunks_ready, upto)

    mem0 = mem0_ref[...].astype(F32)
    new_mem = mem0
    for s in range(2):
        tokens, new_mem = attention(
            xs[s * seg:(s + 1) * seg, :].astype(F32), new_mem, ffn=None,
            before_group=lambda g, s=s: prepare_chunks(FILL_CHUNKS[s][g]))
        store_attention(slice(s * seg, (s + 1) * seg), tokens)
    mem[...] = jnp.concatenate([new_mem, mem0], axis=0)
    b_out[...] = a_out[...] + new_ffn(lambda c: prepare_chunks(c + 2)).finish()
    a_out[:seg, :] = a_out[seg:, :]
    f_in[:seg, :] = f_in[seg:, :]
    start_loads(len(loads))
    finish_loads(n_weight_loads, len(loads), 0)

    def step(t):
        ffn, ffn_resid = new_ffn(), a_out[...]
        prev = b_out[...]
        emit_output(jnp.maximum(t - 4, 0), prev[seg:])
        resid = jnp.concatenate([xs[seg_rows(t), :].astype(F32), prev[:seg]], axis=0)
        tokens, new_mem = attention(resid, mem[...], ffn=ffn)
        mem[...] = new_mem
        store_attention(slice(None), tokens)
        load_x_block(jnp.minimum(t // segs_per_blk + 1, n_blk - 1))
        b_out[...] = ffn_resid + ffn.finish()

    def loop_body(t, carry):
        step(t)
        done = t - 4

        @pl.when((done >= 0) & (done % segs_per_blk == segs_per_blk - 1))
        def _():
            out_copy(done // segs_per_blk).start()

        return carry

    lax.fori_loop(2, n_seg, loop_body, 0)

    ffn, ffn_resid = new_ffn(), a_out[...]
    prev = b_out[...]
    emit_output(n_seg - 4, prev[seg:])
    tokens, new_mem = attention(prev[:seg], mem[n_mem:, :], ffn=ffn)
    last = ffn_resid + ffn.finish()
    store_attention(slice(0, seg), tokens)
    emit_output(n_seg - 3, last[seg:])
    tokens, _ = attention(last[:seg], new_mem, ffn=None)
    store_attention(slice(seg, 2 * seg), tokens)
    last = a_out[...] + new_ffn().finish()
    ys[(n_seg - 2) * seg:(n_seg - 1) * seg, :] = last[:seg]
    emit_output(n_seg - 1, last[seg:])
    out_copy(n_blk - 1).start()
    for b in range(n_blk):
        out_copy(b).wait()


@functools.partial(jax.jit, static_argnames=("A_seg_len",))
def pallas_interleave_layers__memory_aug_recurrent_mem_tr__glu_gated_swiglu__prompt_kernel(
    A_x, A_mem0, A_Wq, A_Wk, A_Wv, A_Wo, A_seg_len, B_x, B_w1, B_w3, B_w2,
):
    del B_x
    batch, seq, d_model = A_x.shape
    _, n_heads, head_dim = A_Wq.shape
    n_mem = A_mem0.shape[1]
    d_ff = B_w1.shape[1]
    seg = int(A_seg_len)
    n_seg = seq // seg
    assert batch == 1 and n_seg * seg == seq and LANES == 4 * seg and seq % LANES == 0
    assert head_dim == LANES and n_heads % HEADS_PER_GROUP == 0 and d_ff % FFN_CHUNK == 0

    n_groups = n_heads // HEADS_PER_GROUP
    n_chunks = d_ff // FFN_CHUNK
    rest = d_model - 2 * HALF
    assert rest == RELAYOUT_ROWS
    hbm = pl.BlockSpec(memory_space=pl.ANY)
    outT = pl.pallas_call(
        functools.partial(_kernel, seg=seg, n_seg=n_seg, n_heads=n_heads, head_dim=head_dim),
        out_shape=jax.ShapeDtypeStruct((d_model, seq), A_x.dtype),
        in_specs=[hbm, pl.BlockSpec(memory_space=pltpu.VMEM)] + [hbm] * 7,
        out_specs=hbm,
        scratch_shapes=[
            pltpu.VMEM((3, d_model * n_heads // 2, head_dim), U32),
            pltpu.VMEM((n_heads, d_model, head_dim), BF16),
            pltpu.VMEM((d_model, d_ff), BF16),
            pltpu.VMEM((d_model, d_ff), BF16),
            pltpu.VMEM((d_model, d_ff), BF16),
            pltpu.VMEM((4, pl.cdiv(d_model, LANES), LANES, LANES), F32),
            pltpu.VMEM((n_groups, 7, HALF // 2, 3 * HALF), U32),
            pltpu.VMEM((n_groups, rest // 2, 6 * HALF), U32),
            pltpu.VMEM((n_groups, 7, HALF // 2, HALF), U32),
            pltpu.VMEM((n_groups, HALF, rest), U32),
            pltpu.VMEM((n_chunks, 7, HALF // 2, 2 * HALF), U32),
            pltpu.VMEM((n_chunks, rest // 2, 4 * HALF), U32),
            pltpu.VMEM((n_chunks, 7, HALF // 2, HALF), U32),
            pltpu.VMEM((n_chunks, HALF, rest), U32),
            pltpu.VMEM((seq // LANES, d_model, LANES), BF16),
            pltpu.VMEM((seq, d_model), BF16),
            pltpu.VMEM((seq, d_model), F32),
            pltpu.VMEM((seq // LANES, d_model, LANES), BF16),
            pltpu.VMEM((2 * n_mem, d_model), F32),
            pltpu.VMEM((2 * seg, d_model), F32),
            pltpu.VMEM((2 * seg, d_model), F32),
            pltpu.VMEM((2 * seg, d_model), F32),
            pltpu.SemaphoreType.DMA((3 * d_model // RELAYOUT_ROWS + n_groups + 3 * n_chunks + seq // LANES,)),
            pltpu.SemaphoreType.DMA((seq // LANES,)),
        ],
        compiler_params=pltpu.CompilerParams(vmem_limit_bytes=120 * 2**20),
    )(
        A_x.reshape(seq, d_model).T,
        A_mem0.reshape(n_mem, d_model),
        A_Wq.reshape(d_model * n_heads, head_dim),
        A_Wk.reshape(d_model * n_heads, head_dim),
        A_Wv.reshape(d_model * n_heads, head_dim),
        A_Wo.transpose(0, 2, 1),
        B_w1,
        B_w3,
        B_w2.T,
    )
    return outT.T.reshape(batch, seq, d_model)
```

```python
import functools
import math

import jax
import jax.numpy as jnp
from jax import lax
import jax.experimental.pallas as pl
import jax.experimental.pallas.tpu as pltpu

F32 = jnp.float32
BF16 = jnp.bfloat16
U32 = jnp.uint32
LANES = 128
HEADS_PER_GROUP = 4
HALF = 2 * LANES
FFN_CHUNK = 2 * HALF
RELAYOUT_ROWS = 64
LOADS_AHEAD = 4
FILL_CHUNKS = ((0, 0, 0, 0, 0, 0, 0, 0), (1, 1, 2, 2, 3, 3, 4, 4))
CHUNKS_AHEAD = 3
FILL_START = 3
FILL_FIRST = 1
FILL_SOFTMAX = 2
FILL_PROJECT = (0, 1, 0, 0, 0, 0, 0)
FILL_LAST = 1
LN_EPS = 1e-5
MASK_VALUE = -1000000000.0
LOG2E = math.log2(math.e)
NT_DIMS = (((1,), (1,)), ((), ()))


def _pack(even_rows, odd_rows):
    return pltpu.pack_elementwise([even_rows, odd_rows], packed_dtype=BF16).astype(U32)


def _split_words(words):
    return (lax.bitcast_convert_type(words << 16, F32),
            lax.bitcast_convert_type(words & jnp.uint32(0xFFFF0000), F32))


def _layernorm(x):
    mean = jnp.mean(x, axis=-1, keepdims=True)
    cen = x - mean
    var = jnp.mean(cen * cen, axis=-1, keepdims=True)
    return cen * lax.rsqrt(var + LN_EPS)


def _dot(lhs, packed_rhs):
    return jnp.dot(lhs, pltpu.bitcast(packed_rhs, BF16), preferred_element_type=F32)


def _strassen_rhs(quads):
    def operands(b11, b12, b21, b22):
        return [b11 + b22, b11, b12 - b22, b21 - b11, b22, b11 + b12, b21 + b22]

    return [_pack(even, odd) for even, odd in
            zip(operands(*(q[0] for q in quads)), operands(*(q[1] for q in quads)))]


def _pad_rows(x, rows):
    if x.shape[0] == rows:
        return x
    return jnp.concatenate([x, jnp.zeros((rows - x.shape[0], x.shape[1]), x.dtype)], axis=0)


def _strassen_lhs(left, right, top):
    a11, a12 = left[:top], right[:top]
    if left.shape[0] == top:
        ops = [a11, None, a11, None, a11 + a12, None, a12]
    else:
        a21, a22 = left[top:], right[top:]
        a22_tall = _pad_rows(a22, top)
        ops = [a11 + a22_tall, a21 + a22, a11, a22, a11 + a12,
               a21 - a11[:a21.shape[0]], a12 - a22_tall]
    return [None if op is None else op.astype(BF16) for op in ops]


def _strassen_combine(m):
    m1, m2, m3, m4, m5, m6, m7 = m
    if m2 is None:
        return m1 - m5 + m7, m3 + m5
    bottom = m2.shape[0]
    left = [m1 + _pad_rows(m4, m1.shape[0]) - m5 + m7, m2 + m4]
    right = [m3 + m5, m1[:bottom] - m2 + m3[:bottom] + m6]
    return jnp.concatenate(left, axis=0), jnp.concatenate(right, axis=0)


class _InProjection:
    def __init__(self, x, top, w_main, w_rest):
        self.ops = _strassen_lhs(x[:, :HALF], x[:, HALF:2 * HALF], top)
        self.rest = x[:, 2 * HALF:].astype(BF16)
        self.w_main, self.w_rest = w_main, w_rest

    def tile(self, block, n):
        cols = slice(n * LANES, (n + 1) * LANES)
        width = self.w_main.shape[-1]
        left, right = _strassen_combine(
            [None if op is None else _dot(op, self.w_main[block, j, :, cols])
             for j, op in enumerate(self.ops)])
        rest = [_dot(self.rest, self.w_rest[block, :, base + n * LANES:base + (n + 1) * LANES])
                for base in (0, width)]
        return left + rest[0], right + rest[1]


class _OutProjection:
    def __init__(self, top, w_main, w_rest, rest_transposed=False):
        self.top, self.w_main, self.w_rest = top, w_main, w_rest
        self.rest_transposed = rest_transposed
        self.acc = None

    def add(self, block, left, right):
        parts = [None if op is None else _dot(op, self.w_main[block, j])
                 for j, op in enumerate(_strassen_lhs(left, right, self.top))]
        both = jnp.concatenate([left, right], axis=1).astype(BF16)
        if self.rest_transposed:
            parts.append(lax.dot_general(pltpu.bitcast(self.w_rest[block], BF16), both, NT_DIMS,
                                         preferred_element_type=F32))
        else:
            parts.append(_dot(both, self.w_rest[block]))
        if self.acc is None:
            self.acc = parts
        else:
            self.acc = [None if a is None else a + b for a, b in zip(self.acc, parts)]

    def result(self):
        rest = self.acc[7].T if self.rest_transposed else self.acc[7]
        return jnp.concatenate([*_strassen_combine(self.acc[:7]), rest], axis=1)


class _Ffn:
    def __init__(self, normed, weights, before_chunk=None):
        in_main, in_rest, out_main, out_rest = weights
        top = normed.shape[0] // 2
        self.project = _InProjection(normed, top, in_main, in_rest)
        self.output = _OutProjection(top, out_main, out_rest)
        self.before_chunk = before_chunk
        self.partial, self.hidden = {}, {}
        n_chunks = in_main.shape[0]
        self.todo = []
        for c in range(n_chunks):
            self.todo += [(self._begin, c), (self._activate, c)]
            if c > 0:
                self.todo.append((self._down, c - 1))
        self.todo.append((self._down, n_chunks - 1))

    def _hidden_tile(self, c, n):
        gate = self.project.tile(c, n)
        up = self.project.tile(c, HALF // LANES + n)
        return [g * jax.nn.sigmoid(g) * u for g, u in zip(gate, up)]

    def _begin(self, c):
        if self.before_chunk is not None:
            self.before_chunk(c)
        self.partial[c] = self._hidden_tile(c, 0)

    def _activate(self, c):
        self.hidden[c] = [jnp.concatenate(pair, axis=1)
                          for pair in zip(self.partial.pop(c), self._hidden_tile(c, 1))]

    def _down(self, c):
        self.output.add(c, *self.hidden.pop(c))

    def run(self, count):
        for fn, c in self.todo[:count]:
            fn(c)
        self.todo = self.todo[count:]

    def finish(self):
        self.run(len(self.todo))
        return self.output.result()


def _attention_mask(rows, seg, n_mem):
    def describe(axis):
        i = lax.broadcasted_iota(jnp.int32, (rows, rows), axis)
        second = i >= seg + n_mem
        pos = jnp.where(second, i - seg - n_mem, jnp.where(i < seg, i + n_mem, i - seg))
        return second.astype(jnp.int32), pos

    q_layer, q_pos = describe(0)
    k_layer, k_pos = describe(1)
    same = q_layer == k_layer
    visible = same & ((q_pos < n_mem) | (q_pos >= k_pos))
    fill = jnp.where(same, MASK_VALUE * LOG2E, -jnp.inf).astype(F32)
    return visible, fill


def _attention(resid, mem, ffn, before_group=None, *, weights, seg, head_dim):
    in_main, in_rest, out_main, out_rest = weights
    n_groups = in_main.shape[0]
    mem_rows = mem.shape[0]
    top = seg + mem_rows
    normed = _layernorm(resid)
    stacked = [normed[:seg], mem] + ([normed[seg:]] if resid.shape[0] > seg else [])
    stacked = jnp.concatenate(stacked, axis=0)
    visible, fill = _attention_mask(stacked.shape[0], seg, mem_rows * seg // resid.shape[0])
    score_scale = head_dim ** -0.5 * LOG2E
    projection = _InProjection(stacked, top, in_main, in_rest)
    output = _OutProjection(top, out_main, out_rest, rest_transposed=True)

    def project(g):
        return [[half.astype(BF16) for half in projection.tile(g, n)]
                for n in range(3 * HALF // LANES)]

    def head(qkv, m, i):
        return qkv[2 * m + i % 2][i // 2]

    def scores(qkv):
        probs = []
        for i in range(HEADS_PER_GROUP):
            s = lax.dot_general(head(qkv, 0, i), head(qkv, 1, i), NT_DIMS,
                                preferred_element_type=F32)
            s = jnp.where(visible, s * score_scale, fill)
            p = jnp.exp2(s - jnp.max(s, axis=-1, keepdims=True))
            probs.append((p.astype(BF16), 1.0 / jnp.sum(p, axis=-1, keepdims=True)))
        return probs

    def mix(qkv, probs):
        o = [jnp.dot(p, head(qkv, 2, i), preferred_element_type=F32) * inv
             for i, (p, inv) in enumerate(probs)]
        return jnp.concatenate(o[:2], axis=1), jnp.concatenate(o[2:], axis=1)

    if ffn is not None:
        ffn.run(FILL_START)
        qkv = project(0)
        ffn.run(FILL_FIRST)
        for g in range(n_groups):
            probs = scores(qkv)
            ffn.run(FILL_SOFTMAX)
            o = mix(qkv, probs)
            if g + 1 < n_groups:
                qkv = project(g + 1)
                ffn.run(FILL_PROJECT[g % len(FILL_PROJECT)])
            else:
                ffn.run(FILL_LAST)
            output.add(g, *o)
    else:
        qkv, o = project(0), None
        nxt = project(1)
        for g in range(n_groups):
            if before_group is not None:
                before_group(g)
            probs = scores(qkv)
            if o is not None:
                output.add(g - 1, *o)
            after = project(g + 2) if g + 2 < n_groups else None
            o = mix(qkv, probs)
            qkv, nxt = nxt, after
        output.add(n_groups - 1, *o)
    out = output.result()
    tokens = [out[:seg]] + ([out[top:]] if resid.shape[0] > seg else [])
    return resid + jnp.concatenate(tokens, axis=0), out[seg:top]


def _kernel(xT_hbm, mem0_ref, wq_hbm, wk_hbm, wv_hbm, woT_hbm, w1_hbm, w3_hbm, w2T_hbm,
            outT_hbm,
            stage, woT, w1_raw, w3_raw, w2T, flipped,
            qkv_main, qkv_rest, wo_main, wo_rest, w13_main, w13_rest, w2_main, w2_rest,
            xT, xs, ys, outT,
            mem, a_out, f_in, b_out, in_sems, out_sems,
            *, seg, n_seg, n_heads, head_dim):
    d_model = xs.shape[1]
    n_mem = mem0_ref.shape[0]
    n_chunks = w1_raw.shape[1] // FFN_CHUNK
    segs_per_blk = LANES // seg
    n_blk = n_seg // segs_per_blk
    attention = functools.partial(_attention, weights=(qkv_main, qkv_rest, wo_main, wo_rest),
                                  seg=seg, head_dim=head_dim)

    def out_copy(b):
        cols = pl.ds(pl.multiple_of(b * LANES, LANES), LANES)
        return pltpu.make_async_copy(outT.at[b], outT_hbm.at[:, cols], out_sems.at[b])

    def seg_rows(s):
        return pl.ds(pl.multiple_of(s * seg, seg), seg)

    def emit_output(s, y):
        ys[seg_rows(s), :] = y
        b = s // segs_per_blk
        rows = ys[pl.ds(pl.multiple_of(b * LANES, LANES), LANES), :]
        outT[b] = rows.T.astype(BF16)

    def new_ffn(before_chunk=None):
        return _Ffn(f_in[...], (w13_main, w13_rest, w2_main, w2_rest), before_chunk)

    def store_attention(rows, tokens):
        a_out[rows, :] = tokens
        f_in[rows, :] = _layernorm(tokens)

    def load_x_block(b):
        start = b * LANES if isinstance(b, int) else pl.multiple_of(b * LANES, LANES)
        xs[pl.ds(start, LANES), :] = xT[b].astype(F32).T.astype(BF16)

    pairs = n_heads // 2
    half_blocks = HALF // RELAYOUT_ROWS

    def x_load(b):
        return xT_hbm.at[:, b * LANES:(b + 1) * LANES], xT.at[b], lambda: None

    def qkv_loads(m, src):
        def head_pair(block, p):
            n = RELAYOUT_ROWS * pairs
            slab = stage.at[m, pl.ds(block * n, n)]
            even, odd = (
                _split_words(slab[pl.ds(r * pairs + p, RELAYOUT_ROWS // 2, stride=2 * pairs), :])
                for r in range(2))
            return list(zip(even, odd))

        def split_main(i):
            rows = slice(i * RELAYOUT_ROWS // 2, (i + 1) * RELAYOUT_ROWS // 2)
            for g in range(pairs // 2):
                quads = [head_pair(i + k * half_blocks, 2 * g + n)
                         for k in range(2) for n in range(2)]
                for h in range(2):
                    col = m * HALF + h * head_dim
                    for j, op in enumerate(_strassen_rhs([q[h] for q in quads])):
                        qkv_main[g, j, rows, col:col + head_dim] = op

        def split_rest():
            for p in range(pairs):
                for h, w in enumerate(head_pair(2 * half_blocks, p)):
                    col = ((p % 2) * 3 + m) * HALF + h * head_dim
                    qkv_rest[p // 2, :, col:col + head_dim] = _pack(*w)

        def load(block, relayout):
            rows = pl.ds(block * RELAYOUT_ROWS * pairs, RELAYOUT_ROWS * pairs)
            return src.bitcast(U32).at[rows], stage.at[m, rows], relayout

        out = [load(2 * half_blocks, split_rest)]
        for i in range(half_blocks):
            out += [load(i, lambda: None),
                    load(i + half_blocks, functools.partial(split_main, i))]
        return out

    def store_out_weights(main, block, transposed, rest=None):
        def columns(k, lo, hi):
            return tuple(
                jnp.concatenate([flipped[k, t, pl.ds(r, LANES // 2, stride=2), :]
                                 for t in range(lo // LANES, hi // LANES)], axis=1)
                for r in range(2))

        for k in range(4):
            piece = _pad_rows(transposed(k).astype(F32), flipped.shape[1] * LANES)
            for t in range(2 * HALF // LANES if rest is None else flipped.shape[1]):
                flipped[k, t] = piece[t * LANES:(t + 1) * LANES].T
        for i in range(2):
            quads = [columns(i + 2 * k, n * HALF, (n + 1) * HALF)
                     for k in range(2) for n in range(2)]
            for j, op in enumerate(_strassen_rhs(quads)):
                main[block, j, i * LANES // 2:(i + 1) * LANES // 2, :] = op
        for k in range(0 if rest is None else 4):
            words = _pack(*columns(k, 2 * HALF, 2 * HALF + LANES))
            rest[block, k * LANES // 2:(k + 1) * LANES // 2, :] = words[:, :rest.shape[-1]]

    def wo_load(g):
        def relayout():
            store_out_weights(wo_main, g, lambda i: woT[g * HEADS_PER_GROUP + i])
            for i in range(HEADS_PER_GROUP):
                wo_rest[g, :, i * head_dim:(i + 1) * head_dim] = pltpu.bitcast(
                    woT[g * HEADS_PER_GROUP + i, 2 * HALF:, :], U32)

        heads = pl.ds(g * HEADS_PER_GROUP, HEADS_PER_GROUP)
        return woT_hbm.at[heads], woT.at[heads], relayout

    def w2_load(c):
        def piece(i):
            return w2T[:, c * FFN_CHUNK + i * LANES:c * FFN_CHUNK + (i + 1) * LANES]

        cols = slice(c * FFN_CHUNK, (c + 1) * FFN_CHUNK)
        return (w2T_hbm.at[:, cols], w2T.at[:, cols],
                lambda: store_out_weights(w2_main, c, piece, w2_rest))

    def w13_load(i, src, raw, c):
        def relayout():
            def piece(row, n_rows, n):
                col = c * FFN_CHUNK + n * HALF
                return pltpu.bitcast(raw[row:row + n_rows, col:col + HALF], U32)

            for r in range(half_blocks):
                quads = [_split_words(piece(k * HALF + r * RELAYOUT_ROWS, RELAYOUT_ROWS, n))
                         for k in range(2) for n in range(2)]
                rows = slice(r * RELAYOUT_ROWS // 2, (r + 1) * RELAYOUT_ROWS // 2)
                for j, op in enumerate(_strassen_rhs(quads)):
                    w13_main[c, j, rows, i * HALF:(i + 1) * HALF] = op
            for n in range(2):
                w13_rest[c, :, (2 * n + i) * HALF:(2 * n + i + 1) * HALF] = (
                    piece(2 * HALF, d_model - 2 * HALF, n))

        cols = slice(c * FFN_CHUNK, (c + 1) * FFN_CHUNK)
        return src.at[:, cols], raw.at[:, cols], relayout

    loads = [x_load(0)]
    for m, src in enumerate([wq_hbm, wk_hbm, wv_hbm]):
        loads += qkv_loads(m, src)
    n_qkv_loads = len(loads)
    loads += [wo_load(g) for g in range(n_heads // HEADS_PER_GROUP)]
    n_attention_loads = len(loads)
    for c in range(n_chunks):
        loads += [w13_load(0, w1_hbm, w1_raw, c), w13_load(1, w3_hbm, w3_raw, c), w2_load(c)]
    n_weight_loads = len(loads)
    loads += [x_load(b) for b in range(1, n_blk)]
    copies = [pltpu.make_async_copy(src, dst, in_sems.at[i])
              for i, (src, dst, _) in enumerate(loads)]

    started = 0

    def start_loads(upto):
        nonlocal started
        for c in copies[started:upto]:
            c.start()
        started = max(started, min(upto, len(copies)))

    def finish_loads(lo, hi, ahead):
        for i in range(lo, hi):
            copies[i].wait()
        start_loads(hi + ahead)
        for i in range(lo, hi):
            loads[i][2]()

    start_loads(1 + LOADS_AHEAD)
    ys[...] = jnp.zeros(ys.shape, ys.dtype)
    for i in range(n_qkv_loads):
        finish_loads(i, i + 1, LOADS_AHEAD)
    start_loads(n_attention_loads + 3)
    load_x_block(0)

    chunks_ready = 0

    def prepare_chunks(upto):
        nonlocal chunks_ready
        for c in range(chunks_ready, min(upto, n_chunks)):
            first = n_attention_loads + 3 * c
            finish_loads(first, first + 3, 3 * CHUNKS_AHEAD)
        chunks_ready = max(chunks_ready, upto)

    def prepare_weights(s, g):
        if s == 0:
            finish_loads(n_qkv_loads + g, n_qkv_loads + g + 1, 3 * CHUNKS_AHEAD)
        prepare_chunks(FILL_CHUNKS[s][g])

    mem0 = mem0_ref[...].astype(F32)
    new_mem = mem0
    for s in range(2):
        tokens, new_mem = attention(
            xs[s * seg:(s + 1) * seg, :].astype(F32), new_mem, ffn=None,
            before_group=functools.partial(prepare_weights, s))
        store_attention(slice(s * seg, (s + 1) * seg), tokens)
    mem[...] = jnp.concatenate([new_mem, mem0], axis=0)
    b_out[...] = a_out[...] + new_ffn(lambda c: prepare_chunks(c + 2)).finish()
    a_out[:seg, :] = a_out[seg:, :]
    f_in[:seg, :] = f_in[seg:, :]
    start_loads(len(loads))
    finish_loads(n_weight_loads, len(loads), 0)

    def step(t):
        ffn, ffn_resid = new_ffn(), a_out[...]
        prev = b_out[...]
        emit_output(jnp.maximum(t - 4, 0), prev[seg:])
        resid = jnp.concatenate([xs[seg_rows(t), :].astype(F32), prev[:seg]], axis=0)
        tokens, new_mem = attention(resid, mem[...], ffn=ffn)
        mem[...] = new_mem
        store_attention(slice(None), tokens)
        load_x_block(jnp.minimum(t // segs_per_blk + 1, n_blk - 1))
        b_out[...] = ffn_resid + ffn.finish()

    def loop_body(t, carry):
        step(t)
        done = t - 4

        @pl.when((done >= 0) & (done % segs_per_blk == segs_per_blk - 1))
        def _():
            out_copy(done // segs_per_blk).start()

        return carry

    lax.fori_loop(2, n_seg, loop_body, 0)

    ffn, ffn_resid = new_ffn(), a_out[...]
    prev = b_out[...]
    emit_output(n_seg - 4, prev[seg:])
    tokens, new_mem = attention(prev[:seg], mem[n_mem:, :], ffn=ffn)
    last = ffn_resid + ffn.finish()
    store_attention(slice(0, seg), tokens)
    emit_output(n_seg - 3, last[seg:])
    tokens, _ = attention(last[:seg], new_mem, ffn=None)
    store_attention(slice(seg, 2 * seg), tokens)
    last = a_out[...] + new_ffn().finish()
    ys[(n_seg - 2) * seg:(n_seg - 1) * seg, :] = last[:seg]
    emit_output(n_seg - 1, last[seg:])
    out_copy(n_blk - 1).start()
    for b in range(n_blk):
        out_copy(b).wait()


@functools.partial(jax.jit, static_argnames=("A_seg_len",))
def pallas_interleave_layers__memory_aug_recurrent_mem_tr__glu_gated_swiglu__prompt_kernel(
    A_x, A_mem0, A_Wq, A_Wk, A_Wv, A_Wo, A_seg_len, B_x, B_w1, B_w3, B_w2,
):
    del B_x
    batch, seq, d_model = A_x.shape
    _, n_heads, head_dim = A_Wq.shape
    n_mem = A_mem0.shape[1]
    d_ff = B_w1.shape[1]
    seg = int(A_seg_len)
    n_seg = seq // seg
    assert batch == 1 and n_seg * seg == seq and LANES == 4 * seg and seq % LANES == 0
    assert head_dim == LANES and n_heads % HEADS_PER_GROUP == 0 and d_ff % FFN_CHUNK == 0

    n_groups = n_heads // HEADS_PER_GROUP
    n_chunks = d_ff // FFN_CHUNK
    rest = d_model - 2 * HALF
    assert rest == RELAYOUT_ROWS
    hbm = pl.BlockSpec(memory_space=pl.ANY)
    outT = pl.pallas_call(
        functools.partial(_kernel, seg=seg, n_seg=n_seg, n_heads=n_heads, head_dim=head_dim),
        out_shape=jax.ShapeDtypeStruct((d_model, seq), A_x.dtype),
        in_specs=[hbm, pl.BlockSpec(memory_space=pltpu.VMEM)] + [hbm] * 7,
        out_specs=hbm,
        scratch_shapes=[
            pltpu.VMEM((3, d_model * n_heads // 2, head_dim), U32),
            pltpu.VMEM((n_heads, d_model, head_dim), BF16),
            pltpu.VMEM((d_model, d_ff), BF16),
            pltpu.VMEM((d_model, d_ff), BF16),
            pltpu.VMEM((d_model, d_ff), BF16),
            pltpu.VMEM((4, pl.cdiv(d_model, LANES), LANES, LANES), F32),
            pltpu.VMEM((n_groups, 7, HALF // 2, 3 * HALF), U32),
            pltpu.VMEM((n_groups, rest // 2, 6 * HALF), U32),
            pltpu.VMEM((n_groups, 7, HALF // 2, HALF), U32),
            pltpu.VMEM((n_groups, rest // 2, 2 * HALF), U32),
            pltpu.VMEM((n_chunks, 7, HALF // 2, 2 * HALF), U32),
            pltpu.VMEM((n_chunks, rest // 2, 4 * HALF), U32),
            pltpu.VMEM((n_chunks, 7, HALF // 2, HALF), U32),
            pltpu.VMEM((n_chunks, HALF, rest), U32),
            pltpu.VMEM((seq // LANES, d_model, LANES), BF16),
            pltpu.VMEM((seq, d_model), BF16),
            pltpu.VMEM((seq, d_model), F32),
            pltpu.VMEM((seq // LANES, d_model, LANES), BF16),
            pltpu.VMEM((2 * n_mem, d_model), F32),
            pltpu.VMEM((2 * seg, d_model), F32),
            pltpu.VMEM((2 * seg, d_model), F32),
            pltpu.VMEM((2 * seg, d_model), F32),
            pltpu.SemaphoreType.DMA((3 * d_model // RELAYOUT_ROWS + n_groups + 3 * n_chunks + seq // LANES,)),
            pltpu.SemaphoreType.DMA((seq // LANES,)),
        ],
        compiler_params=pltpu.CompilerParams(vmem_limit_bytes=120 * 2**20),
    )(
        A_x.reshape(seq, d_model).T,
        A_mem0.reshape(n_mem, d_model),
        A_Wq.reshape(d_model * n_heads, head_dim),
        A_Wk.reshape(d_model * n_heads, head_dim),
        A_Wv.reshape(d_model * n_heads, head_dim),
        A_Wo.transpose(0, 2, 1),
        B_w1,
        B_w3,
        B_w2.T,
    )
    return outT.T.reshape(batch, seq, d_model)
```

```python
import functools
import math

import jax
import jax.numpy as jnp
from jax import lax
import jax.experimental.pallas as pl
import jax.experimental.pallas.tpu as pltpu

F32 = jnp.float32
BF16 = jnp.bfloat16
U32 = jnp.uint32
LANES = 128
HEADS_PER_GROUP = 4
HALF = 2 * LANES
FFN_CHUNK = 2 * HALF
RELAYOUT_ROWS = 64
FIRST_X_BLOCKS = 5
LOADS_AHEAD = 8
FILL_CHUNKS = ((0, 0, 0, 0, 0, 0, 0, 0), (1, 1, 2, 2, 3, 3, 4, 4))
CHUNKS_AHEAD = 5
FILL_START = 3
FILL_FIRST = 1
FILL_SOFTMAX = 2
FILL_PROJECT = (0, 1, 0, 0, 0, 0, 0)
FILL_LAST = 1
LN_EPS = 1e-5
MASK_VALUE = -1000000000.0
LOG2E = math.log2(math.e)
NT_DIMS = (((1,), (1,)), ((), ()))


def _pack(even_rows, odd_rows):
    return pltpu.pack_elementwise([even_rows, odd_rows], packed_dtype=BF16).astype(U32)


def _split_words(words):
    return (lax.bitcast_convert_type(words << 16, F32),
            lax.bitcast_convert_type(words & jnp.uint32(0xFFFF0000), F32))


def _layernorm(x):
    mean = jnp.mean(x, axis=-1, keepdims=True)
    cen = x - mean
    var = jnp.mean(cen * cen, axis=-1, keepdims=True)
    return cen * lax.rsqrt(var + LN_EPS)


def _dot(lhs, packed_rhs):
    return jnp.dot(lhs, pltpu.bitcast(packed_rhs, BF16), preferred_element_type=F32)


def _strassen_rhs(quads):
    def operands(b11, b12, b21, b22):
        return [b11 + b22, b11, b12 - b22, b21 - b11, b22, b11 + b12, b21 + b22]

    return [_pack(even, odd) for even, odd in
            zip(operands(*(q[0] for q in quads)), operands(*(q[1] for q in quads)))]


def _pad_rows(x, rows):
    if x.shape[0] == rows:
        return x
    return jnp.concatenate([x, jnp.zeros((rows - x.shape[0], x.shape[1]), x.dtype)], axis=0)


def _strassen_lhs(left, right, top):
    a11, a12 = left[:top], right[:top]
    if left.shape[0] == top:
        ops = [a11, None, a11, None, a11 + a12, None, a12]
    else:
        a21, a22 = left[top:], right[top:]
        a22_tall = _pad_rows(a22, top)
        ops = [a11 + a22_tall, a21 + a22, a11, a22, a11 + a12,
               a21 - a11[:a21.shape[0]], a12 - a22_tall]
    return [None if op is None else op.astype(BF16) for op in ops]


def _strassen_combine(m):
    m1, m2, m3, m4, m5, m6, m7 = m
    if m2 is None:
        return m1 - m5 + m7, m3 + m5
    bottom = m2.shape[0]
    left = [m1 + _pad_rows(m4, m1.shape[0]) - m5 + m7, m2 + m4]
    right = [m3 + m5, m1[:bottom] - m2 + m3[:bottom] + m6]
    return jnp.concatenate(left, axis=0), jnp.concatenate(right, axis=0)


class _InProjection:
    def __init__(self, x, top, w_main, w_rest):
        self.ops = _strassen_lhs(x[:, :HALF], x[:, HALF:2 * HALF], top)
        self.rest = x[:, 2 * HALF:].astype(BF16)
        self.w_main, self.w_rest = w_main, w_rest

    def tile(self, block, n):
        cols = slice(n * LANES, (n + 1) * LANES)
        width = self.w_main.shape[-1]
        left, right = _strassen_combine(
            [None if op is None else _dot(op, self.w_main[block, j, :, cols])
             for j, op in enumerate(self.ops)])
        rest = [_dot(self.rest, self.w_rest[block, :, base + n * LANES:base + (n + 1) * LANES])
                for base in (0, width)]
        return left + rest[0], right + rest[1]


class _OutProjection:
    def __init__(self, top, w_main, w_rest, rest_transposed=False):
        self.top, self.w_main, self.w_rest = top, w_main, w_rest
        self.rest_transposed = rest_transposed
        self.acc = None

    def add(self, block, left, right):
        parts = [None if op is None else _dot(op, self.w_main[block, j])
                 for j, op in enumerate(_strassen_lhs(left, right, self.top))]
        both = jnp.concatenate([left, right], axis=1).astype(BF16)
        if self.rest_transposed:
            parts.append(lax.dot_general(pltpu.bitcast(self.w_rest[block], BF16), both, NT_DIMS,
                                         preferred_element_type=F32))
        else:
            parts.append(_dot(both, self.w_rest[block]))
        if self.acc is None:
            self.acc = parts
        else:
            self.acc = [None if a is None else a + b for a, b in zip(self.acc, parts)]

    def result(self):
        rest = self.acc[7].T if self.rest_transposed else self.acc[7]
        return jnp.concatenate([*_strassen_combine(self.acc[:7]), rest], axis=1)


class _Ffn:
    def __init__(self, normed, weights, before_chunk=None):
        in_main, in_rest, out_main, out_rest = weights
        top = normed.shape[0] // 2
        self.project = _InProjection(normed, top, in_main, in_rest)
        self.output = _OutProjection(top, out_main, out_rest)
        self.before_chunk = before_chunk
        self.partial, self.hidden = {}, {}
        n_chunks = in_main.shape[0]
        self.todo = []
        for c in range(n_chunks):
            self.todo += [(self._begin, c), (self._activate, c)]
            if c > 0:
                self.todo.append((self._down, c - 1))
        self.todo.append((self._down, n_chunks - 1))

    def _hidden_tile(self, c, n):
        gate = self.project.tile(c, n)
        up = self.project.tile(c, HALF // LANES + n)
        return [g * jax.nn.sigmoid(g) * u for g, u in zip(gate, up)]

    def _begin(self, c):
        if self.before_chunk is not None:
            self.before_chunk(c)
        self.partial[c] = self._hidden_tile(c, 0)

    def _activate(self, c):
        self.hidden[c] = [jnp.concatenate(pair, axis=1)
                          for pair in zip(self.partial.pop(c), self._hidden_tile(c, 1))]

    def _down(self, c):
        self.output.add(c, *self.hidden.pop(c))

    def run(self, count):
        for fn, c in self.todo[:count]:
            fn(c)
        self.todo = self.todo[count:]

    def finish(self):
        self.run(len(self.todo))
        return self.output.result()


def _attention_mask(rows, seg, n_mem):
    def describe(axis):
        i = lax.broadcasted_iota(jnp.int32, (rows, rows), axis)
        second = i >= seg + n_mem
        pos = jnp.where(second, i - seg - n_mem, jnp.where(i < seg, i + n_mem, i - seg))
        return second.astype(jnp.int32), pos

    q_layer, q_pos = describe(0)
    k_layer, k_pos = describe(1)
    same = q_layer == k_layer
    visible = same & ((q_pos < n_mem) | (q_pos >= k_pos))
    fill = jnp.where(same, MASK_VALUE * LOG2E, -jnp.inf).astype(F32)
    return visible, fill


def _attention(resid, mem, ffn, before_group=None, update_mem=True, *, weights, seg, head_dim):
    in_main, in_rest, out_main, out_rest = weights
    n_groups = in_main.shape[0]
    mem_rows = mem.shape[0]
    top = seg + mem_rows
    normed = _layernorm(resid)
    stacked = [normed[:seg], mem] + ([normed[seg:]] if resid.shape[0] > seg else [])
    stacked = jnp.concatenate(stacked, axis=0)
    visible, fill = _attention_mask(stacked.shape[0], seg, mem_rows * seg // resid.shape[0])
    score_scale = head_dim ** -0.5 * LOG2E
    projection = _InProjection(stacked, top, in_main, in_rest)
    query_projection, query_top = projection, top
    if not update_mem:
        query_projection, query_top = _InProjection(normed, seg, in_main, in_rest), seg
        visible, fill = visible[:seg], fill[:seg]
    output = _OutProjection(query_top, out_main, out_rest, rest_transposed=True)

    def project(g):
        tiles = HALF // LANES
        return [[half.astype(BF16)
                 for half in (query_projection if n < tiles else projection).tile(g, n)]
                for n in range(3 * tiles)]

    def head(qkv, m, i):
        return qkv[2 * m + i % 2][i // 2]

    def scores(qkv):
        probs = []
        for i in range(HEADS_PER_GROUP):
            s = lax.dot_general(head(qkv, 0, i), head(qkv, 1, i), NT_DIMS,
                                preferred_element_type=F32)
            s = jnp.where(visible, s * score_scale, fill)
            p = jnp.exp2(s - jnp.max(s, axis=-1, keepdims=True))
            probs.append((p.astype(BF16), 1.0 / jnp.sum(p, axis=-1, keepdims=True)))
        return probs

    def mix(qkv, probs):
        o = [jnp.dot(p, head(qkv, 2, i), preferred_element_type=F32) * inv
             for i, (p, inv) in enumerate(probs)]
        return jnp.concatenate(o[:2], axis=1), jnp.concatenate(o[2:], axis=1)

    if ffn is not None:
        ffn.run(FILL_START)
        qkv = project(0)
        ffn.run(FILL_FIRST)
        for g in range(n_groups):
            probs = scores(qkv)
            ffn.run(FILL_SOFTMAX)
            o = mix(qkv, probs)
            if g + 1 < n_groups:
                qkv = project(g + 1)
                ffn.run(FILL_PROJECT[g % len(FILL_PROJECT)])
            else:
                ffn.run(FILL_LAST)
            output.add(g, *o)
    else:
        qkv, o = project(0), None
        nxt = project(1)
        for g in range(n_groups):
            if before_group is not None:
                before_group(g)
            probs = scores(qkv)
            if o is not None:
                output.add(g - 1, *o)
            after = project(g + 2) if g + 2 < n_groups else None
            o = mix(qkv, probs)
            qkv, nxt = nxt, after
        output.add(n_groups - 1, *o)
    out = output.result()
    tokens = [out[:seg]] + ([out[top:]] if resid.shape[0] > seg else [])
    return resid + jnp.concatenate(tokens, axis=0), (out[seg:top] if update_mem else None)


def _kernel(xT_hbm, mem0_ref, wq_hbm, wk_hbm, wv_hbm, woT_hbm, w1_hbm, w3_hbm, w2T_hbm,
            outT_hbm,
            stage, woT, w1_raw, w3_raw, w2T, flipped,
            qkv_main, qkv_rest, wo_main, wo_rest, w13_main, w13_rest, w2_main, w2_rest,
            xT, xs, ys, outT,
            mem, a_out, f_in, b_out, in_sems, out_sems,
            *, seg, n_seg, n_heads, head_dim):
    d_model = xs.shape[1]
    n_mem = mem0_ref.shape[0]
    n_chunks = w1_raw.shape[1] // FFN_CHUNK
    segs_per_blk = LANES // seg
    n_blk = n_seg // segs_per_blk
    attention = functools.partial(_attention, weights=(qkv_main, qkv_rest, wo_main, wo_rest),
                                  seg=seg, head_dim=head_dim)

    def out_copy(b):
        cols = pl.ds(pl.multiple_of(b * LANES, LANES), LANES)
        return pltpu.make_async_copy(outT.at[b], outT_hbm.at[:, cols], out_sems.at[b])

    def seg_rows(s):
        return pl.ds(pl.multiple_of(s * seg, seg), seg)

    def emit_output(s, y):
        ys[seg_rows(s), :] = y
        b = s // segs_per_blk
        rows = ys[pl.ds(pl.multiple_of(b * LANES, LANES), LANES), :]
        outT[b] = rows.T.astype(BF16)

    def new_ffn(before_chunk=None):
        return _Ffn(f_in[...], (w13_main, w13_rest, w2_main, w2_rest), before_chunk)

    def store_attention(rows, tokens):
        a_out[rows, :] = tokens
        f_in[rows, :] = _layernorm(tokens)

    def load_x_block(b):
        start = b * LANES if isinstance(b, int) else pl.multiple_of(b * LANES, LANES)
        xs[pl.ds(start, LANES), :] = xT[b].astype(F32).T.astype(BF16)

    pairs = n_heads // 2
    half_blocks = HALF // RELAYOUT_ROWS

    def x_load(b, relayout):
        return xT_hbm.at[:, b * LANES:(b + 1) * LANES], xT.at[b], relayout

    def qkv_loads(m, src):
        def head_pair(block, p):
            n = RELAYOUT_ROWS * pairs
            slab = stage.at[m, pl.ds(block * n, n + 2 * pairs)]
            even, odd = (
                _split_words(slab[pl.ds(r * pairs + p, RELAYOUT_ROWS // 2, stride=2 * pairs), :])
                for r in range(2))
            return list(zip(even, odd))

        def split_main(i):
            rows = slice(i * RELAYOUT_ROWS // 2, (i + 1) * RELAYOUT_ROWS // 2)
            for g in range(pairs // 2):
                quads = [head_pair(i + k * half_blocks, 2 * g + n)
                         for k in range(2) for n in range(2)]
                for h in range(2):
                    col = m * HALF + h * head_dim
                    for j, op in enumerate(_strassen_rhs([q[h] for q in quads])):
                        qkv_main[g, j, rows, col:col + head_dim] = op

        def split_rest():
            for p in range(pairs):
                for h, w in enumerate(head_pair(2 * half_blocks, p)):
                    col = ((p % 2) * 3 + m) * HALF + h * head_dim
                    qkv_rest[p // 2, :, col:col + head_dim] = _pack(*w)

        def load(block, relayout):
            rows = pl.ds(block * RELAYOUT_ROWS * pairs, RELAYOUT_ROWS * pairs)
            return src.bitcast(U32).at[rows], stage.at[m, rows], relayout

        out = [load(2 * half_blocks, split_rest)]
        for i in range(half_blocks):
            out += [load(i, lambda: None),
                    load(i + half_blocks, functools.partial(split_main, i))]
        return out

    def store_out_weights(main, block, transposed, rest=None):
        def columns(k, lo, hi):
            return tuple(
                jnp.concatenate([flipped[k, t, pl.ds(r, LANES // 2, stride=2), :]
                                 for t in range(lo // LANES, hi // LANES)], axis=1)
                for r in range(2))

        for k in range(4):
            piece = _pad_rows(transposed(k).astype(F32), flipped.shape[1] * LANES)
            for t in range(2 * HALF // LANES if rest is None else flipped.shape[1]):
                flipped[k, t, :LANES, :] = piece[t * LANES:(t + 1) * LANES].T
        for i in range(2):
            quads = [columns(i + 2 * k, n * HALF, (n + 1) * HALF)
                     for k in range(2) for n in range(2)]
            for j, op in enumerate(_strassen_rhs(quads)):
                main[block, j, i * LANES // 2:(i + 1) * LANES // 2, :] = op
        for k in range(0 if rest is None else 4):
            words = _pack(*columns(k, 2 * HALF, 2 * HALF + LANES))
            rest[block, k * LANES // 2:(k + 1) * LANES // 2, :] = words[:, :rest.shape[-1]]

    def wo_load(g):
        def relayout():
            store_out_weights(wo_main, g, lambda i: woT[g * HEADS_PER_GROUP + i])
            for i in range(HEADS_PER_GROUP):
                wo_rest[g, :, i * head_dim:(i + 1) * head_dim] = pltpu.bitcast(
                    woT[g * HEADS_PER_GROUP + i, 2 * HALF:, :], U32)

        heads = pl.ds(g * HEADS_PER_GROUP, HEADS_PER_GROUP)
        return woT_hbm.at[heads], woT.at[heads], relayout

    def w2_load(c):
        def piece(i):
            return w2T[:, c * FFN_CHUNK + i * LANES:c * FFN_CHUNK + (i + 1) * LANES]

        cols = slice(c * FFN_CHUNK, (c + 1) * FFN_CHUNK)
        return (w2T_hbm.at[:, cols], w2T.at[:, cols],
                lambda: store_out_weights(w2_main, c, piece, w2_rest))

    def w13_load(i, src, raw, c):
        def relayout():
            def piece(row, n_rows, n):
                col = c * FFN_CHUNK + n * HALF
                return pltpu.bitcast(raw[row:row + n_rows, col:col + HALF], U32)

            for r in range(half_blocks):
                quads = [_split_words(piece(k * HALF + r * RELAYOUT_ROWS, RELAYOUT_ROWS, n))
                         for k in range(2) for n in range(2)]
                rows = slice(r * RELAYOUT_ROWS // 2, (r + 1) * RELAYOUT_ROWS // 2)
                for j, op in enumerate(_strassen_rhs(quads)):
                    w13_main[c, j, rows, i * HALF:(i + 1) * HALF] = op
            for n in range(2):
                w13_rest[c, :, (2 * n + i) * HALF:(2 * n + i + 1) * HALF] = (
                    piece(2 * HALF, d_model - 2 * HALF, n))

        cols = slice(c * FFN_CHUNK, (c + 1) * FFN_CHUNK)
        return src.at[:, cols], raw.at[:, cols], relayout

    loads = [x_load(b, functools.partial(load_x_block, b)) for b in range(FIRST_X_BLOCKS)]
    for m, src in enumerate([wq_hbm, wk_hbm, wv_hbm]):
        loads += qkv_loads(m, src)
    n_qkv_loads = len(loads)
    loads += [wo_load(g) for g in range(n_heads // HEADS_PER_GROUP)]
    n_attention_loads = len(loads)
    for c in range(n_chunks):
        loads += [w13_load(0, w1_hbm, w1_raw, c), w13_load(1, w3_hbm, w3_raw, c), w2_load(c)]
    n_weight_loads = len(loads)
    loads += [x_load(b, lambda: None) for b in range(FIRST_X_BLOCKS, n_blk)]
    copies = [pltpu.make_async_copy(src, dst, in_sems.at[i])
              for i, (src, dst, _) in enumerate(loads)]

    started = 0

    def start_loads(upto):
        nonlocal started
        for c in copies[started:upto]:
            c.start()
        started = max(started, min(upto, len(copies)))

    def finish_loads(lo, hi, ahead):
        for i in range(lo, hi):
            copies[i].wait()
        start_loads(hi + ahead)
        for i in range(lo, hi):
            loads[i][2]()

    start_loads(1 + LOADS_AHEAD)
    ys[...] = jnp.zeros(ys.shape, ys.dtype)
    for i in range(n_qkv_loads):
        finish_loads(i, i + 1, LOADS_AHEAD)
    start_loads(n_attention_loads + 3)

    chunks_ready = 0

    def prepare_chunks(upto):
        nonlocal chunks_ready
        for c in range(chunks_ready, min(upto, n_chunks)):
            first = n_attention_loads + 3 * c
            finish_loads(first, first + 3, 3 * CHUNKS_AHEAD)
        chunks_ready = max(chunks_ready, upto)

    def prepare_weights(s, g):
        if s == 0:
            finish_loads(n_qkv_loads + g, n_qkv_loads + g + 1, 3 * CHUNKS_AHEAD)
        prepare_chunks(FILL_CHUNKS[s][g])

    mem0 = mem0_ref[...].astype(F32)
    new_mem = mem0
    for s in range(2):
        tokens, new_mem = attention(
            xs[s * seg:(s + 1) * seg, :].astype(F32), new_mem, ffn=None,
            before_group=functools.partial(prepare_weights, s))
        store_attention(slice(s * seg, (s + 1) * seg), tokens)
    mem[...] = jnp.concatenate([new_mem, mem0], axis=0)
    b_out[...] = a_out[...] + new_ffn(lambda c: prepare_chunks(c + 2)).finish()
    a_out[:seg, :] = a_out[seg:, :]
    f_in[:seg, :] = f_in[seg:, :]
    start_loads(len(loads))
    finish_loads(n_weight_loads, len(loads), 0)

    def step(t):
        ffn, ffn_resid = new_ffn(), a_out[...]
        prev = b_out[...]
        emit_output(jnp.maximum(t - 4, 0), prev[seg:])
        resid = jnp.concatenate([xs[seg_rows(t), :].astype(F32), prev[:seg]], axis=0)
        tokens, new_mem = attention(resid, mem[...], ffn=ffn)
        mem[...] = new_mem
        store_attention(slice(None), tokens)
        load_x_block(jnp.minimum(t // segs_per_blk + 1, n_blk - 1))
        b_out[...] = ffn_resid + ffn.finish()

    def loop_body(t, carry):
        step(t)
        done = t - 4

        @pl.when((done >= 0) & (done % segs_per_blk == segs_per_blk - 1))
        def _():
            out_copy(done // segs_per_blk).start()

        return carry

    lax.fori_loop(2, n_seg, loop_body, 0)

    ffn, ffn_resid = new_ffn(), a_out[...]
    prev = b_out[...]
    emit_output(n_seg - 4, prev[seg:])
    tokens, new_mem = attention(prev[:seg], mem[n_mem:, :], ffn=ffn)
    last = ffn_resid + ffn.finish()
    store_attention(slice(0, seg), tokens)
    emit_output(n_seg - 3, last[seg:])
    tokens, _ = attention(last[:seg], new_mem, ffn=None, update_mem=False)
    store_attention(slice(seg, 2 * seg), tokens)
    last = a_out[...] + new_ffn().finish()
    ys[(n_seg - 2) * seg:(n_seg - 1) * seg, :] = last[:seg]
    emit_output(n_seg - 1, last[seg:])
    out_copy(n_blk - 1).start()
    for b in range(n_blk):
        out_copy(b).wait()


@functools.partial(jax.jit, static_argnames=("A_seg_len",))
def pallas_interleave_layers__memory_aug_recurrent_mem_tr__glu_gated_swiglu__prompt_kernel(
    A_x, A_mem0, A_Wq, A_Wk, A_Wv, A_Wo, A_seg_len, B_x, B_w1, B_w3, B_w2,
):
    del B_x
    batch, seq, d_model = A_x.shape
    _, n_heads, head_dim = A_Wq.shape
    n_mem = A_mem0.shape[1]
    d_ff = B_w1.shape[1]
    seg = int(A_seg_len)
    n_seg = seq // seg
    assert batch == 1 and n_seg * seg == seq and LANES == 4 * seg and seq % LANES == 0
    assert head_dim == LANES and n_heads % HEADS_PER_GROUP == 0 and d_ff % FFN_CHUNK == 0

    n_groups = n_heads // HEADS_PER_GROUP
    n_chunks = d_ff // FFN_CHUNK
    rest = d_model - 2 * HALF
    assert rest == RELAYOUT_ROWS
    hbm = pl.BlockSpec(memory_space=pl.ANY)
    outT = pl.pallas_call(
        functools.partial(_kernel, seg=seg, n_seg=n_seg, n_heads=n_heads, head_dim=head_dim),
        out_shape=jax.ShapeDtypeStruct((d_model, seq), A_x.dtype),
        in_specs=[hbm, pl.BlockSpec(memory_space=pltpu.VMEM)] + [hbm] * 7,
        out_specs=hbm,
        scratch_shapes=[
            pltpu.VMEM((3, (d_model + 2) * n_heads // 2, head_dim), U32),
            pltpu.VMEM((n_heads, d_model, head_dim), BF16),
            pltpu.VMEM((d_model, d_ff), BF16),
            pltpu.VMEM((d_model, d_ff), BF16),
            pltpu.VMEM((d_model, d_ff), BF16),
            pltpu.VMEM((4, pl.cdiv(d_model, LANES), LANES + 8, LANES), F32),
            pltpu.VMEM((n_groups, 7, HALF // 2, 3 * HALF), U32),
            pltpu.VMEM((n_groups, rest // 2, 6 * HALF), U32),
            pltpu.VMEM((n_groups, 7, HALF // 2, HALF), U32),
            pltpu.VMEM((n_groups, rest // 2, 2 * HALF), U32),
            pltpu.VMEM((n_chunks, 7, HALF // 2, 2 * HALF), U32),
            pltpu.VMEM((n_chunks, rest // 2, 4 * HALF), U32),
            pltpu.VMEM((n_chunks, 7, HALF // 2, HALF), U32),
            pltpu.VMEM((n_chunks, HALF, rest), U32),
            pltpu.VMEM((seq // LANES, d_model, LANES), BF16),
            pltpu.VMEM((seq, d_model), BF16),
            pltpu.VMEM((seq, d_model), F32),
            pltpu.VMEM((seq // LANES, d_model, LANES), BF16),
            pltpu.VMEM((2 * n_mem, d_model), F32),
            pltpu.VMEM((2 * seg, d_model), F32),
            pltpu.VMEM((2 * seg, d_model), F32),
            pltpu.VMEM((2 * seg, d_model), F32),
            pltpu.SemaphoreType.DMA((3 * d_model // RELAYOUT_ROWS + n_groups + 3 * n_chunks + seq // LANES,)),
            pltpu.SemaphoreType.DMA((seq // LANES,)),
        ],
        compiler_params=pltpu.CompilerParams(vmem_limit_bytes=120 * 2**20),
    )(
        A_x.reshape(seq, d_model).T,
        A_mem0.reshape(n_mem, d_model),
        A_Wq.reshape(d_model * n_heads, head_dim),
        A_Wk.reshape(d_model * n_heads, head_dim),
        A_Wv.reshape(d_model * n_heads, head_dim),
        A_Wo.transpose(0, 2, 1),
        B_w1,
        B_w3,
        B_w2.T,
    )
    return outT.T.reshape(batch, seq, d_model)
```

```python
import functools
import math

import jax
import jax.numpy as jnp
from jax import lax
import jax.experimental.pallas as pl
import jax.experimental.pallas.tpu as pltpu

F32 = jnp.float32
BF16 = jnp.bfloat16
U32 = jnp.uint32
LANES = 128
HEADS_PER_GROUP = 4
HALF = 2 * LANES
FFN_CHUNK = 2 * HALF
RELAYOUT_ROWS = 64
FIRST_X_BLOCKS = 5
LOADS_AHEAD = 8
FILL_CHUNKS = ((0, 0, 0, 0, 0, 0, 0, 0), (1, 1, 2, 2, 3, 3, 4, 4))
CHUNKS_AHEAD = 5
FILL_START = 2
FILL_SOFTMAX = (3, 3, 3, 3, 3, 2, 2, 2)
FILL_LAST = 1
LN_EPS = 1e-5
MASK_VALUE = -1000000000.0
LOG2E = math.log2(math.e)
NT_DIMS = (((1,), (1,)), ((), ()))


def _pack(even_rows, odd_rows):
    return pltpu.pack_elementwise([even_rows, odd_rows], packed_dtype=BF16).astype(U32)


def _split_words(words):
    return (lax.bitcast_convert_type(words << 16, F32),
            lax.bitcast_convert_type(words & jnp.uint32(0xFFFF0000), F32))


def _layernorm(x):
    mean = jnp.mean(x, axis=-1, keepdims=True)
    cen = x - mean
    var = jnp.mean(cen * cen, axis=-1, keepdims=True)
    return cen * lax.rsqrt(var + LN_EPS)


def _dot(lhs, packed_rhs):
    return jnp.dot(lhs, pltpu.bitcast(packed_rhs, BF16), preferred_element_type=F32)


def _strassen_rhs(quads):
    def operands(b11, b12, b21, b22):
        return [b11 + b22, b11, b12 - b22, b21 - b11, b22, b11 + b12, b21 + b22]

    return [_pack(even, odd) for even, odd in
            zip(operands(*(q[0] for q in quads)), operands(*(q[1] for q in quads)))]


def _pad_rows(x, rows):
    if x.shape[0] == rows:
        return x
    return jnp.concatenate([x, jnp.zeros((rows - x.shape[0], x.shape[1]), x.dtype)], axis=0)


def _strassen_lhs(left, right, top):
    a11, a12 = left[:top], right[:top]
    if left.shape[0] == top:
        ops = [a11, None, a11, None, a11 + a12, None, a12]
    else:
        a21, a22 = left[top:], right[top:]
        a22_tall = _pad_rows(a22, top)
        ops = [a11 + a22_tall, a21 + a22, a11, a22, a11 + a12,
               a21 - a11[:a21.shape[0]], a12 - a22_tall]
    return [None if op is None else op.astype(BF16) for op in ops]


def _strassen_combine(m):
    m1, m2, m3, m4, m5, m6, m7 = m
    if m2 is None:
        return m1 - m5 + m7, m3 + m5
    bottom = m2.shape[0]
    left = [m1 + _pad_rows(m4, m1.shape[0]) - m5 + m7, m2 + m4]
    right = [m3 + m5, m1[:bottom] - m2 + m3[:bottom] + m6]
    return jnp.concatenate(left, axis=0), jnp.concatenate(right, axis=0)


class _InProjection:
    def __init__(self, x, top, w_main, w_rest):
        self.ops = _strassen_lhs(x[:, :HALF], x[:, HALF:2 * HALF], top)
        self.rest = x[:, 2 * HALF:].astype(BF16)
        self.w_main, self.w_rest = w_main, w_rest

    def tile(self, block, n):
        cols = slice(n * LANES, (n + 1) * LANES)
        width = self.w_main.shape[-1]
        left, right = _strassen_combine(
            [None if op is None else _dot(op, self.w_main[block, j, :, cols])
             for j, op in enumerate(self.ops)])
        rest = [_dot(self.rest, self.w_rest[block, :, base + n * LANES:base + (n + 1) * LANES])
                for base in (0, width)]
        return left + rest[0], right + rest[1]


class _OutProjection:
    def __init__(self, top, w_main, w_rest, rest_transposed=False):
        self.top, self.w_main, self.w_rest = top, w_main, w_rest
        self.rest_transposed = rest_transposed
        self.acc = None

    def add(self, block, left, right):
        parts = [None if op is None else _dot(op, self.w_main[block, j])
                 for j, op in enumerate(_strassen_lhs(left, right, self.top))]
        both = jnp.concatenate([left, right], axis=1).astype(BF16)
        if self.rest_transposed:
            parts.append(lax.dot_general(pltpu.bitcast(self.w_rest[block], BF16), both, NT_DIMS,
                                         preferred_element_type=F32))
        else:
            parts.append(_dot(both, self.w_rest[block]))
        if self.acc is None:
            self.acc = parts
        else:
            self.acc = [None if a is None else a + b for a, b in zip(self.acc, parts)]

    def result(self):
        rest = self.acc[7].T if self.rest_transposed else self.acc[7]
        return jnp.concatenate([*_strassen_combine(self.acc[:7]), rest], axis=1)


class _Ffn:
    def __init__(self, normed, weights, before_chunk=None):
        in_main, in_rest, out_main, out_rest = weights
        top = normed.shape[0] // 2
        self.project = _InProjection(normed, top, in_main, in_rest)
        self.output = _OutProjection(top, out_main, out_rest)
        self.before_chunk = before_chunk
        self.partial, self.hidden = {}, {}
        n_chunks = in_main.shape[0]
        self.todo = []
        for c in range(n_chunks):
            self.todo += [(self._begin, c), (self._activate, c)]
            if c > 0:
                self.todo.append((self._down, c - 1))
        self.todo.append((self._down, n_chunks - 1))

    def _hidden_tile(self, c, n):
        gate = self.project.tile(c, n)
        up = self.project.tile(c, HALF // LANES + n)
        return [g * jax.nn.sigmoid(g) * u for g, u in zip(gate, up)]

    def _begin(self, c):
        if self.before_chunk is not None:
            self.before_chunk(c)
        self.partial[c] = self._hidden_tile(c, 0)

    def _activate(self, c):
        self.hidden[c] = [jnp.concatenate(pair, axis=1)
                          for pair in zip(self.partial.pop(c), self._hidden_tile(c, 1))]

    def _down(self, c):
        self.output.add(c, *self.hidden.pop(c))

    def run(self, count):
        for fn, c in self.todo[:count]:
            fn(c)
        self.todo = self.todo[count:]

    def finish(self):
        self.run(len(self.todo))
        return self.output.result()


def _attention_mask(rows, seg, n_mem):
    def describe(axis):
        i = lax.broadcasted_iota(jnp.int32, (rows, rows), axis)
        second = i >= seg + n_mem
        pos = jnp.where(second, i - seg - n_mem, jnp.where(i < seg, i + n_mem, i - seg))
        return second.astype(jnp.int32), pos

    q_layer, q_pos = describe(0)
    k_layer, k_pos = describe(1)
    same = q_layer == k_layer
    visible = same & ((q_pos < n_mem) | (q_pos >= k_pos))
    fill = jnp.where(same, MASK_VALUE * LOG2E, -jnp.inf).astype(F32)
    return visible, fill


def _attention(resid, mem, ffn, before_group=None, update_mem=True, *, weights, seg, head_dim):
    in_main, in_rest, out_main, out_rest = weights
    n_groups = in_main.shape[0]
    mem_rows = mem.shape[0]
    top = seg + mem_rows
    normed = _layernorm(resid)
    stacked = [normed[:seg], mem] + ([normed[seg:]] if resid.shape[0] > seg else [])
    stacked = jnp.concatenate(stacked, axis=0)
    visible, fill = _attention_mask(stacked.shape[0], seg, mem_rows * seg // resid.shape[0])
    score_scale = head_dim ** -0.5 * LOG2E
    projection = _InProjection(stacked, top, in_main, in_rest)
    query_projection, query_top = projection, top
    if not update_mem:
        query_projection, query_top = _InProjection(normed, seg, in_main, in_rest), seg
        visible, fill = visible[:seg], fill[:seg]
    output = _OutProjection(query_top, out_main, out_rest, rest_transposed=True)

    def project(g):
        tiles = HALF // LANES
        return [[half.astype(BF16)
                 for half in (query_projection if n < tiles else projection).tile(g, n)]
                for n in range(3 * tiles)]

    def head(qkv, m, i):
        return qkv[2 * m + i % 2][i // 2]

    def scores(qkv):
        probs = []
        for i in range(HEADS_PER_GROUP):
            s = lax.dot_general(head(qkv, 0, i), head(qkv, 1, i), NT_DIMS,
                                preferred_element_type=F32)
            s = jnp.where(visible, s * score_scale, fill)
            p = jnp.exp2(s - jnp.max(s, axis=-1, keepdims=True))
            probs.append((p.astype(BF16), 1.0 / jnp.sum(p, axis=-1, keepdims=True)))
        return probs

    def mix(qkv, probs):
        o = [jnp.dot(p, head(qkv, 2, i), preferred_element_type=F32) * inv
             for i, (p, inv) in enumerate(probs)]
        return jnp.concatenate(o[:2], axis=1), jnp.concatenate(o[2:], axis=1)

    if ffn is not None:
        ffn.run(FILL_START)
        qkv = project(0)
        for g in range(n_groups):
            probs = scores(qkv)
            ffn.run(FILL_SOFTMAX[g % len(FILL_SOFTMAX)])
            o = mix(qkv, probs)
            if g + 1 < n_groups:
                qkv = project(g + 1)
            else:
                ffn.run(FILL_LAST)
            output.add(g, *o)
    else:
        qkv, o = project(0), None
        nxt = project(1)
        for g in range(n_groups):
            if before_group is not None:
                before_group(g)
            probs = scores(qkv)
            if o is not None:
                output.add(g - 1, *o)
            after = project(g + 2) if g + 2 < n_groups else None
            o = mix(qkv, probs)
            qkv, nxt = nxt, after
        output.add(n_groups - 1, *o)
    out = output.result()
    tokens = [out[:seg]] + ([out[top:]] if resid.shape[0] > seg else [])
    return resid + jnp.concatenate(tokens, axis=0), (out[seg:top] if update_mem else None)


def _kernel(xT_hbm, mem0_ref, wq_hbm, wk_hbm, wv_hbm, woT_hbm, w1_hbm, w3_hbm, w2T_hbm,
            outT_hbm,
            stage, woT, w1_raw, w3_raw, w2T, flipped,
            qkv_main, qkv_rest, wo_main, wo_rest, w13_main, w13_rest, w2_main, w2_rest,
            xT, xs, ys, outT,
            mem, a_out, f_in, b_out, in_sems, out_sems,
            *, seg, n_seg, n_heads, head_dim):
    d_model = xs.shape[1]
    n_mem = mem0_ref.shape[0]
    n_chunks = w1_raw.shape[1] // FFN_CHUNK
    segs_per_blk = LANES // seg
    n_blk = n_seg // segs_per_blk
    attention = functools.partial(_attention, weights=(qkv_main, qkv_rest, wo_main, wo_rest),
                                  seg=seg, head_dim=head_dim)

    def out_copy(b):
        cols = pl.ds(pl.multiple_of(b * LANES, LANES), LANES)
        return pltpu.make_async_copy(outT.at[b], outT_hbm.at[:, cols], out_sems.at[b])

    def seg_rows(s):
        return pl.ds(pl.multiple_of(s * seg, seg), seg)

    def emit_output(s, y):
        ys[seg_rows(s), :] = y
        b = s // segs_per_blk
        rows = ys[pl.ds(pl.multiple_of(b * LANES, LANES), LANES), :]
        outT[b] = rows.T.astype(BF16)

    def new_ffn(before_chunk=None):
        return _Ffn(f_in[...], (w13_main, w13_rest, w2_main, w2_rest), before_chunk)

    def store_attention(rows, tokens):
        a_out[rows, :] = tokens
        f_in[rows, :] = _layernorm(tokens)

    def load_x_block(b):
        start = b * LANES if isinstance(b, int) else pl.multiple_of(b * LANES, LANES)
        xs[pl.ds(start, LANES), :] = xT[b].astype(F32).T.astype(BF16)

    pairs = n_heads // 2
    half_blocks = HALF // RELAYOUT_ROWS

    def x_load(b, relayout):
        return xT_hbm.at[:, b * LANES:(b + 1) * LANES], xT.at[b], relayout

    def qkv_loads(m, src):
        def head_pair(block, p):
            n = RELAYOUT_ROWS * pairs
            slab = stage.at[m, pl.ds(block * n, n + 2 * pairs)]
            even, odd = (
                _split_words(slab[pl.ds(r * pairs + p, RELAYOUT_ROWS // 2, stride=2 * pairs), :])
                for r in range(2))
            return list(zip(even, odd))

        def split_main(i):
            rows = slice(i * RELAYOUT_ROWS // 2, (i + 1) * RELAYOUT_ROWS // 2)
            for g in range(pairs // 2):
                quads = [head_pair(i + k * half_blocks, 2 * g + n)
                         for k in range(2) for n in range(2)]
                for h in range(2):
                    col = m * HALF + h * head_dim
                    for j, op in enumerate(_strassen_rhs([q[h] for q in quads])):
                        qkv_main[g, j, rows, col:col + head_dim] = op

        def split_rest():
            for p in range(pairs):
                for h, w in enumerate(head_pair(2 * half_blocks, p)):
                    col = ((p % 2) * 3 + m) * HALF + h * head_dim
                    qkv_rest[p // 2, :, col:col + head_dim] = _pack(*w)

        def load(block, relayout):
            rows = pl.ds(block * RELAYOUT_ROWS * pairs, RELAYOUT_ROWS * pairs)
            return src.bitcast(U32).at[rows], stage.at[m, rows], relayout

        out = [load(2 * half_blocks, split_rest)]
        for i in range(half_blocks):
            out += [load(i, lambda: None),
                    load(i + half_blocks, functools.partial(split_main, i))]
        return out

    def store_out_weights(main, block, transposed, rest=None):
        def columns(k, lo, hi):
            return tuple(
                jnp.concatenate([flipped[k, t, pl.ds(r, LANES // 2, stride=2), :]
                                 for t in range(lo // LANES, hi // LANES)], axis=1)
                for r in range(2))

        for k in range(4):
            piece = _pad_rows(transposed(k).astype(F32), flipped.shape[1] * LANES)
            for t in range(2 * HALF // LANES if rest is None else flipped.shape[1]):
                flipped[k, t, :LANES, :] = piece[t * LANES:(t + 1) * LANES].T
        for i in range(2):
            quads = [columns(i + 2 * k, n * HALF, (n + 1) * HALF)
                     for k in range(2) for n in range(2)]
            for j, op in enumerate(_strassen_rhs(quads)):
                main[block, j, i * LANES // 2:(i + 1) * LANES // 2, :] = op
        for k in range(0 if rest is None else 4):
            words = _pack(*columns(k, 2 * HALF, 2 * HALF + LANES))
            rest[block, k * LANES // 2:(k + 1) * LANES // 2, :] = words[:, :rest.shape[-1]]

    def wo_load(g):
        def relayout():
            store_out_weights(wo_main, g, lambda i: woT[g * HEADS_PER_GROUP + i])
            for i in range(HEADS_PER_GROUP):
                wo_rest[g, :, i * head_dim:(i + 1) * head_dim] = pltpu.bitcast(
                    woT[g * HEADS_PER_GROUP + i, 2 * HALF:, :], U32)

        heads = pl.ds(g * HEADS_PER_GROUP, HEADS_PER_GROUP)
        return woT_hbm.at[heads], woT.at[heads], relayout

    def w2_load(c):
        def piece(i):
            return w2T[:, c * FFN_CHUNK + i * LANES:c * FFN_CHUNK + (i + 1) * LANES]

        cols = slice(c * FFN_CHUNK, (c + 1) * FFN_CHUNK)
        return (w2T_hbm.at[:, cols], w2T.at[:, cols],
                lambda: store_out_weights(w2_main, c, piece, w2_rest))

    def w13_load(i, src, raw, c):
        def relayout():
            def piece(row, n_rows, n):
                col = c * FFN_CHUNK + n * HALF
                return pltpu.bitcast(raw[row:row + n_rows, col:col + HALF], U32)

            for r in range(half_blocks):
                quads = [_split_words(piece(k * HALF + r * RELAYOUT_ROWS, RELAYOUT_ROWS, n))
                         for k in range(2) for n in range(2)]
                rows = slice(r * RELAYOUT_ROWS // 2, (r + 1) * RELAYOUT_ROWS // 2)
                for j, op in enumerate(_strassen_rhs(quads)):
                    w13_main[c, j, rows, i * HALF:(i + 1) * HALF] = op
            for n in range(2):
                w13_rest[c, :, (2 * n + i) * HALF:(2 * n + i + 1) * HALF] = (
                    piece(2 * HALF, d_model - 2 * HALF, n))

        cols = slice(c * FFN_CHUNK, (c + 1) * FFN_CHUNK)
        return src.at[:, cols], raw.at[:, cols], relayout

    loads = [x_load(b, functools.partial(load_x_block, b)) for b in range(FIRST_X_BLOCKS)]
    for m, src in enumerate([wq_hbm, wk_hbm, wv_hbm]):
        loads += qkv_loads(m, src)
    n_qkv_loads = len(loads)
    loads += [wo_load(g) for g in range(n_heads // HEADS_PER_GROUP)]
    n_attention_loads = len(loads)
    for c in range(n_chunks):
        loads += [w13_load(0, w1_hbm, w1_raw, c), w13_load(1, w3_hbm, w3_raw, c), w2_load(c)]
    n_weight_loads = len(loads)
    loads += [x_load(b, lambda: None) for b in range(FIRST_X_BLOCKS, n_blk)]
    copies = [pltpu.make_async_copy(src, dst, in_sems.at[i])
              for i, (src, dst, _) in enumerate(loads)]

    started = 0

    def start_loads(upto):
        nonlocal started
        for c in copies[started:upto]:
            c.start()
        started = max(started, min(upto, len(copies)))

    def finish_loads(lo, hi, ahead):
        for i in range(lo, hi):
            copies[i].wait()
        start_loads(hi + ahead)
        for i in range(lo, hi):
            loads[i][2]()

    start_loads(1 + LOADS_AHEAD)
    ys[...] = jnp.zeros(ys.shape, ys.dtype)
    for i in range(n_qkv_loads):
        finish_loads(i, i + 1, LOADS_AHEAD)
    start_loads(n_attention_loads + 3)

    chunks_ready = 0

    def prepare_chunks(upto):
        nonlocal chunks_ready
        for c in range(chunks_ready, min(upto, n_chunks)):
            first = n_attention_loads + 3 * c
            finish_loads(first, first + 3, 3 * CHUNKS_AHEAD)
        chunks_ready = max(chunks_ready, upto)

    def prepare_weights(s, g):
        if s == 0:
            finish_loads(n_qkv_loads + g, n_qkv_loads + g + 1, 3 * CHUNKS_AHEAD)
        prepare_chunks(FILL_CHUNKS[s][g])

    mem0 = mem0_ref[...].astype(F32)
    new_mem = mem0
    for s in range(2):
        tokens, new_mem = attention(
            xs[s * seg:(s + 1) * seg, :].astype(F32), new_mem, ffn=None,
            before_group=functools.partial(prepare_weights, s))
        store_attention(slice(s * seg, (s + 1) * seg), tokens)
    mem[...] = jnp.concatenate([new_mem, mem0], axis=0)
    b_out[...] = a_out[...] + new_ffn(lambda c: prepare_chunks(c + 2)).finish()
    a_out[:seg, :] = a_out[seg:, :]
    f_in[:seg, :] = f_in[seg:, :]
    start_loads(len(loads))
    finish_loads(n_weight_loads, len(loads), 0)

    def step(t):
        ffn, ffn_resid = new_ffn(), a_out[...]
        prev = b_out[...]
        emit_output(jnp.maximum(t - 4, 0), prev[seg:])
        resid = jnp.concatenate([xs[seg_rows(t), :].astype(F32), prev[:seg]], axis=0)
        tokens, new_mem = attention(resid, mem[...], ffn=ffn)
        mem[...] = new_mem
        store_attention(slice(None), tokens)
        load_x_block(jnp.minimum(t // segs_per_blk + 1, n_blk - 1))
        b_out[...] = ffn_resid + ffn.finish()

    def loop_body(t, carry):
        step(t)
        done = t - 4

        @pl.when((done >= 0) & (done % segs_per_blk == segs_per_blk - 1))
        def _():
            out_copy(done // segs_per_blk).start()

        return carry

    lax.fori_loop(2, n_seg, loop_body, 0)

    ffn, ffn_resid = new_ffn(), a_out[...]
    prev = b_out[...]
    emit_output(n_seg - 4, prev[seg:])
    tokens, new_mem = attention(prev[:seg], mem[n_mem:, :], ffn=ffn)
    last = ffn_resid + ffn.finish()
    store_attention(slice(0, seg), tokens)
    emit_output(n_seg - 3, last[seg:])
    tokens, _ = attention(last[:seg], new_mem, ffn=None, update_mem=False)
    store_attention(slice(seg, 2 * seg), tokens)
    last = a_out[...] + new_ffn().finish()
    ys[(n_seg - 2) * seg:(n_seg - 1) * seg, :] = last[:seg]
    emit_output(n_seg - 1, last[seg:])
    out_copy(n_blk - 1).start()
    for b in range(n_blk):
        out_copy(b).wait()


@functools.partial(jax.jit, static_argnames=("A_seg_len",))
def pallas_interleave_layers__memory_aug_recurrent_mem_tr__glu_gated_swiglu__prompt_kernel(
    A_x, A_mem0, A_Wq, A_Wk, A_Wv, A_Wo, A_seg_len, B_x, B_w1, B_w3, B_w2,
):
    del B_x
    batch, seq, d_model = A_x.shape
    _, n_heads, head_dim = A_Wq.shape
    n_mem = A_mem0.shape[1]
    d_ff = B_w1.shape[1]
    seg = int(A_seg_len)
    n_seg = seq // seg
    assert batch == 1 and n_seg * seg == seq and LANES == 4 * seg and seq % LANES == 0
    assert head_dim == LANES and n_heads % HEADS_PER_GROUP == 0 and d_ff % FFN_CHUNK == 0

    n_groups = n_heads // HEADS_PER_GROUP
    n_chunks = d_ff // FFN_CHUNK
    rest = d_model - 2 * HALF
    assert rest == RELAYOUT_ROWS
    hbm = pl.BlockSpec(memory_space=pl.ANY)
    outT = pl.pallas_call(
        functools.partial(_kernel, seg=seg, n_seg=n_seg, n_heads=n_heads, head_dim=head_dim),
        out_shape=jax.ShapeDtypeStruct((d_model, seq), A_x.dtype),
        in_specs=[hbm, pl.BlockSpec(memory_space=pltpu.VMEM)] + [hbm] * 7,
        out_specs=hbm,
        scratch_shapes=[
            pltpu.VMEM((3, (d_model + 2) * n_heads // 2, head_dim), U32),
            pltpu.VMEM((n_heads, d_model, head_dim), BF16),
            pltpu.VMEM((d_model, d_ff), BF16),
            pltpu.VMEM((d_model, d_ff), BF16),
            pltpu.VMEM((d_model, d_ff), BF16),
            pltpu.VMEM((4, pl.cdiv(d_model, LANES), LANES + 8, LANES), F32),
            pltpu.VMEM((n_groups, 7, HALF // 2, 3 * HALF), U32),
            pltpu.VMEM((n_groups, rest // 2, 6 * HALF), U32),
            pltpu.VMEM((n_groups, 7, HALF // 2, HALF), U32),
            pltpu.VMEM((n_groups, rest // 2, 2 * HALF), U32),
            pltpu.VMEM((n_chunks, 7, HALF // 2, 2 * HALF), U32),
            pltpu.VMEM((n_chunks, rest // 2, 4 * HALF), U32),
            pltpu.VMEM((n_chunks, 7, HALF // 2, HALF), U32),
            pltpu.VMEM((n_chunks, HALF, rest), U32),
            pltpu.VMEM((seq // LANES, d_model, LANES), BF16),
            pltpu.VMEM((seq, d_model), BF16),
            pltpu.VMEM((seq, d_model), F32),
            pltpu.VMEM((seq // LANES, d_model, LANES), BF16),
            pltpu.VMEM((2 * n_mem, d_model), F32),
            pltpu.VMEM((2 * seg, d_model), F32),
            pltpu.VMEM((2 * seg, d_model), F32),
            pltpu.VMEM((2 * seg, d_model), F32),
            pltpu.SemaphoreType.DMA((3 * d_model // RELAYOUT_ROWS + n_groups + 3 * n_chunks + seq // LANES,)),
            pltpu.SemaphoreType.DMA((seq // LANES,)),
        ],
        compiler_params=pltpu.CompilerParams(vmem_limit_bytes=120 * 2**20),
    )(
        A_x.reshape(seq, d_model).T,
        A_mem0.reshape(n_mem, d_model),
        A_Wq.reshape(d_model * n_heads, head_dim),
        A_Wk.reshape(d_model * n_heads, head_dim),
        A_Wv.reshape(d_model * n_heads, head_dim),
        A_Wo.transpose(0, 2, 1),
        B_w1,
        B_w3,
        B_w2.T,
    )
    return outT.T.reshape(batch, seq, d_model)
```

```python
import functools
import math

import jax
import jax.numpy as jnp
from jax import lax
import jax.experimental.pallas as pl
import jax.experimental.pallas.tpu as pltpu

F32 = jnp.float32
BF16 = jnp.bfloat16
U32 = jnp.uint32
LANES = 128
HEADS_PER_GROUP = 4
HALF = 2 * LANES
FFN_CHUNK = 2 * HALF
RELAYOUT_ROWS = 64
FIRST_X_BLOCKS = 5
LOADS_AHEAD = 8
FILL_CHUNKS = ((0, 0, 0, 0, 0, 0, 0, 0), (1, 1, 2, 2, 3, 3, 4, 4))
CHUNKS_AHEAD = 5
FILL_START = 2
FILL_SOFTMAX = (3, 3, 3, 3, 3, 2, 2, 2)
FILL_LAST = 1
LN_EPS = 1e-5
MASK_VALUE = -1000000000.0
LOG2E = math.log2(math.e)
NT_DIMS = (((1,), (1,)), ((), ()))


def _pack(even_rows, odd_rows):
    return pltpu.pack_elementwise([even_rows, odd_rows], packed_dtype=BF16).astype(U32)


def _split_words(words):
    return (lax.bitcast_convert_type(words << 16, F32),
            lax.bitcast_convert_type(words & jnp.uint32(0xFFFF0000), F32))


def _layernorm(x):
    mean = jnp.mean(x, axis=-1, keepdims=True)
    cen = x - mean
    var = jnp.mean(cen * cen, axis=-1, keepdims=True)
    return cen * lax.rsqrt(var + LN_EPS)


def _dot(lhs, packed_rhs):
    return jnp.dot(lhs, pltpu.bitcast(packed_rhs, BF16), preferred_element_type=F32)


def _strassen_rhs(quads):
    def operands(b11, b12, b21, b22):
        return [b11 + b22, b11, b12 - b22, b21 - b11, b22, b11 + b12, b21 + b22]

    return [_pack(even, odd) for even, odd in
            zip(operands(*(q[0] for q in quads)), operands(*(q[1] for q in quads)))]


def _pad_rows(x, rows):
    if x.shape[0] == rows:
        return x
    return jnp.concatenate([x, jnp.zeros((rows - x.shape[0], x.shape[1]), x.dtype)], axis=0)


def _strassen_lhs(left, right, top):
    a11, a12 = left[:top], right[:top]
    if left.shape[0] == top:
        ops = [a11, None, a11, None, a11 + a12, None, a12]
    else:
        a21, a22 = left[top:], right[top:]
        a22_tall = _pad_rows(a22, top)
        ops = [a11 + a22_tall, a21 + a22, a11, a22, a11 + a12,
               a21 - a11[:a21.shape[0]], a12 - a22_tall]
    return [None if op is None else op.astype(BF16) for op in ops]


def _strassen_combine(m):
    m1, m2, m3, m4, m5, m6, m7 = m
    if m2 is None:
        return m1 - m5 + m7, m3 + m5
    bottom = m2.shape[0]
    left = [m1 + _pad_rows(m4, m1.shape[0]) - m5 + m7, m2 + m4]
    right = [m3 + m5, m1[:bottom] - m2 + m3[:bottom] + m6]
    return jnp.concatenate(left, axis=0), jnp.concatenate(right, axis=0)


class _InProjection:
    def __init__(self, x, top, w_main, w_rest):
        self.ops = _strassen_lhs(x[:, :HALF], x[:, HALF:2 * HALF], top)
        self.rest = x[:, 2 * HALF:].astype(BF16)
        self.w_main, self.w_rest = w_main, w_rest

    def tile(self, block, n):
        cols = slice(n * LANES, (n + 1) * LANES)
        width = self.w_main.shape[-1]
        left, right = _strassen_combine(
            [None if op is None else _dot(op, self.w_main[block, j, :, cols])
             for j, op in enumerate(self.ops)])
        rest = [_dot(self.rest, self.w_rest[block, :, base + n * LANES:base + (n + 1) * LANES])
                for base in (0, width)]
        return left + rest[0], right + rest[1]


class _OutProjection:
    def __init__(self, top, w_main, w_rest, rest_transposed=False):
        self.top, self.w_main, self.w_rest = top, w_main, w_rest
        self.rest_transposed = rest_transposed
        self.acc = None

    def add(self, block, left, right):
        parts = [None if op is None else _dot(op, self.w_main[block, j])
                 for j, op in enumerate(_strassen_lhs(left, right, self.top))]
        both = jnp.concatenate([left, right], axis=1).astype(BF16)
        if self.rest_transposed:
            parts.append(lax.dot_general(pltpu.bitcast(self.w_rest[block], BF16), both, NT_DIMS,
                                         preferred_element_type=F32))
        else:
            parts.append(_dot(both, self.w_rest[block]))
        if self.acc is None:
            self.acc = parts
        else:
            self.acc = [None if a is None else a + b for a, b in zip(self.acc, parts)]

    def result(self):
        rest = self.acc[7].T if self.rest_transposed else self.acc[7]
        return jnp.concatenate([*_strassen_combine(self.acc[:7]), rest], axis=1)


class _Ffn:
    def __init__(self, normed, weights, before_chunk=None):
        in_main, in_rest, out_main, out_rest = weights
        top = normed.shape[0] // 2
        self.project = _InProjection(normed, top, in_main, in_rest)
        self.output = _OutProjection(top, out_main, out_rest)
        self.before_chunk = before_chunk
        self.partial, self.hidden = {}, {}
        n_chunks = in_main.shape[0]
        self.todo = []
        for c in range(n_chunks):
            self.todo += [(self._begin, c), (self._activate, c)]
            if c > 0:
                self.todo.append((self._down, c - 1))
        self.todo.append((self._down, n_chunks - 1))

    def _hidden_tile(self, c, n):
        gate = self.project.tile(c, n)
        up = self.project.tile(c, HALF // LANES + n)
        return [g * jax.nn.sigmoid(g) * u for g, u in zip(gate, up)]

    def _begin(self, c):
        if self.before_chunk is not None:
            self.before_chunk(c)
        self.partial[c] = self._hidden_tile(c, 0)

    def _activate(self, c):
        self.hidden[c] = [jnp.concatenate(pair, axis=1)
                          for pair in zip(self.partial.pop(c), self._hidden_tile(c, 1))]

    def _down(self, c):
        self.output.add(c, *self.hidden.pop(c))

    def run(self, count):
        for fn, c in self.todo[:count]:
            fn(c)
        self.todo = self.todo[count:]

    def finish(self):
        self.run(len(self.todo))
        return self.output.result()


def _attention_mask(rows, seg, n_mem):
    def describe(axis):
        i = lax.broadcasted_iota(jnp.int32, (rows, rows), axis)
        second = i >= seg + n_mem
        pos = jnp.where(second, i - seg - n_mem, jnp.where(i < seg, i + n_mem, i - seg))
        return second.astype(jnp.int32), pos

    q_layer, q_pos = describe(0)
    k_layer, k_pos = describe(1)
    same = q_layer == k_layer
    visible = same & ((q_pos < n_mem) | (q_pos >= k_pos))
    fill = jnp.where(same, MASK_VALUE * LOG2E, -jnp.inf).astype(F32)
    return visible, fill


def _attention(resid, mem, ffn, before_group=None, update_mem=True, *, weights, seg, head_dim):
    in_main, in_rest, out_main, out_rest = weights
    n_groups = in_main.shape[0]
    mem_rows = mem.shape[0]
    top = seg + mem_rows
    normed = _layernorm(resid)
    stacked = [normed[:seg], mem] + ([normed[seg:]] if resid.shape[0] > seg else [])
    stacked = jnp.concatenate(stacked, axis=0)
    visible, fill = _attention_mask(stacked.shape[0], seg, mem_rows * seg // resid.shape[0])
    score_scale = head_dim ** -0.5 * LOG2E
    projection = _InProjection(stacked, top, in_main, in_rest)
    query_projection, query_top = projection, top
    if not update_mem:
        query_projection, query_top = _InProjection(normed, seg, in_main, in_rest), seg
        visible, fill = visible[:seg], fill[:seg]
    output = _OutProjection(query_top, out_main, out_rest, rest_transposed=True)

    def project(g):
        tiles = HALF // LANES
        return [[half.astype(BF16)
                 for half in (query_projection if n < tiles else projection).tile(g, n)]
                for n in range(3 * tiles)]

    def head(qkv, m, i):
        return qkv[2 * m + i % 2][i // 2]

    def scores(qkv):
        probs = []
        for i in range(HEADS_PER_GROUP):
            s = lax.dot_general(head(qkv, 0, i), head(qkv, 1, i), NT_DIMS,
                                preferred_element_type=F32)
            s = jnp.where(visible, s * score_scale, fill)
            p = jnp.exp2(s - jnp.max(s, axis=-1, keepdims=True))
            probs.append((p.astype(BF16), 1.0 / jnp.sum(p, axis=-1, keepdims=True)))
        return probs

    def mix(qkv, probs):
        o = [jnp.dot(p, head(qkv, 2, i), preferred_element_type=F32) * inv
             for i, (p, inv) in enumerate(probs)]
        return jnp.concatenate(o[:2], axis=1), jnp.concatenate(o[2:], axis=1)

    if ffn is not None:
        ffn.run(FILL_START)
        qkv = project(0)
        for g in range(n_groups):
            probs = scores(qkv)
            ffn.run(FILL_SOFTMAX[g % len(FILL_SOFTMAX)])
            o = mix(qkv, probs)
            if g + 1 < n_groups:
                qkv = project(g + 1)
            else:
                ffn.run(FILL_LAST)
            output.add(g, *o)
    else:
        qkv, o = project(0), None
        nxt = project(1)
        for g in range(n_groups):
            if before_group is not None:
                before_group(g)
            probs = scores(qkv)
            if o is not None:
                output.add(g - 1, *o)
            after = project(g + 2) if g + 2 < n_groups else None
            o = mix(qkv, probs)
            qkv, nxt = nxt, after
        output.add(n_groups - 1, *o)
    out = output.result()
    tokens = [out[:seg]] + ([out[top:]] if resid.shape[0] > seg else [])
    return resid + jnp.concatenate(tokens, axis=0), (out[seg:top] if update_mem else None)


def _kernel(xT_hbm, mem0_ref, wq_hbm, wk_hbm, wv_hbm, woT_hbm, w1_hbm, w3_hbm, w2T_hbm,
            outT_hbm,
            stage, woT, w1_raw, w3_raw, w2T, flipped,
            qkv_main, qkv_rest, wo_main, wo_rest, w13_main, w13_rest, w2_main, w2_rest,
            xT, xs, ys, outT,
            mem, a_out, f_in, b_out, in_sems, out_sems,
            *, seg, n_seg, n_heads, head_dim):
    d_model = xs.shape[1]
    n_mem = mem0_ref.shape[0]
    n_chunks = w1_raw.shape[1] // FFN_CHUNK
    segs_per_blk = LANES // seg
    n_blk = n_seg // segs_per_blk
    attention = functools.partial(_attention, weights=(qkv_main, qkv_rest, wo_main, wo_rest),
                                  seg=seg, head_dim=head_dim)

    def out_copy(b):
        cols = pl.ds(pl.multiple_of(b * LANES, LANES), LANES)
        return pltpu.make_async_copy(outT.at[b], outT_hbm.at[:, cols], out_sems.at[b])

    def seg_rows(s):
        return pl.ds(pl.multiple_of(s * seg, seg), seg)

    def emit_output(s, y):
        ys[seg_rows(s), :] = y
        b = s // segs_per_blk
        rows = ys[pl.ds(pl.multiple_of(b * LANES, LANES), LANES), :]
        outT[b] = rows.T.astype(BF16)

    def new_ffn(before_chunk=None):
        return _Ffn(f_in[...], (w13_main, w13_rest, w2_main, w2_rest), before_chunk)

    def store_attention(rows, tokens):
        a_out[rows, :] = tokens
        f_in[rows, :] = _layernorm(tokens)

    def load_x_block(b):
        start = b * LANES if isinstance(b, int) else pl.multiple_of(b * LANES, LANES)
        xs[pl.ds(start, LANES), :] = xT[b].astype(F32).T.astype(BF16)

    pairs = n_heads // 2
    half_blocks = HALF // RELAYOUT_ROWS

    def x_load(b, relayout):
        return xT_hbm.at[:, b * LANES:(b + 1) * LANES], xT.at[b], relayout

    def qkv_loads(m, src):
        def head_pair(block, p):
            n = RELAYOUT_ROWS * pairs
            slab = stage.at[m, pl.ds(block * n, n + 2 * pairs)]
            even, odd = (
                _split_words(slab[pl.ds(r * pairs + p, RELAYOUT_ROWS // 2, stride=2 * pairs), :])
                for r in range(2))
            return list(zip(even, odd))

        def split_main(i):
            rows = slice(i * RELAYOUT_ROWS // 2, (i + 1) * RELAYOUT_ROWS // 2)
            for g in range(pairs // 2):
                quads = [head_pair(i + k * half_blocks, 2 * g + n)
                         for k in range(2) for n in range(2)]
                for h in range(2):
                    col = m * HALF + h * head_dim
                    for j, op in enumerate(_strassen_rhs([q[h] for q in quads])):
                        qkv_main[g, j, rows, col:col + head_dim] = op

        def split_rest():
            for p in range(pairs):
                for h, w in enumerate(head_pair(2 * half_blocks, p)):
                    col = ((p % 2) * 3 + m) * HALF + h * head_dim
                    qkv_rest[p // 2, :, col:col + head_dim] = _pack(*w)

        def load(block, relayout):
            rows = pl.ds(block * RELAYOUT_ROWS * pairs, RELAYOUT_ROWS * pairs)
            return src.bitcast(U32).at[rows], stage.at[m, rows], relayout

        out = [load(2 * half_blocks, split_rest), load(half_blocks, lambda: None)]
        for i in reversed(range(half_blocks)):
            if i > 0:
                out.append(load(i + half_blocks, lambda: None))
            out.append(load(i, functools.partial(split_main, i)))
        return out

    def store_out_weights(main, block, transposed, rest=None):
        def columns(k, lo, hi):
            return tuple(
                jnp.concatenate([flipped[k, t, pl.ds(r, LANES // 2, stride=2), :]
                                 for t in range(lo // LANES, hi // LANES)], axis=1)
                for r in range(2))

        for k in range(4):
            piece = _pad_rows(transposed(k).astype(F32), flipped.shape[1] * LANES)
            for t in range(2 * HALF // LANES if rest is None else flipped.shape[1]):
                flipped[k, t, :LANES, :] = piece[t * LANES:(t + 1) * LANES].T
        for i in range(2):
            quads = [columns(i + 2 * k, n * HALF, (n + 1) * HALF)
                     for k in range(2) for n in range(2)]
            for j, op in enumerate(_strassen_rhs(quads)):
                main[block, j, i * LANES // 2:(i + 1) * LANES // 2, :] = op
        for k in range(0 if rest is None else 4):
            words = _pack(*columns(k, 2 * HALF, 2 * HALF + LANES))
            rest[block, k * LANES // 2:(k + 1) * LANES // 2, :] = words[:, :rest.shape[-1]]

    def wo_load(g):
        def relayout():
            store_out_weights(wo_main, g, lambda i: woT[g * HEADS_PER_GROUP + i])
            for i in range(HEADS_PER_GROUP):
                wo_rest[g, :, i * head_dim:(i + 1) * head_dim] = pltpu.bitcast(
                    woT[g * HEADS_PER_GROUP + i, 2 * HALF:, :], U32)

        heads = pl.ds(g * HEADS_PER_GROUP, HEADS_PER_GROUP)
        return woT_hbm.at[heads], woT.at[heads], relayout

    def w2_load(c):
        def piece(i):
            return w2T[:, c * FFN_CHUNK + i * LANES:c * FFN_CHUNK + (i + 1) * LANES]

        cols = slice(c * FFN_CHUNK, (c + 1) * FFN_CHUNK)
        return (w2T_hbm.at[:, cols], w2T.at[:, cols],
                lambda: store_out_weights(w2_main, c, piece, w2_rest))

    def w13_load(i, src, raw, c):
        def relayout():
            def piece(row, n_rows, n):
                col = c * FFN_CHUNK + n * HALF
                return pltpu.bitcast(raw[row:row + n_rows, col:col + HALF], U32)

            for r in range(half_blocks):
                quads = [_split_words(piece(k * HALF + r * RELAYOUT_ROWS, RELAYOUT_ROWS, n))
                         for k in range(2) for n in range(2)]
                rows = slice(r * RELAYOUT_ROWS // 2, (r + 1) * RELAYOUT_ROWS // 2)
                for j, op in enumerate(_strassen_rhs(quads)):
                    w13_main[c, j, rows, i * HALF:(i + 1) * HALF] = op
            for n in range(2):
                w13_rest[c, :, (2 * n + i) * HALF:(2 * n + i + 1) * HALF] = (
                    piece(2 * HALF, d_model - 2 * HALF, n))

        cols = slice(c * FFN_CHUNK, (c + 1) * FFN_CHUNK)
        return src.at[:, cols], raw.at[:, cols], relayout

    loads = [x_load(b, functools.partial(load_x_block, b)) for b in range(FIRST_X_BLOCKS)]
    for m, src in enumerate([wq_hbm, wk_hbm, wv_hbm]):
        loads += qkv_loads(m, src)
    n_qkv_loads = len(loads)
    loads += [wo_load(g) for g in range(n_heads // HEADS_PER_GROUP)]
    n_attention_loads = len(loads)
    for c in range(n_chunks):
        loads += [w13_load(0, w1_hbm, w1_raw, c), w13_load(1, w3_hbm, w3_raw, c), w2_load(c)]
    n_weight_loads = len(loads)
    loads += [x_load(b, lambda: None) for b in range(FIRST_X_BLOCKS, n_blk)]
    copies = [pltpu.make_async_copy(src, dst, in_sems.at[i])
              for i, (src, dst, _) in enumerate(loads)]

    started = 0

    def start_loads(upto):
        nonlocal started
        for c in copies[started:upto]:
            c.start()
        started = max(started, min(upto, len(copies)))

    def finish_loads(lo, hi, ahead):
        for i in range(lo, hi):
            copies[i].wait()
        start_loads(hi + ahead)
        for i in range(lo, hi):
            loads[i][2]()

    start_loads(1 + LOADS_AHEAD)
    ys[...] = jnp.zeros(ys.shape, ys.dtype)
    for i in range(n_qkv_loads):
        finish_loads(i, i + 1, LOADS_AHEAD)
    start_loads(n_attention_loads + 3)

    chunks_ready = 0

    def prepare_chunks(upto):
        nonlocal chunks_ready
        for c in range(chunks_ready, min(upto, n_chunks)):
            first = n_attention_loads + 3 * c
            finish_loads(first, first + 3, 3 * CHUNKS_AHEAD)
        chunks_ready = max(chunks_ready, upto)

    def prepare_weights(s, g):
        if s == 0:
            finish_loads(n_qkv_loads + g, n_qkv_loads + g + 1, 3 * CHUNKS_AHEAD)
        prepare_chunks(FILL_CHUNKS[s][g])

    mem0 = mem0_ref[...].astype(F32)
    new_mem = mem0
    for s in range(2):
        tokens, new_mem = attention(
            xs[s * seg:(s + 1) * seg, :].astype(F32), new_mem, ffn=None,
            before_group=functools.partial(prepare_weights, s))
        store_attention(slice(s * seg, (s + 1) * seg), tokens)
    mem[...] = jnp.concatenate([new_mem, mem0], axis=0)
    b_out[...] = a_out[...] + new_ffn(lambda c: prepare_chunks(c + 2)).finish()
    a_out[:seg, :] = a_out[seg:, :]
    f_in[:seg, :] = f_in[seg:, :]
    start_loads(len(loads))
    finish_loads(n_weight_loads, len(loads), 0)

    def step(t):
        ffn, ffn_resid = new_ffn(), a_out[...]
        prev = b_out[...]
        emit_output(jnp.maximum(t - 4, 0), prev[seg:])
        resid = jnp.concatenate([xs[seg_rows(t), :].astype(F32), prev[:seg]], axis=0)
        tokens, new_mem = attention(resid, mem[...], ffn=ffn)
        mem[...] = new_mem
        store_attention(slice(None), tokens)
        load_x_block(jnp.minimum(t // segs_per_blk + 1, n_blk - 1))
        b_out[...] = ffn_resid + ffn.finish()

    def loop_body(t, carry):
        step(t)
        done = t - 4

        @pl.when((done >= 0) & (done % segs_per_blk == segs_per_blk - 1))
        def _():
            out_copy(done // segs_per_blk).start()

        return carry

    lax.fori_loop(2, n_seg, loop_body, 0)

    ffn, ffn_resid = new_ffn(), a_out[...]
    prev = b_out[...]
    emit_output(n_seg - 4, prev[seg:])
    tokens, new_mem = attention(prev[:seg], mem[n_mem:, :], ffn=ffn)
    last = ffn_resid + ffn.finish()
    store_attention(slice(0, seg), tokens)
    emit_output(n_seg - 3, last[seg:])
    tokens, _ = attention(last[:seg], new_mem, ffn=None, update_mem=False)
    store_attention(slice(seg, 2 * seg), tokens)
    last = a_out[...] + new_ffn().finish()
    ys[(n_seg - 2) * seg:(n_seg - 1) * seg, :] = last[:seg]
    emit_output(n_seg - 1, last[seg:])
    out_copy(n_blk - 1).start()
    for b in range(n_blk):
        out_copy(b).wait()


@functools.partial(jax.jit, static_argnames=("A_seg_len",))
def pallas_interleave_layers__memory_aug_recurrent_mem_tr__glu_gated_swiglu__prompt_kernel(
    A_x, A_mem0, A_Wq, A_Wk, A_Wv, A_Wo, A_seg_len, B_x, B_w1, B_w3, B_w2,
):
    del B_x
    batch, seq, d_model = A_x.shape
    _, n_heads, head_dim = A_Wq.shape
    n_mem = A_mem0.shape[1]
    d_ff = B_w1.shape[1]
    seg = int(A_seg_len)
    n_seg = seq // seg
    assert batch == 1 and n_seg * seg == seq and LANES == 4 * seg and seq % LANES == 0
    assert head_dim == LANES and n_heads % HEADS_PER_GROUP == 0 and d_ff % FFN_CHUNK == 0

    n_groups = n_heads // HEADS_PER_GROUP
    n_chunks = d_ff // FFN_CHUNK
    rest = d_model - 2 * HALF
    assert rest == RELAYOUT_ROWS
    hbm = pl.BlockSpec(memory_space=pl.ANY)
    outT = pl.pallas_call(
        functools.partial(_kernel, seg=seg, n_seg=n_seg, n_heads=n_heads, head_dim=head_dim),
        out_shape=jax.ShapeDtypeStruct((d_model, seq), A_x.dtype),
        in_specs=[hbm, pl.BlockSpec(memory_space=pltpu.VMEM)] + [hbm] * 7,
        out_specs=hbm,
        scratch_shapes=[
            pltpu.VMEM((3, (d_model + 2) * n_heads // 2, head_dim), U32),
            pltpu.VMEM((n_heads, d_model, head_dim), BF16),
            pltpu.VMEM((d_model, d_ff), BF16),
            pltpu.VMEM((d_model, d_ff), BF16),
            pltpu.VMEM((d_model, d_ff), BF16),
            pltpu.VMEM((4, pl.cdiv(d_model, LANES), LANES + 8, LANES), F32),
            pltpu.VMEM((n_groups, 7, HALF // 2, 3 * HALF), U32),
            pltpu.VMEM((n_groups, rest // 2, 6 * HALF), U32),
            pltpu.VMEM((n_groups, 7, HALF // 2, HALF), U32),
            pltpu.VMEM((n_groups, rest // 2, 2 * HALF), U32),
            pltpu.VMEM((n_chunks, 7, HALF // 2, 2 * HALF), U32),
            pltpu.VMEM((n_chunks, rest // 2, 4 * HALF), U32),
            pltpu.VMEM((n_chunks, 7, HALF // 2, HALF), U32),
            pltpu.VMEM((n_chunks, HALF, rest), U32),
            pltpu.VMEM((seq // LANES, d_model, LANES), BF16),
            pltpu.VMEM((seq, d_model), BF16),
            pltpu.VMEM((seq, d_model), F32),
            pltpu.VMEM((seq // LANES, d_model, LANES), BF16),
            pltpu.VMEM((2 * n_mem, d_model), F32),
            pltpu.VMEM((2 * seg, d_model), F32),
            pltpu.VMEM((2 * seg, d_model), F32),
            pltpu.VMEM((2 * seg, d_model), F32),
            pltpu.SemaphoreType.DMA((3 * d_model // RELAYOUT_ROWS + n_groups + 3 * n_chunks + seq // LANES,)),
            pltpu.SemaphoreType.DMA((seq // LANES,)),
        ],
        compiler_params=pltpu.CompilerParams(vmem_limit_bytes=120 * 2**20),
    )(
        A_x.reshape(seq, d_model).T,
        A_mem0.reshape(n_mem, d_model),
        A_Wq.reshape(d_model * n_heads, head_dim),
        A_Wk.reshape(d_model * n_heads, head_dim),
        A_Wv.reshape(d_model * n_heads, head_dim),
        A_Wo.transpose(0, 2, 1),
        B_w1,
        B_w3,
        B_w2.T,
    )
    return outT.T.reshape(batch, seq, d_model)
```
